```python
import os as _os
_os.environ.setdefault('JAX_PLATFORMS', 'cpu')
import jax
import jax.numpy as jnp

def _softmax(x, axis=-1):
    return jax.nn.softmax(x, axis=axis)

def _gelu(x):
    return jax.nn.gelu(x, approximate=True)

def _silu(x):
    return jax.nn.silu(x)

def _sigmoid(x):
    return jax.nn.sigmoid(x)

def _layernorm(x, axis=-1, eps=1e-05):
    m = jnp.mean(x, axis=axis, keepdims=True)
    v = jnp.var(x, axis=axis, keepdims=True)
    return (x - m) / jnp.sqrt(v + eps)

def _scatter_add(tgt, idx, src, axis=0):
    return tgt.at[idx].add(src)

def _segment_sum(src, seg, n):
    return jax.ops.segment_sum(src, seg, n)

class _Rng:

    def __init__(self, key):
        self._k = key

    def _next(self):
        self._k, sub = jax.random.split(self._k)
        return sub

    def normal(self, shape):
        return jax.random.normal(self._next(), shape, dtype=jnp.bfloat16)

    def randint(self, lo, hi, shape):
        return jax.random.randint(self._next(), shape, lo, hi, dtype=jnp.int32)

    def uniform(self, shape, lo=0.0, hi=1.0):
        return jax.random.uniform(self._next(), shape, jnp.bfloat16, lo, hi)

    def permutation(self, n):
        return jax.random.permutation(self._next(), n)
kernel_name = 'concat_heads__memory_aug_recurrent_mem_tr__spectral_gfnet__prompt'

def setup_inputs():
    _rng = _Rng(jax.random.key(int.from_bytes(__import__("os").urandom(4), "little")))
    _w = lambda a: (lambda t: t.astype(jnp.bfloat16) if jnp.issubdtype(t.dtype, jnp.floating) else t)(jnp.asarray(a))

    def _A_setup():
        B, S, Dm = (1, 2048, 640)
        H, Dh = (32, 128)
        M, seg = (8, 32)
        seg = min(seg, S)
        S = S // seg * seg
        return {'x': _w((lambda *s: _rng.normal(s) * 0.05)(B, S, Dm)), 'mem0': _w((lambda *s: _rng.normal(s) * 0.4)(B, M, Dm)), 'Wq': _w((lambda *s: _rng.normal(s) * 3.2)(Dm, H, Dh) * Dm ** (-0.5)), 'Wk': _w((lambda *s: _rng.normal(s) * 3.2)(Dm, H, Dh) * Dm ** (-0.5)), 'Wv': _w((lambda *s: _rng.normal(s) * 0.4)(Dm, H, Dh) * Dm ** (-0.5)), 'Wo': _w((lambda *s: _rng.normal(s) * 0.4)(H, Dh, Dm) * (H * Dh) ** (-0.5)), 'seg_len': seg}
    _A_in = _A_setup()

    def _B_setup():
        B, S, D = (1, 2048, 640)
        Df = D // 2 + 1
        return {'x': _w((lambda *s: _rng.normal(s) * 0.05)(B, S, D)), 'w_r': _w((lambda *s: _rng.normal(s) * 0.05)(S, Df) * 0.02), 'w_i': _w((lambda *s: _rng.normal(s) * 0.05)(S, Df) * 0.02)}
    _B_in = _B_setup()
    return {'A_x': _A_in['x'], 'A_mem0': _A_in['mem0'], 'A_Wq': _A_in['Wq'], 'A_Wk': _A_in['Wk'], 'A_Wv': _A_in['Wv'], 'A_Wo': _A_in['Wo'], 'A_seg_len': _A_in['seg_len'], 'B_x': _B_in['x'], 'B_w_r': _B_in['w_r'], 'B_w_i': _B_in['w_i']}

def reference(A_x, A_mem0, A_Wq, A_Wk, A_Wv, A_Wo, A_seg_len, B_x, B_w_r, B_w_i):

    def _A_ref(x, mem0, Wq, Wk, Wv, Wo, seg_len):
        B, S, Dm = x.shape
        H, Dh = (Wq.shape[1], Wq.shape[2])
        M = mem0.shape[1]
        scale = Dh ** (-0.5)
        n_seg = S // seg_len
        L = M + seg_len
        idx = jnp.arange(L)
        mask = (idx[:, None] < M) | (idx[:, None] >= idx[None, :])
        mem = mem0
        outs = []
        for s in range(n_seg):
            xs = x[:, s * seg_len:(s + 1) * seg_len, :].copy()
            h = jnp.concatenate([mem, xs], axis=1)
            q = jnp.einsum('btd,dhe->bhte', h, Wq)
            k = jnp.einsum('btd,dhe->bhte', h, Wk)
            v = jnp.einsum('btd,dhe->bhte', h, Wv)
            scores = jnp.einsum('bhqe,bhke->bhqk', q, k) * scale
            scores = jnp.where(mask[None, None], scores, -1000000000.0)
            p = _softmax(scores, axis=-1)
            o = jnp.einsum('bhqk,bhke->bhqe', p, v)
            o = jnp.einsum('bhte,hed->btd', o, Wo)
            mem = o[:, :M, :].copy()
            outs.append(o[:, M:, :])
        return jnp.concatenate(outs, axis=1)

    def _B_ref(x, w_r, w_i):
        B, S, D = x.shape
        X = (lambda x, axes=(-2, -1): jnp.fft.rfft2(x.astype(jnp.float32), axes=axes))(x, axes=(-2, -1))
        W = w_r + 1j * w_i
        X = X * W
        y = (lambda x, s, axes=(-2, -1): jnp.fft.irfft2(x, s=s, axes=axes).astype(jnp.bfloat16))(X, (S, D), axes=(-2, -1))
        return y
    a = _A_ref(A_x, A_mem0, A_Wq, A_Wk, A_Wv, A_Wo, A_seg_len)
    b = _B_ref(B_x, B_w_r, B_w_i)
    return jnp.concatenate([a, b], axis=-1)
```

```python
import functools

import numpy as np
import jax
import jax.numpy as jnp
from jax import lax
import jax.experimental.pallas as pl
import jax.experimental.pallas.tpu as pltpu

bf16 = jnp.bfloat16
f32 = jnp.float32
u32 = jnp.uint32

S, D = 2048, 640
H, E = 32, 128
M, SEG = 8, 32
L = M + SEG
G = H // 2
DF = D // 2 + 1
HF = D // 2
NT = D // 128
N1, N2 = 16, 128
NPAIR = S // (2 * SEG)
LAG1, LAG2 = 2, 5
CH = (0, 3, 6, 9, 11, 13, 15, 16)
DP = D // 2
WPIECE = 40
WUNIT = 120
WPITCH = 40
XA0 = 64
XPITCH = 24


def _dft_tables():
    d = np.arange(D)[None, :]
    c = np.arange(D)[:, None]
    f = np.where(c <= HF, c, c - HF)
    ang = 2 * np.pi * ((f * d) % D) / D
    fdt = np.where(c <= HF, np.cos(ang), -np.sin(ang))
    s1 = np.arange(N1)[:, None, None]
    s2 = np.arange(N2)[None, :, None]
    k2 = np.arange(N2)[None, None, :]
    a = 2 * np.pi * (((s1 + N1 * s2) * k2) % S) / S
    gm = np.concatenate([np.cos(a), -np.sin(a)], axis=2)
    def cv(v):
        b = v.astype(np.float32).astype(bf16).view(np.uint16).astype(np.uint32)
        return b[..., 0::2, :] | (b[..., 1::2, :] << 16)
    return cv(fdt), cv(gm)


def _fft_list(re, im, sign):
    n = len(re)
    if n == 1:
        return re, im
    er, ei = _fft_list(re[0::2], im[0::2], sign)
    orr, oi = _fft_list(re[1::2], im[1::2], sign)
    h = n // 2
    outr = [None] * n
    outi = [None] * n
    r = np.float32(np.sqrt(0.5))
    for k in range(h):
        a, b = orr[k], oi[k]
        if 4 * k == n:
            if sign > 0:
                outr[k], outi[k] = er[k] - b, ei[k] + a
                outr[k + h], outi[k + h] = er[k] + b, ei[k] - a
            else:
                outr[k], outi[k] = er[k] + b, ei[k] - a
                outr[k + h], outi[k + h] = er[k] - b, ei[k] + a
            continue
        if k == 0:
            tr, ti = a, b
        elif 8 * k == n:
            tr, ti = ((a - b) * r, (a + b) * r) if sign > 0 else ((a + b) * r, (b - a) * r)
        elif 8 * k == 3 * n:
            tr, ti = ((a + b) * (-r), (a - b) * r) if sign > 0 else ((b - a) * r, (a + b) * (-r))
        else:
            c = np.float32(np.cos(2 * np.pi * k / n))
            s = np.float32(sign * np.sin(2 * np.pi * k / n))
            tr, ti = a * c - b * s, a * s + b * c
        outr[k], outi[k] = er[k] + tr, ei[k] + ti
        outr[k + h], outi[k + h] = er[k] - tr, ei[k] - ti
    return outr, outi


def _unzip_rows(a, b):
    lo = (a & u32(0xFFFF)) | (b << 16)
    hi = (a >> 16) | (b & u32(0xFFFF0000))
    return lo, hi


def _kernel(xa_hbm, mem_hbm, wq_hbm, wk_hbm, wv_hbm, wo_hbm, xb_hbm, wr_hbm, wi_hbm,
            fdt_hbm, gm_hbm, out_hbm,
            xa, mem, wraw, wo, xb, wr, wi, fdt, gm,
            wqkv, vre, vim, wt, ob32, oa, ob, o_scr, stash,
            sem_in, sem_xb, sem_w, sem_wo, sem_out):
    def cp(src, dst, sem):
        return pltpu.make_async_copy(src, dst, sem)

    c_fd = cp(fdt_hbm, fdt, sem_in.at[0])
    c_gm = cp(gm_hbm, gm, sem_in.at[1])
    c_wr = cp(wr_hbm, wr, sem_in.at[2])
    c_wi = cp(wi_hbm, wi, sem_in.at[3])
    c_mem = cp(mem_hbm, mem, sem_in.at[4])
    c_xa0 = cp(xa_hbm.at[pl.ds(0, XA0), :], xa.at[pl.ds(0, XA0), :], sem_in.at[5])
    c_xa1 = cp(xa_hbm.at[pl.ds(XA0, S - XA0), :], xa.at[pl.ds(XA0, S - XA0), :], sem_in.at[6])
    xb3 = xb.reshape(NT * N2 // 2, XPITCH, 128)
    wraw3 = wraw.reshape(3 * DP, WPITCH, E)
    c_xb = [cp(xb_hbm.bitcast(u32).at[:, :, pl.ds(j * 128, 128)],
               xb3.at[pl.ds(j * (N2 // 2), N2 // 2), pl.ds(0, N1), :], sem_xb.at[j]) for j in range(NT)]
    c_w = []
    for m, w_hbm in enumerate((wq_hbm, wk_hbm, wv_hbm)):
        for c in range(DP // WPIECE):
            r0 = m * DP + c * WPIECE
            c_w.append(cp(w_hbm.bitcast(u32).at[pl.ds(c * WPIECE, WPIECE)],
                          wraw3.at[pl.ds(r0, WPIECE), pl.ds(0, H), :], sem_w.at[r0 // WUNIT]))
    c_wo = [cp(wo_hbm.bitcast(u32).at[:, pl.ds(j * 128, 128)], wo.at[j], sem_wo.at[j]) for j in range(NT)]
    for c in (c_fd, *c_xb, c_gm, c_wr, c_wi, c_mem, c_xa0):
        c.start()
    for c in (*c_w, *c_wo, c_xa1):
        c.start(priority=1)

    def relayout_wait(u):
        view = wraw3.at[pl.ds(u * WUNIT, WUNIT), pl.ds(0, H), :]
        cp(view, view, sem_w.at[u]).wait()

    def relayout(u):
        rows = pl.ds(pl.multiple_of(u * WUNIT, 8), WUNIT)
        for g in range(G):
            base = u * (WUNIT * WPITCH) + g
            lo, hi = _unzip_rows(wraw[pl.ds(base, WUNIT, stride=WPITCH), :],
                                 wraw[pl.ds(base + G, WUNIT, stride=WPITCH), :])
            wqkv[2 * g, rows, :] = lo
            wqkv[2 * g + 1, rows, :] = hi

    c_fd.wait()
    for c in c_xb:
        c.wait()
    c_gm.wait()
    row8 = lax.broadcasted_iota(jnp.int32, (8, N2), 0)
    first = row8 == 0

    def p12(q, carry):
        los, his = [], []
        for j in range(NT):
            base = j * (N2 // 2) * XPITCH + q
            lo, hi = _unzip_rows(xb[pl.ds(base, N2 // 2, stride=XPITCH), :],
                                 xb[pl.ds(base + N1 // 2, N2 // 2, stride=XPITCH), :])
            los.append(pltpu.bitcast(lo, bf16))
            his.append(pltpu.bitcast(hi, bf16))
        xg = jnp.concatenate([jnp.concatenate(los, axis=1), jnp.concatenate(his, axis=1)], axis=0)
        xdt = lax.dot_general(pltpu.bitcast(fdt[...], bf16), xg, (((1,), (1,)), ((), ())), preferred_element_type=f32)
        for par in range(2):
            s1 = 2 * q + par
            t = jnp.dot(xdt[:, par * N2:(par + 1) * N2].astype(bf16), pltpu.bitcast(gm[s1], bf16),
                        preferred_element_type=f32)
            t1, t2 = t[:, 0:N2], t[:, N2:]
            vre[s1, 0:8] = t1[0:8] - jnp.where(first, 0.0, t2[HF:HF + 8])
            vim[s1, 0:8] = jnp.where(first, 0.0, t1[HF:HF + 8]) + t2[0:8]
            vre[s1, 8:HF] = t1[8:HF] - t2[HF + 8:]
            vim[s1, 8:HF] = t1[HF + 8:] + t2[8:HF]
            vre[s1, HF:HF + 8] = t1[HF:HF + 8]
            vim[s1, HF:HF + 8] = t2[HF:HF + 8]
        return carry
    lax.fori_loop(0, N1 // 2, p12, 0)

    c_wr.wait()
    c_wi.wait()

    def filt(rows, wrows):
        re = [vre[s1, rows, :] for s1 in range(N1)]
        im = [vim[s1, rows, :] for s1 in range(N1)]
        xr, xi = _fft_list(re, im, -1)
        yr, yi = [], []
        for k1 in range(N1):
            a = wr[wrows, k1 * N2:(k1 + 1) * N2].astype(f32)
            b = wi[wrows, k1 * N2:(k1 + 1) * N2].astype(f32)
            yr.append(xr[k1] * a - xi[k1] * b)
            yi.append(xr[k1] * b + xi[k1] * a)
        return _fft_list(yr, yi, +1)

    zr, zi = filt(slice(0, 8), slice(0, 8))
    nr, ni = filt(slice(HF, HF + 8), slice(HF, HF + 1))
    for s1 in range(N1):
        wt[s1, 0:8, 0:N2] = jnp.where(first, 0.5 * zr[s1], zr[s1]).astype(bf16)
        wt[s1, 0:8, N2:] = jnp.where(first, 0.5 * zi[s1], zi[s1]).astype(bf16)
        wt[s1, HF:HF + 8, 0:N2] = jnp.where(first, 0.5 * nr[s1], zi[s1]).astype(bf16)
        wt[s1, HF:HF + 8, N2:] = jnp.where(first, 0.5 * ni[s1], -zr[s1]).astype(bf16)

    def p3(ch, carry):
        r0 = pl.multiple_of(ch * 8, 8)
        zr, zi = filt(pl.ds(r0, 8), pl.ds(r0, 8))
        for s1 in range(N1):
            zib = zi[s1].astype(bf16)
            wt[s1, pl.ds(r0, 8), 0:N2] = zr[s1].astype(bf16)
            wt[s1, pl.ds(r0, 8), N2:] = zib
            wt[s1, pl.ds(HF + r0, 8), 0:N2] = zib
            wt[s1, pl.ds(HF + r0, 8), N2:] = (-zr[s1]).astype(bf16)
        return carry
    lax.fori_loop(1, HF // 8, p3, 0)

    def p45(q, carry):
        relayout_wait(q)
        relayout(q)
        rs = [lax.dot_general(pltpu.bitcast(gm[2 * q + par], bf16), wt[2 * q + par], (((1,), (1,)), ((), ())),
                              preferred_element_type=f32).astype(bf16) for par in range(2)]
        yy = jnp.dot(jnp.concatenate(rs, axis=0), pltpu.bitcast(fdt[...], bf16),
                     preferred_element_type=f32) * (2.0 / (D * S))
        w = pltpu.pack_elementwise([yy[0:N2], yy[N2:]], packed_dtype=bf16)
        for j in range(NT):
            ob32[j, pl.ds(q, N2, stride=N1 // 2), :] = w[:, j * 128:(j + 1) * 128]
        return carry
    lax.fori_loop(0, N1 // 2, p45, 0)

    def p6(i, carry):
        r0 = pl.multiple_of(i * 128, 128)
        for j in range(NT):
            ob[pl.ds(2 * r0, 256), j * 128:(j + 1) * 128] = pltpu.bitcast(ob32[j, pl.ds(r0, 128), :], bf16)
        return carry
    lax.fori_loop(0, S // 256, p6, 0)
    c_ob = cp(ob, out_hbm.at[:, pl.ds(D, D)], sem_out.at[0])
    c_ob.start()

    for c in c_wo:
        c.wait()
    c_mem.wait()
    c_xa0.wait()

    r = lax.broadcasted_iota(jnp.int32, (2 * L, 2 * L), 0)
    c = lax.broadcasted_iota(jnp.int32, (2 * L, 2 * L), 1)
    rb = r >= L
    cb = c >= L
    rr = jnp.where(rb, r - L, r)
    cc = jnp.where(cb, c - L, c)
    mask = (rb == cb) & ((rr < M) | (rr >= cc))
    scale = E ** -0.5

    def step(lhs, even):
        nrow_o = 32 if even else 48
        qkv, ps, acc = {}, {}, [None]

        def proj(g):
            wg = jnp.concatenate([wqkv[2 * g + par, m * DP:(m + 1) * DP, :]
                                  for m in range(3) for par in range(2)], axis=1)
            t = jnp.dot(lhs, pltpu.bitcast(wg, bf16), preferred_element_type=f32)
            col = lambda a, i: a[:, i * E:(i + 1) * E]
            if even:
                stash[g] = t[40:48]
                parts = [jnp.concatenate([col(t, 2 * i)[0:40], col(t, 2 * i + 1)[0:40]], axis=0)
                         for i in range(3)]
            else:
                st = stash[g]
                parts = [jnp.concatenate(
                    [col(t, 2 * i)[0:8], col(st, 2 * i), col(t, 2 * i)[8:32],
                     col(t, 2 * i + 1)[0:8], col(st, 2 * i + 1), col(t, 2 * i + 1)[8:32]], axis=0)
                    for i in range(3)]
            qkv[g] = ((parts[0] * scale).astype(bf16), parts[1].astype(bf16), parts[2].astype(bf16))

        def scores(g):
            q2, k2, _ = qkv[g]
            s = lax.dot_general(q2, k2, (((1,), (1,)), ((), ())), preferred_element_type=f32)
            s = jnp.where(mask, s, -1e9)
            e = jnp.exp(s - jnp.max(s, axis=-1, keepdims=True))
            l = jnp.sum(e, axis=-1, keepdims=True)
            ps[g] = (e * pl.reciprocal(l, approx=True)).astype(bf16)

        def pv(g):
            o2 = jnp.dot(ps[g], qkv[g][2], preferred_element_type=f32)
            o_scr[0:40, (2 * g) * E:(2 * g + 1) * E] = o2[0:40]
            o_scr[0:40, (2 * g + 1) * E:(2 * g + 2) * E] = o2[40:80]

        def wo_chunk(c):
            a, b = CH[c] * 2 * E, CH[c + 1] * 2 * E
            w = jnp.concatenate([wo[j, a // 2:b // 2, :] for j in range(NT)], axis=1)
            t = jnp.dot(o_scr[0:nrow_o, a:b].astype(bf16), pltpu.bitcast(w, bf16), preferred_element_type=f32)
            acc[0] = t if acc[0] is None else acc[0] + t

        ch = 0
        for t in range(G + LAG2):
            if t < G:
                proj(t)
            else:
                assert CH[ch + 1] <= t - LAG2
                wo_chunk(ch)
                ch += 1
            if 0 <= t - LAG1 < G:
                scores(t - LAG1)
            if 0 <= t - LAG2 < G:
                pv(t - LAG2)
        while ch < len(CH) - 1:
            wo_chunk(ch)
            ch += 1
        return acc[0]

    def out_copy(base):
        return cp(oa.at[pl.ds(base, 64), :], out_hbm.at[pl.ds(base, 64), pl.ds(0, D)], sem_out.at[1])

    def body(p, mem_v):
        base = pl.multiple_of(p * 64, 64)

        @pl.when(p == XA0 // 64)
        def _():
            c_xa1.wait()
        xs = xa[pl.ds(base, 64), :].astype(f32)
        lhs = jnp.concatenate([mem_v, xs[0:40]], axis=0).astype(bf16)
        out_e = step(lhs, True)
        o_scr[40:48, :] = o_scr[32:40, :]
        lhs = jnp.concatenate([out_e[0:8], xs[40:64]], axis=0).astype(bf16)
        out_o = step(lhs, False)
        res = jnp.concatenate([out_e[8:32], out_o[40:48], out_o[8:40]], axis=0)
        oa[pl.ds(base, 64), :] = res.astype(bf16)
        out_copy(base).start()
        return out_o[0:8]

    lax.fori_loop(0, NPAIR, body, mem[...].astype(f32))

    c_ob.wait()
    cp(oa, out_hbm.at[:, pl.ds(0, D)], sem_out.at[1]).wait()


@functools.partial(jax.jit, static_argnames=("A_seg_len",))
def pallas_concat_heads__memory_aug_recurrent_mem_tr__spectral_gfnet__prompt_kernel(
    A_x: jax.Array,
    A_mem0: jax.Array,
    A_Wq: jax.Array,
    A_Wk: jax.Array,
    A_Wv: jax.Array,
    A_Wo: jax.Array,
    A_seg_len,
    B_x: jax.Array,
    B_w_r: jax.Array,
    B_w_i: jax.Array,
):
    assert A_seg_len == SEG and A_x.shape == (1, S, D) and B_x.shape == (1, S, D)
    fdt, gm = _dft_tables()
    args = (
        A_x.reshape(S, D), A_mem0.reshape(M, D),
        A_Wq.reshape(DP, 2 * H, E), A_Wk.reshape(DP, 2 * H, E), A_Wv.reshape(DP, 2 * H, E),
        A_Wo.reshape(H * E, D),
        B_x.reshape(N2 // 2, 2 * N1, D), B_w_r.T, B_w_i.T, fdt, gm,
    )
    V = pltpu.VMEM
    scratch = [
        V((S, D), bf16), V((M, D), bf16), V((3 * DP * WPITCH, E), u32), V((NT, H * E // 2, 128), u32),
        V((NT * (N2 // 2) * XPITCH, 128), u32), V((DF, S), bf16), V((DF, S), bf16),
        V((D // 2, D), u32), V((N1, N2 // 2, 2 * N2), u32),
        V((H, 3 * DP, E), u32),
        V((N1, HF + 8, N2), f32), V((N1, HF + 8, N2), f32), V((N1, D, 2 * N2), bf16),
        V((NT, S // 2, 128), u32),
        V((S, D), bf16), V((S, D), bf16), V((48, H * E), f32), V((G, 8, 6 * E), f32),
        pltpu.SemaphoreType.DMA((7,)), pltpu.SemaphoreType.DMA((NT,)),
        pltpu.SemaphoreType.DMA((3 * DP // WUNIT,)),
        pltpu.SemaphoreType.DMA((NT,)), pltpu.SemaphoreType.DMA((2,)),
    ]
    out = pl.pallas_call(
        _kernel,
        out_shape=jax.ShapeDtypeStruct((S, 2 * D), bf16),
        in_specs=[pl.BlockSpec(memory_space=pltpu.HBM)] * len(args),
        out_specs=pl.BlockSpec(memory_space=pl.ANY),
        scratch_shapes=scratch,
        compiler_params=pltpu.CompilerParams(vmem_limit_bytes=110 * 1024 * 1024),
    )(*args)
    return out.reshape(1, S, 2 * D)
```

```python
import numpy as np
import jax
import jax.numpy as jnp
from jax import lax
import jax.experimental.pallas as pl
import jax.experimental.pallas.tpu as pltpu

bf16 = jnp.bfloat16
f32 = jnp.float32
u32 = jnp.uint32

S, D = 2048, 640
H, E = 32, 128
M, SEG = 8, 32
L = M + SEG
G = H // 2
DF = D // 2 + 1
HF = D // 2
NT = D // 128
N1, N2 = 16, 128
NPAIR = S // (2 * SEG)
LAG1, LAG2 = 2, 5
CH = (0, 3, 6, 9, 11, 13, 14, 15, 16)
DP = D // 2
WPIECE = 40
WUNIT = 120
HPITCH = 3 * DP + 8
UB = 2
RB = 4
UA = 4
XA0 = 64 * UA
XPITCH = 24


def _base_tables():
    def cs(num, den):
        ang = 2 * np.pi * (num % den) / den
        return np.cos(ang), np.sin(ang)
    d = np.arange(D)[None, :]
    td = np.concatenate([*cs(np.arange(8)[:, None] * d, D),
                         *cs(8 * np.arange(HF // 8)[:, None] * d, D)], 0)
    k2 = np.arange(N2)[None, :]
    ts = np.concatenate([*cs(np.arange(N1)[:, None] * k2, S),
                         *cs(N1 * np.arange(N2)[:, None] * k2, S)], 0)
    return td.astype(np.float32), ts.astype(np.float32)


def _fft_list(re, im, sign):
    n = len(re)
    if n == 1:
        return re, im
    er, ei = _fft_list(re[0::2], im[0::2], sign)
    orr, oi = _fft_list(re[1::2], im[1::2], sign)
    h = n // 2
    outr = [None] * n
    outi = [None] * n
    r = np.float32(np.sqrt(0.5))
    for k in range(h):
        a, b = orr[k], oi[k]
        if 4 * k == n:
            if sign > 0:
                outr[k], outi[k] = er[k] - b, ei[k] + a
                outr[k + h], outi[k + h] = er[k] + b, ei[k] - a
            else:
                outr[k], outi[k] = er[k] + b, ei[k] - a
                outr[k + h], outi[k + h] = er[k] - b, ei[k] + a
            continue
        if k == 0:
            tr, ti = a, b
        elif 8 * k == n:
            tr, ti = ((a - b) * r, (a + b) * r) if sign > 0 else ((a + b) * r, (b - a) * r)
        elif 8 * k == 3 * n:
            tr, ti = ((a + b) * (-r), (a - b) * r) if sign > 0 else ((b - a) * r, (a + b) * (-r))
        else:
            c = np.float32(np.cos(2 * np.pi * k / n))
            s = np.float32(sign * np.sin(2 * np.pi * k / n))
            tr, ti = a * c - b * s, a * s + b * c
        outr[k], outi[k] = er[k] + tr, ei[k] + ti
        outr[k + h], outi[k + h] = er[k] - tr, ei[k] - ti
    return outr, outi


def _unzip_rows(a, b):
    lo = (a & u32(0xFFFF)) | (b << 16)
    hi = (a >> 16) | (b & u32(0xFFFF0000))
    return lo, hi


def _kernel(xa_hbm, mem_hbm, wq_hbm, wk_hbm, wv_hbm, wo_hbm, xb_hbm, wr_hbm, wi_hbm,
            td_hbm, ts_hbm, out_hbm,
            xa, mem, wraw, wo, xb, wr, wi, td, ts, fdt, gm,
            wqkv, vre, vim, wt, rsc, ob32, obuf, o_scr, stash,
            sem_in, sem_xb, sem_w, sem_wo, sem_out):
    def cp(src, dst, sem):
        return pltpu.make_async_copy(src, dst, sem)

    c_td = cp(td_hbm, td, sem_in.at[0])
    c_ts = cp(ts_hbm, ts, sem_in.at[1])
    c_wr = cp(wr_hbm, wr, sem_in.at[2])
    c_wi = cp(wi_hbm, wi, sem_in.at[3])
    c_mem = cp(mem_hbm, mem, sem_in.at[4])
    c_xa0 = cp(xa_hbm.at[pl.ds(0, XA0), :], xa.at[pl.ds(0, XA0), :], sem_in.at[5])
    c_xa1 = cp(xa_hbm.at[pl.ds(XA0, S - XA0), :], xa.at[pl.ds(XA0, S - XA0), :], sem_in.at[6])
    xb3 = xb.reshape(NT * N2 // 2 + 1, XPITCH, 128)
    c_xb = [cp(xb_hbm.bitcast(u32).at[:, :, pl.ds(j * 128, 128)],
               xb3.at[pl.ds(j * (N2 // 2), N2 // 2), pl.ds(0, N1), :], sem_xb.at[j]) for j in range(NT)]
    c_w = []
    for m, w_hbm in enumerate((wq_hbm, wk_hbm, wv_hbm)):
        for c in range(DP // WPIECE):
            r0 = m * DP + c * WPIECE
            c_w.append(cp(w_hbm.bitcast(u32).at[pl.ds(c * WPIECE, WPIECE)],
                          wraw.at[pl.ds(r0, WPIECE)], sem_w.at[r0 // WUNIT]))
    c_wo = [cp(wo_hbm.bitcast(u32).at[:, pl.ds(j * 128, 128)], wo.at[j], sem_wo.at[0]) for j in range(NT)]
    for c in (c_td, c_ts, *c_xb):
        c.start()
    for c in c_w:
        c.start(priority=1)

    def relayout_wait(u):
        view = wraw.at[pl.ds(u * WUNIT, WUNIT)]
        cp(view, view, sem_w.at[u]).wait()

    def relayout(u, i0, i1, zero=None):
        for i in range(i0, i1):
            dp = u * WUNIT + i
            a, b = wraw[dp, 0:G, :], wraw[dp, G:H, :]
            if zero is not None:
                a = a | zero
            lo, hi = _unzip_rows(a, b)
            wqkv[0, pl.ds(dp, G, stride=HPITCH), :] = lo
            wqkv[1, pl.ds(dp, G, stride=HPITCH), :] = hi

    row8 = lax.broadcasted_iota(jnp.int32, (8, N2), 0)
    first = row8 == 0
    pack = lambda v: pltpu.bitcast(v.astype(bf16), u32)
    c_td.wait()
    cb, sb = td[0:8, :], td[8:16, :]
    na = HF // 8
    lane = lax.broadcasted_iota(jnp.int32, (8, D), 1)
    nyq = jnp.where((lane & 1) == 0, 1.0, -1.0)
    row0 = lax.broadcasted_iota(jnp.int32, (8, D), 0) == 0
    for a2 in range(na // 2):
        cs_, sn_ = [], []
        for a in (2 * a2, 2 * a2 + 1):
            ca, sa = td[16 + a:17 + a, :], td[16 + na + a:17 + na + a, :]
            cs_.append(ca * cb - sa * sb)
            ns = -(sa * cb + ca * sb)
            sn_.append(jnp.where(row0, nyq, ns) if a == 0 else ns)
        fdt[8 * a2:8 * a2 + 8, :] = pack(jnp.concatenate(cs_, axis=0))
        fdt[HF // 2 + 8 * a2:HF // 2 + 8 * a2 + 8, :] = pack(jnp.concatenate(sn_, axis=0))
    c_ts.wait()

    def gen_gm(s1, carry):
        ca, sa = ts[pl.ds(s1, 1), :], ts[pl.ds(N1 + s1, 1), :]
        cb, sb = ts[2 * N1:2 * N1 + N2, :], ts[2 * N1 + N2:, :]
        gm[s1, :, 0:N2] = pack(ca * cb - sa * sb)
        gm[s1, :, N2:] = pack(-(sa * cb + ca * sb))
        return carry
    lax.fori_loop(0, N1, gen_gm, 0)

    for c in c_xb:
        c.wait()
    for c in (c_wr, c_wi, c_mem, c_xa0):
        c.start()

    def p1(q):
        los, his = [], []
        for j in range(NT):
            base = j * (N2 // 2) * XPITCH + q
            lo, hi = _unzip_rows(xb[pl.ds(base, N2 // 2, stride=XPITCH), :],
                                 xb[pl.ds(base + N1 // 2, N2 // 2, stride=XPITCH), :])
            los.append(pltpu.bitcast(lo, bf16))
            his.append(pltpu.bitcast(hi, bf16))
        xg = jnp.concatenate([jnp.concatenate(los, axis=1), jnp.concatenate(his, axis=1)], axis=0)
        return lax.dot_general(pltpu.bitcast(fdt[...], bf16), xg, (((1,), (1,)), ((), ())),
                               preferred_element_type=f32).astype(bf16)

    def p2(q, xdt):
        for par in range(2):
            s1 = 2 * q + par
            t = jnp.dot(xdt[:, par * N2:(par + 1) * N2], pltpu.bitcast(gm[s1], bf16), preferred_element_type=f32)
            t1, t2 = t[:, 0:N2], t[:, N2:]
            vre[s1, 0:8] = t1[0:8] - jnp.where(first, 0.0, t2[HF:HF + 8])
            vim[s1, 0:8] = jnp.where(first, 0.0, t1[HF:HF + 8]) + t2[0:8]
            vre[s1, 8:HF] = t1[8:HF] - t2[HF + 8:]
            vim[s1, 8:HF] = t1[HF + 8:] + t2[8:HF]
            vre[s1, HF:HF + 8] = t1[HF:HF + 8]
            vim[s1, HF:HF + 8] = t2[HF:HF + 8]

    def p12(i, carry):
        xs = [p1(UB * i + k) for k in range(UB)]
        for k in range(UB):
            p2(UB * i + k, xs[k])
        return carry
    lax.fori_loop(0, N1 // 2 // UB, p12, 0)

    c_wr.wait()
    c_wi.wait()

    def filt(rows, wrows):
        re = [vre[s1, rows, :] for s1 in range(N1)]
        im = [vim[s1, rows, :] for s1 in range(N1)]
        xr, xi = _fft_list(re, im, -1)
        yr, yi = [], []
        for k1 in range(N1):
            a = wr[wrows, k1 * N2:(k1 + 1) * N2].astype(f32)
            b = wi[wrows, k1 * N2:(k1 + 1) * N2].astype(f32)
            yr.append(xr[k1] * a - xi[k1] * b)
            yi.append(xr[k1] * b + xi[k1] * a)
        return _fft_list(yr, yi, +1)

    zr, zi = filt(slice(0, 8), slice(0, 8))
    nr, ni = filt(slice(HF, HF + 8), slice(HF, HF + 1))
    for s1 in range(N1):
        wt[s1, 0:8, 0:N2] = jnp.where(first, 0.5 * zr[s1], zr[s1]).astype(bf16)
        wt[s1, 0:8, N2:] = jnp.where(first, 0.5 * zi[s1], zi[s1]).astype(bf16)
        wt[s1, HF:HF + 8, 0:N2] = jnp.where(first, 0.5 * nr[s1], zi[s1]).astype(bf16)
        wt[s1, HF:HF + 8, N2:] = jnp.where(first, 0.5 * ni[s1], -zr[s1]).astype(bf16)

    def p3(ch, carry):
        r0 = pl.multiple_of(ch * 8, 8)
        zr, zi = filt(pl.ds(r0, 8), pl.ds(r0, 8))
        for s1 in range(N1):
            zib = zi[s1].astype(bf16)
            wt[s1, pl.ds(r0, 8), 0:N2] = zr[s1].astype(bf16)
            wt[s1, pl.ds(r0, 8), N2:] = zib
            wt[s1, pl.ds(HF + r0, 8), 0:N2] = zib
            wt[s1, pl.ds(HF + r0, 8), N2:] = (-zr[s1]).astype(bf16)
        return carry
    lax.fori_loop(1, HF // 8, p3, 0)

    for c in c_wo:
        c.start(priority=1)

    def p4(i, carry):
        for k in range(2 * UB):
            s1 = 2 * UB * i + k
            rsc[s1] = pltpu.bitcast(lax.dot_general(
                pltpu.bitcast(gm[s1], bf16), wt[s1], (((1,), (1,)), ((), ())),
                preferred_element_type=f32).astype(bf16), u32)
        return carry
    lax.fori_loop(0, N1 // 2 // UB, p4, 0)

    def p5(i, carry):
        for k in range(UB):
            relayout_wait(UB * i + k)
        zero = None
        npc = WUNIT // (NT * RB)
        hb = N2 // RB
        pc = 0
        for k in range(UB):
            q = UB * i + k
            for rb in range(RB):
                rows = slice(rb * hb // 2, (rb + 1) * hb // 2)
                rc = pltpu.bitcast(jnp.concatenate([rsc[2 * q, rows], rsc[2 * q + 1, rows]], axis=0), bf16)
                for j in range(NT):
                    yy = jnp.dot(rc, pltpu.bitcast(fdt[:, j * 128:(j + 1) * 128], bf16),
                                 preferred_element_type=f32) * (2.0 / (D * S))
                    w = pltpu.pack_elementwise([yy[0:hb], yy[hb:]], packed_dtype=bf16)
                    ob32[j, pl.ds(q + rb * hb * (N1 // 2), hb, stride=N1 // 2), :] = w
                    pc = rb * NT + j
                    relayout(q, pc * npc, (pc + 1) * npc, zero)
                    zero = (pltpu.bitcast(w[0:G], u32) >> 16) >> 16
        return carry
    lax.fori_loop(0, N1 // 2 // UB, p5, 0)

    c_xa1.start(priority=1)

    def p6(i, carry):
        r0 = pl.multiple_of(i * 128, 128)
        for j in range(NT):
            obuf[pl.ds(2 * r0, 256), D + j * 128:D + (j + 1) * 128] = pltpu.bitcast(ob32[j, pl.ds(r0, 128), :], bf16)
        return carry
    lax.fori_loop(0, S // 256, p6, 0)
    c_mem.wait()
    c_xa0.wait()

    r = lax.broadcasted_iota(jnp.int32, (2 * L, 2 * L), 0)
    c = lax.broadcasted_iota(jnp.int32, (2 * L, 2 * L), 1)
    rb = r >= L
    cb = c >= L
    rr = jnp.where(rb, r - L, r)
    cc = jnp.where(cb, c - L, c)
    mask = (rb == cb) & ((rr < M) | (rr >= cc))
    scale = E ** -0.5

    def step(lhs, even):
        nrow_o = 32 if even else 48
        qkv, ps, acc = {}, {}, [None]

        def proj(g):
            wg = jnp.concatenate([wqkv[par, g * HPITCH + m * DP:g * HPITCH + (m + 1) * DP, :]
                                  for m in range(3) for par in range(2)], axis=1)
            t = jnp.dot(lhs, pltpu.bitcast(wg, bf16), preferred_element_type=f32)
            col = lambda a, i: a[:, i * E:(i + 1) * E]
            if even:
                stash[g] = t[40:48]
                parts = [jnp.concatenate([col(t, 2 * i)[32:40], col(t, 2 * i)[0:32],
                                          col(t, 2 * i + 1)[32:40], col(t, 2 * i + 1)[0:32]], axis=0)
                         for i in range(3)]
            else:
                st = stash[g]
                parts = [jnp.concatenate(
                    [col(t, 2 * i)[16:24], col(st, 2 * i), col(t, 2 * i)[24:32], col(t, 2 * i)[0:16],
                     col(t, 2 * i + 1)[16:24], col(st, 2 * i + 1), col(t, 2 * i + 1)[24:32],
                     col(t, 2 * i + 1)[0:16]], axis=0)
                    for i in range(3)]
            qkv[g] = ((parts[0] * scale).astype(bf16), parts[1].astype(bf16), parts[2].astype(bf16))

        def scores(g):
            q2, k2, _ = qkv[g]
            s = lax.dot_general(q2, k2, (((1,), (1,)), ((), ())), preferred_element_type=f32)
            s = jnp.where(mask, s, -1e9)
            e = jnp.exp(s - jnp.max(s, axis=-1, keepdims=True))
            l = jnp.sum(e, axis=-1, keepdims=True)
            ps[g] = (e * pl.reciprocal(l, approx=True)).astype(bf16)

        def pv(g):
            o2 = jnp.dot(ps[g], qkv[g][2], preferred_element_type=f32)
            o_scr[0:40, (2 * g) * E:(2 * g + 1) * E] = o2[0:40]
            o_scr[0:40, (2 * g + 1) * E:(2 * g + 2) * E] = o2[40:80]

        def wo_chunk(c):
            a, b = CH[c] * 2 * E, CH[c + 1] * 2 * E
            w = jnp.concatenate([wo[j, a // 2:b // 2, :] for j in range(NT)], axis=1)
            t = jnp.dot(o_scr[0:nrow_o, a:b].astype(bf16), pltpu.bitcast(w, bf16), preferred_element_type=f32)
            acc[0] = t if acc[0] is None else acc[0] + t

        ch = 0
        for t in range(G + LAG2):
            if t < G:
                proj(t)
            else:
                assert CH[ch + 1] <= t - LAG2
                wo_chunk(ch)
                ch += 1
            if 0 <= t - LAG1 < G:
                scores(t - LAG1)
            if 0 <= t - LAG2 < G:
                pv(t - LAG2)
        while ch < len(CH) - 1:
            wo_chunk(ch)
            ch += 1
        return acc[0]

    def out_copy(p):
        rows = pl.ds(pl.multiple_of(p * 64, 64), 64)
        return cp(obuf.at[rows, :], out_hbm.at[rows, :], sem_out.at[0])

    def pair(p, mem_v):
        base = pl.multiple_of(p * 64, 64)
        xs = xa[pl.ds(base, 64), :].astype(f32)
        lhs = jnp.concatenate([xs[0:32], mem_v, xs[32:40]], axis=0).astype(bf16)
        out_e = step(lhs, True)
        o_scr[40:48, :] = o_scr[32:40, :]
        lhs = jnp.concatenate([xs[48:64], out_e[0:8], xs[40:48]], axis=0).astype(bf16)
        out_o = step(lhs, False)
        res = jnp.concatenate([out_e[8:32], out_o[40:48], out_o[8:40]], axis=0)
        obuf[pl.ds(base, 64), 0:D] = res.astype(bf16)
        return out_o[0:8]

    def body(p, mem_v):
        @pl.when(p == 1)
        def _():
            c_xa1.wait()

        @pl.when(p > 0)
        def _():
            out_copy(p * UA - 1).start()
        for k in range(UA):
            if k > 0:
                out_copy(p * UA + k - 1).start()
            mem_v = pair(p * UA + k, mem_v)
        return mem_v

    cp(wo, wo, sem_wo.at[0]).wait()
    lax.fori_loop(0, NPAIR // UA, body, mem[...].astype(f32))

    out_copy(NPAIR - 1).start()
    cp(obuf, out_hbm, sem_out.at[0]).wait()


@jax.jit
def pallas_concat_heads__memory_aug_recurrent_mem_tr__spectral_gfnet__prompt_kernel(
    A_x: jax.Array,
    A_mem0: jax.Array,
    A_Wq: jax.Array,
    A_Wk: jax.Array,
    A_Wv: jax.Array,
    A_Wo: jax.Array,
    A_seg_len,
    B_x: jax.Array,
    B_w_r: jax.Array,
    B_w_i: jax.Array,
):
    del A_seg_len
    assert A_x.shape == (1, S, D) and B_x.shape == (1, S, D)
    td, ts = _base_tables()
    args = (
        A_x.reshape(S, D), A_mem0.reshape(M, D),
        A_Wq.reshape(DP, 2 * H, E), A_Wk.reshape(DP, 2 * H, E), A_Wv.reshape(DP, 2 * H, E),
        A_Wo.reshape(H * E, D),
        B_x.reshape(N2 // 2, 2 * N1, D), B_w_r.T, B_w_i.T, td, ts,
    )
    V = pltpu.VMEM
    scratch = [
        V((S, D), bf16), V((M, D), bf16), V((3 * DP, H, E), u32), V((NT, H * E // 2, 128), u32),
        V(((NT * (N2 // 2) + 1) * XPITCH, 128), u32), V((DF, S), bf16), V((DF, S), bf16),
        V(td.shape, f32), V(ts.shape, f32), V((D // 2, D), u32), V((N1, N2 // 2, 2 * N2), u32),
        V((2, (G + 1) * HPITCH, E), u32),
        V((N1, HF + 8, N2), f32), V((N1, HF + 8, N2), f32), V((N1, D, 2 * N2), bf16),
        V((N1, N2 // 2, D), u32),
        V((NT, S // 2 + 8, 128), u32),
        V((S, 2 * D), bf16), V((48, H * E), f32), V((G, 8, 6 * E), f32),
        pltpu.SemaphoreType.DMA((7,)), pltpu.SemaphoreType.DMA((NT,)),
        pltpu.SemaphoreType.DMA((3 * DP // WUNIT,)),
        pltpu.SemaphoreType.DMA((1,)), pltpu.SemaphoreType.DMA((1,)),
    ]
    out = pl.pallas_call(
        _kernel,
        out_shape=jax.ShapeDtypeStruct((S, 2 * D), bf16),
        in_specs=[pl.BlockSpec(memory_space=pltpu.HBM)] * len(args),
        out_specs=pl.BlockSpec(memory_space=pl.ANY),
        scratch_shapes=scratch,
        compiler_params=pltpu.CompilerParams(vmem_limit_bytes=110 * 1024 * 1024, disable_bounds_checks=True),
    )(*args)
    return out.reshape(1, S, 2 * D)
```

```python
import numpy as np
import jax
import jax.numpy as jnp
from jax import lax
import jax.experimental.pallas as pl
import jax.experimental.pallas.tpu as pltpu

bf16 = jnp.bfloat16
f32 = jnp.float32
u32 = jnp.uint32

S, D = 2048, 640
H, E = 32, 128
M, SEG = 8, 32
L = M + SEG
G = H // 2
DF = D // 2 + 1
HF = D // 2
NT = D // 128
N1, N2 = 16, 128
NPAIR = S // (2 * SEG)
LAG1, LAG2 = 2, 5
CH = (0, 3, 6, 9, 11, 13, 14, 15, 16)
DP = D // 2
WPIECE = 40
NPIECE = 3 * DP // WPIECE
NQ = DP // WPIECE
QPITCH = DP + 8
KPITCH = 2 * DP + 8
UB = 2
RB = 4
FG = [(4, 4), (8, 4), (12, 4), (14, 4)]
NF1 = 2
NBQ = 8
RLP = 10
XG = 8
UF = 1
B0 = 1
UA = 4
QP = 16
XPITCH = 24
C5 = (float(np.cos(2 * np.pi / 5)), float(np.cos(4 * np.pi / 5)))
S5 = (float(np.sin(2 * np.pi / 5)), float(np.sin(4 * np.pi / 5)))
HI16 = 0xFFFF0000


def _cos_sin(num, den):
    r = num - den * jnp.floor((num + 0.5) * (1.0 / den))
    ang = r * (2.0 * np.pi / den)
    return jnp.cos(ang), jnp.sin(ang)


def _fft_list(re, im, sign):
    n = len(re)
    if n == 1:
        return re, im
    er, ei = _fft_list(re[0::2], im[0::2], sign)
    orr, oi = _fft_list(re[1::2], im[1::2], sign)
    h = n // 2
    outr = [None] * n
    outi = [None] * n
    r = np.float32(np.sqrt(0.5))
    for k in range(h):
        a, b = orr[k], oi[k]
        if 4 * k == n:
            if sign > 0:
                outr[k], outi[k] = er[k] - b, ei[k] + a
                outr[k + h], outi[k + h] = er[k] + b, ei[k] - a
            else:
                outr[k], outi[k] = er[k] + b, ei[k] - a
                outr[k + h], outi[k + h] = er[k] - b, ei[k] + a
            continue
        if k == 0:
            tr, ti = a, b
        elif 8 * k == n:
            tr, ti = ((a - b) * r, (a + b) * r) if sign > 0 else ((a + b) * r, (b - a) * r)
        elif 8 * k == 3 * n:
            tr, ti = ((a + b) * (-r), (a - b) * r) if sign > 0 else ((b - a) * r, (a + b) * (-r))
        else:
            c = np.float32(np.cos(2 * np.pi * k / n))
            s = np.float32(sign * np.sin(2 * np.pi * k / n))
            tr, ti = a * c - b * s, a * s + b * c
        outr[k], outi[k] = er[k] + tr, ei[k] + ti
        outr[k + h], outi[k + h] = er[k] - tr, ei[k] - ti
    return outr, outi


def _unzip_rows(a, b):
    lo = (a & u32(0xFFFF)) | (b << 16)
    hi = (a >> 16) | (b & u32(HI16))
    return lo, hi


def _radix5(x):
    t1, t2, t3, t4 = x[1] + x[4], x[2] + x[3], x[1] - x[4], x[2] - x[3]
    return (x[0] + t1 + t2,
            x[0] + C5[0] * t1 + C5[1] * t2, S5[0] * t3 + S5[1] * t4,
            x[0] + C5[1] * t1 + C5[0] * t2, S5[1] * t3 - S5[0] * t4)


def _radix5_t(z0, zc1, zs1, zc2, zs2, k):
    z0 = z0 * k
    p1 = z0 + (k * C5[0]) * zc1 + (k * C5[1]) * zc2
    p2 = z0 + (k * C5[1]) * zc1 + (k * C5[0]) * zc2
    q1 = (k * S5[0]) * zs1 + (k * S5[1]) * zs2
    q2 = (k * S5[1]) * zs1 - (k * S5[0]) * zs2
    return z0 + (zc1 + zc2) * k, p1 + q1, p2 + q2, p2 - q2, p1 - q1


def _kernel(xa_hbm, mem_hbm, wq_hbm, wk_hbm, wv_hbm, wo_hbm, xb_hbm, wr_hbm, wi_hbm,
            out_hbm,
            xa, mem, wraw, wo, xb, wf, wn, ts, tt, ti, gm,
            wq, wkv, vre, vim, wt, rsc, ob32, xpk, qpre, obuf, o_scr, stash, fstash,
            sem_in, sem_xb, sem_f, sem_w, sem_wo, sem_out, sem_ob):
    def cp(src, dst, sem):
        return pltpu.make_async_copy(src, dst, sem)

    def xa_copy(p0, n, r0, nr, sem):
        return cp(xa_hbm.at[pl.ds(p0, n), pl.ds(r0, nr), :], xa.at[pl.ds(p0, n), pl.ds(r0, nr), :], sem)

    c_mem = cp(mem_hbm, mem, sem_in.at[0])
    c_xp = xa_copy(0, NPAIR, 0, QP, sem_in.at[1])
    c_xa0 = xa_copy(0, UA + 1, QP, 64 - QP, sem_in.at[2])
    c_xa1 = xa_copy(UA + 1, NPAIR - UA - 1, QP, 64 - QP, sem_in.at[3])
    c_n = [cp(w.at[pl.ds(HF, 1), :], wn.at[i], sem_in.at[4 + i]) for i, w in enumerate((wr_hbm, wi_hbm))]
    xb3 = xb.reshape(NT * N2 // 2 + 1, XPITCH, 128)
    xr = N2 // 2 // XG
    c_xb = [cp(xb_hbm.bitcast(u32).at[pl.ds(k * xr, xr), :, pl.ds(j * 128, 128)],
               xb3.at[pl.ds(j * (N2 // 2) + k * xr, xr), pl.ds(0, N1), :], sem_xb.at[0])
            for k in range(XG) for j in range(NT)]
    c_f = [cp(w.at[pl.ds(0, HF), :].bitcast(u32).at[:, pl.ds(k1 * N2, N2)], wf.at[i * N1 + k1, pl.ds(0, HF // 2), :],
              sem_f.at[0]) for i, w in enumerate((wr_hbm, wi_hbm)) for k1 in range(N1)]
    c_w = []
    for m, w_hbm in enumerate((wq_hbm, wk_hbm, wv_hbm)):
        for c in range(DP // WPIECE):
            r0 = m * DP + c * WPIECE
            c_w.append(cp(w_hbm.bitcast(u32).at[pl.ds(c * WPIECE, WPIECE)],
                          wraw.at[pl.ds(r0, WPIECE)], sem_w.at[r0 // WPIECE]))
    c_wo = cp(wo_hbm.bitcast(u32), wo, sem_wo.at[0])
    for c in (*c_n, *c_xb):
        c.start()

    def relayout_wait(u):
        view = wraw.at[pl.ds(u * WPIECE, WPIECE)]
        cp(view, view, sem_w.at[u]).wait()

    def relayout(u, part, nparts, zero=None, kv=False, width=1):
        dst, pitch, off = (wkv, KPITCH, DP) if kv else (wq, QPITCH, 0)
        n = width * WPIECE // nparts
        for i in range(n):
            dp = u * WPIECE + part * n + i
            a, b = wraw[dp, 0:G, :], wraw[dp, G:H, :]
            if zero is not None:
                a = a | zero
            lo, hi = _unzip_rows(a, b)
            dst[0, pl.ds(dp - off, G, stride=pitch), :] = lo
            dst[1, pl.ds(dp - off, G, stride=pitch), :] = hi

    def token(v):
        return (pltpu.bitcast(v[0:G, 0:128], u32) >> 16) >> 16

    first = lax.broadcasted_iota(jnp.int32, (8, N2), 0) == 0
    pack = lambda v: pltpu.bitcast(v.astype(bf16), u32)
    pack2 = lambda lo, hi: pltpu.pack_elementwise([lo, hi], packed_dtype=bf16)
    iota = lambda shape, dim: lax.broadcasted_iota(jnp.int32, shape, dim).astype(f32)

    def gen_tt(it, carry):
        r, g4 = it >> 2, it & 3
        f = (r + 5 * ((r ^ (g4 >> 1)) & 1) + 160 * (g4 & 1)).astype(f32) + 10.0 * iota((16, 128), 0)
        c, sn = _cos_sin(f * iota((16, 128), 1), D)
        sg = jnp.where(r >= 3, 1.0, -1.0)
        nyq = jnp.where((lax.broadcasted_iota(jnp.int32, (16, 128), 1) & 1) == 0, 1.0, -1.0)
        is_nyq = lax.broadcasted_iota(jnp.int32, (16, 128), 0) + it == 0
        r0 = pl.multiple_of(8 * g4, 8)
        tt[r, pl.ds(r0, 8), 0:128] = pack(c)
        tt[r, pl.ds(r0, 8), 128:] = pack(sg * sn)
        tt[r, pl.ds(32 + r0, 8), 0:128] = pack(jnp.where(is_nyq, nyq, -sn))
        tt[r, pl.ds(32 + r0, 8), 128:] = pack(sg * c)
        r1 = pl.multiple_of(16 * g4, 16)
        ti[r, pl.ds(r1, 16), 0:128] = pack2(c, jnp.where(is_nyq, nyq, -sn))
        ti[r, pl.ds(r1, 16), 128:] = pack2(sg * sn, sg * c)
        return carry
    lax.fori_loop(0, 20, gen_tt, 0)

    def gen_ts(i, carry):
        n = iota((16, N2), 0) + 16.0 * jnp.maximum(i - 1, 0).astype(f32)
        c, sn = _cos_sin(jnp.where(i == 0, n, float(N1) * n) * iota((16, N2), 1), S)
        rows = pl.ds(pl.multiple_of(16 * i, 16), 16)
        ts[0, rows, :] = c
        ts[1, rows, :] = sn
        return carry
    lax.fori_loop(0, 1 + N2 // 16, gen_ts, 0)
    for c in c_f:
        c.start()

    def gen_gm(s1, carry):
        ca, sa = ts[0, pl.ds(s1, 1), :], ts[1, pl.ds(s1, 1), :]
        cb, sb = ts[0, N1:, :], ts[1, N1:, :]
        gm[s1, :, 0:N2] = pack(ca * cb - sa * sb)
        gm[s1, :, N2:] = pack(-(sa * cb + ca * sb))
        return carry
    lax.fori_loop(0, N1, gen_gm, 0)
    for c in (*c_w[:NQ], c_xp):
        c.start()

    def dft_mats(t):
        return (pltpu.bitcast(t[0, :, 0:128], bf16),
                pltpu.bitcast(jnp.concatenate([t[1], t[4]], axis=0), bf16),
                pltpu.bitcast(jnp.concatenate([t[2], t[3]], axis=0), bf16))

    xb_all = xb3.at[pl.ds(0, NT * N2 // 2), pl.ds(0, N1), :]
    cp(xb_all, xb_all, sem_xb.at[0]).wait()
    for c in (*c_w[NQ:], c_mem, c_xa0):
        c.start()
    c_wo.start(priority=1)
    nt = (((1,), (1,)), ((), ()))

    def p1(q):
        wa, wb = [], []
        for j in range(NT):
            base = j * (N2 // 2) * XPITCH + q
            wa.append(xb[pl.ds(base, N2 // 2, stride=XPITCH), :])
            wb.append(xb[pl.ds(base + N1 // 2, N2 // 2, stride=XPITCH), :])
        us = []
        for sel in (lambda v: v << 16, lambda v: v & u32(HI16)):
            ua = _radix5([pltpu.bitcast(sel(v), f32) for v in wa])
            ub = _radix5([pltpu.bitcast(sel(v), f32) for v in wb])
            us.append([pltpu.bitcast(pltpu.pack_elementwise([x, y], packed_dtype=bf16), bf16)
                       for x, y in zip(ua, ub)])
        u = [jnp.concatenate([us[0][k], us[1][k]], axis=0) for k in range(5)]
        t0, t1, t2 = dft_mats(tt)
        x0 = lax.dot_general(t0, u[0], nt, preferred_element_type=f32)
        x14 = lax.dot_general(t1, jnp.concatenate(u[1:3], axis=1), nt, preferred_element_type=f32)
        x23 = lax.dot_general(t2, jnp.concatenate(u[3:5], axis=1), nt, preferred_element_type=f32)
        return jnp.concatenate([x0, x14[0:128], x23, x14[128:]], axis=0).astype(bf16)

    def p2(q, xdt):
        for par in range(2):
            s1 = 2 * q + par
            t = jnp.dot(xdt[:, par * N2:(par + 1) * N2], pltpu.bitcast(gm[s1], bf16), preferred_element_type=f32)
            t1, t2 = t[:, 0:N2], t[:, N2:]
            vre[s1, 0:8] = t1[0:8] - jnp.where(first, 0.0, t2[64:72])
            vim[s1, 0:8] = jnp.where(first, 0.0, t1[64:72]) + t2[0:8]
            vre[s1, HF:HF + 8] = t1[64:72]
            vim[s1, HF:HF + 8] = t2[64:72]
            for r in range(5):
                m0 = 8 if r == 0 else 0
                re, im = slice(128 * r + m0, 128 * r + 64), slice(128 * r + 64 + m0, 128 * r + 128)
                vre[s1, 64 * r + m0:64 * r + 64] = t1[re] - t2[im]
                vim[s1, 64 * r + m0:64 * r + 64] = t1[im] + t2[re]

    def p12(i, carry):
        xs = [p1(UB * i + k) for k in range(UB)]
        for k in range(UB):
            p2(UB * i + k, xs[k])
        return carry
    lax.fori_loop(0, N1 // 2 // UB, p12, 0)

    wf_all = wf.at[:, pl.ds(0, HF // 2), :]
    cp(wf_all, wf_all, sem_f.at[0]).wait()
    for c in c_n:
        c.wait()

    def filt(rows, wload):
        re = [vre[s1, rows, :] for s1 in range(N1)]
        im = [vim[s1, rows, :] for s1 in range(N1)]
        xr, xi = _fft_list(re, im, -1)
        yr, yi = [], []
        for k1 in range(N1):
            a, b = wload(0, k1), wload(1, k1)
            yr.append(xr[k1] * a - xi[k1] * b)
            yi.append(xr[k1] * b + xi[k1] * a)
        return _fft_list(yr, yi, +1)

    def p3(r, odd, j):
        start = ((r + 5 * ((r ^ odd) & 1)) >> 1) + 40 * j
        sel = (lambda v: v & u32(HI16)) if odd else (lambda v: v << 16)
        rows = pl.ds(pl.multiple_of(64 * r + 32 * odd + 8 * j, 8), 8)
        zr, zi = filt(rows, lambda i, k1: pltpu.bitcast(sel(wf[i * N1 + k1, pl.ds(start, 8, stride=5), :]), f32))
        for s1 in range(N1):
            wt[s1, rows, 0:N2] = pack2(zr[s1], zi[s1])
            wt[s1, rows, N2:] = pack2(zi[s1], -zr[s1])

    def bq(g, k):
        rows = pl.ds(pl.multiple_of(g * QPITCH, 8), DP)
        w = pltpu.bitcast(jnp.concatenate([wq[0, rows, :], wq[1, rows, :]], axis=1), bf16)
        rb = NPAIR * QP // NBQ
        t = jnp.dot(pltpu.bitcast(xpk[k * rb // 2:(k + 1) * rb // 2, :], bf16), w, preferred_element_type=f32)
        qpre[g, k * rb:(k + 1) * rb, :] = t
        return t

    def p3j(j, carry):
        relayout_wait(2 * j)
        relayout_wait(2 * j + 1)

        def p3r(r, carry):
            relayout(2 * j, r, 5, width=2)
            p3(r, 0, j)
            p3(r, 1, j)
            return carry
        return lax.fori_loop(0, 5, p3r, carry)
    lax.fori_loop(0, NQ // 2, p3j, 0)
    c_xp.wait()
    xpk[...] = pltpu.bitcast(xa[:, 0:QP, :].reshape(NPAIR * QP, D), u32)

    nr, ni = filt(slice(HF, HF + 8), lambda i, k1: wn[i, :, k1 * N2:(k1 + 1) * N2].astype(f32))
    first2 = lax.broadcasted_iota(jnp.int32, (8, 2 * N2), 0) == 0
    for s1 in range(N1):
        z = wt[s1, 0:8, :]
        fixed = pack2(0.5 * pltpu.bitcast(z << 16, f32), 0.5 * jnp.concatenate([nr[s1], ni[s1]], axis=1))
        wt[s1, 0:8, :] = jnp.where(first2, fixed, z)

    def p45q(i, carry):
        for k in range(2 * UF):
            relayout_wait(NQ + 2 * UF * i + k)
        state = [0, None]

        def rl(v):
            k, zero = state
            if k < 2 * UF * RLP:
                relayout(NQ + 2 * UF * i + k // RLP, k % RLP, RLP, zero, True)
            state[0], state[1] = k + 1, token(v)

        hb = N2 // RB
        for kf in range(UF):
            q = UF * i + kf
            for k in range(B0):
                rl(bq(2 * q, k))
            for par in range(2):
                s1 = 2 * q + par
                t = lax.dot_general(pltpu.bitcast(gm[s1], bf16), pltpu.bitcast(wt[s1], bf16), nt,
                                    preferred_element_type=f32)
                rsc[2 * kf + par] = pltpu.bitcast(t.astype(bf16), u32)
                rl(t)
            for k in range(B0, NBQ):
                rl(bq(2 * q, k))
            t0, t1, t2 = dft_mats(ti)
            for rb in range(RB):
                rows = slice(rb * hb // 2, (rb + 1) * hb // 2)
                rc = pltpu.bitcast(jnp.concatenate([rsc[2 * kf, rows], rsc[2 * kf + 1, rows]], axis=0), bf16)
                z0 = jnp.dot(rc[:, 0:128], t0, preferred_element_type=f32)
                z1 = jnp.dot(jnp.concatenate([rc[:, 128:256], rc[:, 512:640]], axis=1), t1,
                             preferred_element_type=f32)
                z2 = jnp.dot(rc[:, 256:512], t2, preferred_element_type=f32)
                ys = _radix5_t(z0, z1[:, 0:128], z1[:, 128:], z2[:, 0:128], z2[:, 128:], 2.0 / (D * S))
                for j in range(NT):
                    ob32[j, pl.ds(q + rb * hb * (N1 // 2), hb, stride=N1 // 2), :] = pack2(ys[j][0:hb], ys[j][hb:])
                rl(z0)
            for k in range(NBQ):
                rl(bq(2 * q + 1, k))
        assert state[0] >= 2 * UF * RLP
        return carry
    lax.fori_loop(0, N1 // 2 // UF, p45q, 0)

    c_mem.wait()
    c_xa0.wait()

    r = lax.broadcasted_iota(jnp.int32, (2 * L, 2 * L), 0)
    c = lax.broadcasted_iota(jnp.int32, (2 * L, 2 * L), 1)
    rb = r >= L
    cb = c >= L
    rr = jnp.where(rb, r - L, r)
    cc = jnp.where(cb, c - L, c)
    mask = (rb == cb) & ((rr < M) | (rr >= cc))
    scale = E ** -0.5

    def wcol(g, c):
        if c < 2:
            return wq[c, g * QPITCH:g * QPITCH + DP, :]
        r0 = g * KPITCH + (c // 2 - 1) * DP
        return wkv[c % 2, r0:r0 + DP, :]

    def filler(p, i0, i1):
        xn = xa[p, 0:32, :]
        if i0 == i1:
            return
        w = jnp.concatenate([wcol(g, c) for g, c in FG[i0:i1]], axis=1)
        t = jnp.dot(xn, pltpu.bitcast(w, bf16), preferred_element_type=f32)
        for i in range(i0, i1):
            fstash[i] = t[:, (i - i0) * E:(i - i0 + 1) * E]

    def step(lhs, even, p):
        nrow_o = 32 if even else 48
        qkv, ps, acc = {}, {}, [None]

        def proj(g):
            def mm(rows, cols):
                w = jnp.concatenate([wcol(g, c) for c in cols], axis=1)
                return jnp.dot(rows, pltpu.bitcast(w, bf16), preferred_element_type=f32)

            if not even:
                t = mm(lhs, range(6))
            else:
                tq = jnp.concatenate([qpre[g, pl.ds(pl.multiple_of(p * QP, QP), QP), :], mm(lhs[QP:], (0, 1))], axis=0)
                moved = [c for gg, c in FG if gg == g]
                if not moved:
                    t = jnp.concatenate([tq, mm(lhs, range(2, 6))], axis=1)
                else:
                    rest = [c for c in range(2, 6) if c not in moved]
                    order = [c for pr in zip(rest, moved + [None] * 4) for c in pr if c is not None]
                    tc = {}
                    for c in order:
                        if c in moved:
                            tc[c] = jnp.concatenate([fstash[FG.index((g, c))], mm(lhs[32:48], (c,))], axis=0)
                        else:
                            tc[c] = mm(lhs, (c,))
                    t = jnp.concatenate([tq] + [tc[c] for c in range(2, 6)], axis=1)
            col = lambda a, i: a[:, i * E:(i + 1) * E]
            if even:
                stash[g] = t[40:48]
                parts = [jnp.concatenate([col(t, 2 * i)[32:40], col(t, 2 * i)[0:32],
                                          col(t, 2 * i + 1)[32:40], col(t, 2 * i + 1)[0:32]], axis=0)
                         for i in range(3)]
            else:
                st = stash[g]
                parts = [jnp.concatenate(
                    [col(t, 2 * i)[16:24], col(st, 2 * i), col(t, 2 * i)[24:32], col(t, 2 * i)[0:16],
                     col(t, 2 * i + 1)[16:24], col(st, 2 * i + 1), col(t, 2 * i + 1)[24:32],
                     col(t, 2 * i + 1)[0:16]], axis=0)
                    for i in range(3)]
            qkv[g] = ((parts[0] * scale).astype(bf16), parts[1].astype(bf16), parts[2].astype(bf16))

        def scores(g):
            q2, k2, _ = qkv[g]
            s = lax.dot_general(q2, k2, (((1,), (1,)), ((), ())), preferred_element_type=f32)
            s = jnp.where(mask, s, -1e9)
            e = jnp.exp(s - jnp.max(s, axis=-1, keepdims=True))
            l = jnp.sum(e, axis=-1, keepdims=True)
            ps[g] = (e * pl.reciprocal(l, approx=True)).astype(bf16)

        def pv(g):
            o2 = jnp.dot(ps[g], qkv[g][2], preferred_element_type=f32)
            o_scr[0:40, (2 * g) * E:(2 * g + 1) * E] = o2[0:40]
            o_scr[0:40, (2 * g + 1) * E:(2 * g + 2) * E] = o2[40:80]

        def wo_chunk(c):
            a, b = CH[c] * 2 * E, CH[c + 1] * 2 * E
            w = wo[a // 2:b // 2, :]
            t = jnp.dot(o_scr[0:nrow_o, a:b].astype(bf16), pltpu.bitcast(w, bf16), preferred_element_type=f32)
            acc[0] = t if acc[0] is None else acc[0] + t

        ch = 0
        for t in range(G + LAG2):
            if t < G:
                proj(t)
            else:
                assert CH[ch + 1] <= t - LAG2
                wo_chunk(ch)
                ch += 1
            if 0 <= t - LAG1 < G:
                scores(t - LAG1)
            if 0 <= t - LAG2 < G:
                pv(t - LAG2)
        while ch < len(CH) - 1:
            wo_chunk(ch)
            ch += 1
        return acc[0]

    def out_copy(p):
        rows = pl.ds(pl.multiple_of(p * 64, 64), 64)
        return cp(obuf.at[rows, :], out_hbm.at[rows, pl.ds(0, D)], sem_out.at[0])

    def pair(p, mem_v):
        base = pl.multiple_of(p * 64, 64)
        xs = xa[p].astype(f32)
        lhs = jnp.concatenate([xs[0:32], mem_v, xs[32:40]], axis=0).astype(bf16)
        out_e = step(lhs, True, p)
        o_scr[40:48, :] = o_scr[32:40, :]
        pn = jnp.minimum(p + 1, NPAIR - 1)
        filler(pn, 0, NF1)
        lhs = jnp.concatenate([xs[48:64], out_e[0:8], xs[40:48]], axis=0).astype(bf16)
        out_o = step(lhs, False, p)
        filler(pn, NF1, len(FG))
        res = jnp.concatenate([out_e[8:32], out_o[40:48], out_o[8:40]], axis=0)
        obuf[pl.ds(base, 64), :] = res.astype(bf16)
        return out_o[0:8]

    def body(p, mem_v):
        @pl.when(p == 1)
        def _():
            c_xa1.wait()

        @pl.when(p > 0)
        def _():
            out_copy(p * UA - 1).start()
        for k in range(UA):
            if k > 0:
                out_copy(p * UA + k - 1).start()
            mem_v = pair(p * UA + k, mem_v)
        return mem_v

    filler(0, 0, len(FG))
    cp(wo, wo, sem_wo.at[0]).wait()
    c_xa1.start(priority=1)
    c_ob = [cp(ob32.bitcast(bf16).at[j, pl.ds(0, S), :], out_hbm.at[:, pl.ds(D + j * 128, 128)], sem_ob.at[j])
            for j in range(NT)]
    for c in c_ob:
        c.start(priority=1)
    lax.fori_loop(0, NPAIR // UA, body, mem[...].astype(f32))

    out_copy(NPAIR - 1).start()
    for c in c_ob:
        c.wait()
    cp(obuf, obuf, sem_out.at[0]).wait()


@jax.jit
def pallas_concat_heads__memory_aug_recurrent_mem_tr__spectral_gfnet__prompt_kernel(
    A_x: jax.Array,
    A_mem0: jax.Array,
    A_Wq: jax.Array,
    A_Wk: jax.Array,
    A_Wv: jax.Array,
    A_Wo: jax.Array,
    A_seg_len,
    B_x: jax.Array,
    B_w_r: jax.Array,
    B_w_i: jax.Array,
):
    del A_seg_len
    assert A_x.shape == (1, S, D) and B_x.shape == (1, S, D)
    args = (
        A_x.reshape(NPAIR, 64, D), A_mem0.reshape(M, D),
        A_Wq.reshape(DP, 2 * H, E), A_Wk.reshape(DP, 2 * H, E), A_Wv.reshape(DP, 2 * H, E),
        A_Wo.reshape(H * E, D),
        B_x.reshape(N2 // 2, 2 * N1, D), B_w_r.T, B_w_i.T,
    )
    V = pltpu.VMEM
    scratch = [
        V((NPAIR, 64, D), bf16), V((M, D), bf16), V((3 * DP, H, E), u32), V((H * E // 2, D), u32),
        V(((NT * (N2 // 2) + 1) * XPITCH, 128), u32), V((2 * N1, HF // 2 + 8, N2), u32), V((2, 1, S), bf16),
        V((2, N1 + N2, N2), f32), V((5, 64, 256), u32), V((5, 64, 256), u32), V((N1, N2 // 2, 2 * N2), u32),
        V((2, (G + 1) * QPITCH, E), u32), V((2, (G + 1) * KPITCH, E), u32),
        V((N1, HF + 8, N2), f32), V((N1, HF + 8, N2), f32), V((N1, HF, 2 * N2), u32),
        V((2 * UF, N2 // 2, D), u32), V((NT, S // 2 + 8, 128), u32), V((NPAIR * QP // 2, D), u32),
        V((G, NPAIR * QP, 2 * E), f32),
        V((S, D), bf16), V((48, H * E), f32), V((G, 8, 6 * E), f32), V((len(FG), 32, E), f32),
        pltpu.SemaphoreType.DMA((6,)), pltpu.SemaphoreType.DMA((NT,)), pltpu.SemaphoreType.DMA((1,)),
        pltpu.SemaphoreType.DMA((NPIECE,)),
        pltpu.SemaphoreType.DMA((1,)), pltpu.SemaphoreType.DMA((1,)), pltpu.SemaphoreType.DMA((NT,)),
    ]
    out = pl.pallas_call(
        _kernel,
        out_shape=jax.ShapeDtypeStruct((S, 2 * D), bf16),
        in_specs=[pl.BlockSpec(memory_space=pltpu.HBM)] * len(args),
        out_specs=pl.BlockSpec(memory_space=pl.ANY),
        scratch_shapes=scratch,
        compiler_params=pltpu.CompilerParams(vmem_limit_bytes=110 * 1024 * 1024, disable_bounds_checks=True),
    )(*args)
    return out.reshape(1, S, 2 * D)
```

```python
import numpy as np
import jax
import jax.numpy as jnp
from jax import lax
import jax.experimental.pallas as pl
import jax.experimental.pallas.tpu as pltpu

bf16 = jnp.bfloat16
f32 = jnp.float32
u32 = jnp.uint32

S, D = 2048, 640
H, E = 32, 128
M, SEG = 8, 32
L = M + SEG
G = H // 2
DF = D // 2 + 1
HF = D // 2
NT = D // 128
N1, N2 = 16, 128
NPAIR = S // (2 * SEG)
LAG1, LAG2 = 2, 5
CH = (0, 3, 6, 9, 11, 13, 14, 15, 16)
DP = D // 2
WPIECE = 40
NPIECE = 3 * DP // WPIECE
NQ = DP // WPIECE
QPITCH = DP + 8
KPITCH = 2 * DP + 8
UB = 2
RB = 4
FG = [(4, 4), (8, 4), (12, 4), (14, 4)]
NF1 = 2
NBQ = 8
RLP = 10
XG = 8
B0 = 2
U3 = 2
RPITCH = N2 + 8
UA = 4
QP = 16
C5 = (float(np.cos(2 * np.pi / 5)), float(np.cos(4 * np.pi / 5)))
S5 = (float(np.sin(2 * np.pi / 5)), float(np.sin(4 * np.pi / 5)))
HI16 = 0xFFFF0000


def _cos_sin(num, den):
    r = num - den * jnp.floor((num + 0.5) * (1.0 / den))
    ang = r * (2.0 * np.pi / den)
    return jnp.cos(ang), jnp.sin(ang)


def _fft_list(re, im, sign):
    n = len(re)
    if n == 1:
        return re, im
    er, ei = _fft_list(re[0::2], im[0::2], sign)
    orr, oi = _fft_list(re[1::2], im[1::2], sign)
    h = n // 2
    outr = [None] * n
    outi = [None] * n
    r = np.float32(np.sqrt(0.5))
    for k in range(h):
        a, b = orr[k], oi[k]
        if 4 * k == n:
            if sign > 0:
                outr[k], outi[k] = er[k] - b, ei[k] + a
                outr[k + h], outi[k + h] = er[k] + b, ei[k] - a
            else:
                outr[k], outi[k] = er[k] + b, ei[k] - a
                outr[k + h], outi[k + h] = er[k] - b, ei[k] + a
            continue
        if k == 0:
            tr, ti = a, b
        elif 8 * k == n:
            tr, ti = ((a - b) * r, (a + b) * r) if sign > 0 else ((a + b) * r, (b - a) * r)
        elif 8 * k == 3 * n:
            tr, ti = ((a + b) * (-r), (a - b) * r) if sign > 0 else ((b - a) * r, (a + b) * (-r))
        else:
            c = np.float32(np.cos(2 * np.pi * k / n))
            s = np.float32(sign * np.sin(2 * np.pi * k / n))
            tr, ti = a * c - b * s, a * s + b * c
        outr[k], outi[k] = er[k] + tr, ei[k] + ti
        outr[k + h], outi[k + h] = er[k] - tr, ei[k] - ti
    return outr, outi


def _unzip_rows(a, b):
    lo = (a & u32(0xFFFF)) | (b << 16)
    hi = (a >> 16) | (b & u32(HI16))
    return lo, hi


def _radix5(x):
    t1, t2, t3, t4 = x[1] + x[4], x[2] + x[3], x[1] - x[4], x[2] - x[3]
    return (x[0] + t1 + t2,
            x[0] + C5[0] * t1 + C5[1] * t2, S5[0] * t3 + S5[1] * t4,
            x[0] + C5[1] * t1 + C5[0] * t2, S5[1] * t3 - S5[0] * t4)


def _radix5_t(z0, zc1, zs1, zc2, zs2, k):
    z0 = z0 * k
    p1 = z0 + (k * C5[0]) * zc1 + (k * C5[1]) * zc2
    p2 = z0 + (k * C5[1]) * zc1 + (k * C5[0]) * zc2
    q1 = (k * S5[0]) * zs1 + (k * S5[1]) * zs2
    q2 = (k * S5[1]) * zs1 - (k * S5[0]) * zs2
    return z0 + (zc1 + zc2) * k, p1 + q1, p2 + q2, p2 - q2, p1 - q1


def _kernel(xa_hbm, mem_hbm, wq_hbm, wk_hbm, wv_hbm, wo_hbm, xb_hbm, wr_hbm, wi_hbm,
            out_hbm,
            xa, mem, wraw, wo, xbr, xb, wr, wi, ts, tt, gm,
            wq, wkv, vre, vim, rsc, xpk, qpre, obuf, o_scr, stash, fstash,
            sem_in, sem_xb, sem_w, sem_out):
    def cp(src, dst, sem):
        return pltpu.make_async_copy(src, dst, sem)

    def xa_copy(p0, n, r0, nr, sem):
        return cp(xa_hbm.at[pl.ds(p0, n), pl.ds(r0, nr), :], xa.at[pl.ds(p0, n), pl.ds(r0, nr), :], sem)

    c_mem = cp(mem_hbm, mem, sem_in.at[0])
    c_xp = xa_copy(0, NPAIR, 0, QP, sem_in.at[1])
    c_xa0 = xa_copy(0, UA + 1, QP, 64 - QP, sem_in.at[2])
    c_xa1 = xa_copy(UA + 1, NPAIR - UA - 1, QP, 64 - QP, sem_in.at[3])
    c_f = [cp(wr_hbm, wr, sem_in.at[4]), cp(wi_hbm, wi, sem_in.at[5])]
    c_wo = cp(wo_hbm, wo, sem_in.at[6])
    xr = S // XG
    c_xb = [cp(xb_hbm.at[pl.ds(k * xr, xr), :], xbr.at[pl.ds(k * xr, xr), :], sem_xb.at[k]) for k in range(XG)]
    c_w = []
    for m, w_hbm in enumerate((wq_hbm, wk_hbm, wv_hbm)):
        for c in range(NQ):
            c_w.append(cp(w_hbm.at[pl.ds(c * WPIECE, WPIECE)], wraw.at[pl.ds(m * DP + c * WPIECE, WPIECE)],
                          sem_w.at[m * NQ + c]))
    for c in c_xb:
        c.start()

    def relayout_wait(u):
        view = wraw.at[pl.ds(u * WPIECE, WPIECE)]
        cp(view, view, sem_w.at[u]).wait()

    def relayout(u, part, nparts, zero=None, kv=False):
        dst, pitch, off = (wkv, KPITCH, DP) if kv else (wq, QPITCH, 0)
        n = WPIECE // nparts
        for i in range(n):
            dp = u * WPIECE + part * n + i
            ab = pltpu.bitcast(wraw[dp], u32)
            a, b = ab[0:G], ab[G:]
            if zero is not None:
                a = a | zero
            lo, hi = _unzip_rows(a, b)
            dst[0, pl.ds(dp - off, G, stride=pitch), :] = lo
            dst[1, pl.ds(dp - off, G, stride=pitch), :] = hi

    def token(v):
        return (pltpu.bitcast(v[0:G, 0:128], u32) >> 16) >> 16

    def xb_words(k):
        c_xb[k].wait()
        w = pltpu.bitcast(xbr[k * xr:(k + 1) * xr, :], u32)
        for j in range(NT):
            xb[j, k * xr // 2:(k + 1) * xr // 2, :] = w[:, j * 128:(j + 1) * 128]

    first = lax.broadcasted_iota(jnp.int32, (8, N2), 0) == 0
    pack = lambda v: pltpu.bitcast(v.astype(bf16), u32)
    iota = lambda shape, dim: lax.broadcasted_iota(jnp.int32, shape, dim).astype(f32)

    def gen_tt(it, carry):
        r, g4 = it >> 2, it & 3
        f = (r + 80 * g4).astype(f32) + 5.0 * iota((16, 128), 0)
        c, sn = _cos_sin(f * iota((16, 128), 1), D)
        sg = jnp.where(r >= 3, 1.0, -1.0)
        nyq = jnp.where((lax.broadcasted_iota(jnp.int32, (16, 128), 1) & 1) == 0, 1.0, -1.0)
        is_nyq = lax.broadcasted_iota(jnp.int32, (16, 128), 0) + it == 0
        r0 = pl.multiple_of(8 * g4, 8)
        tt[r, pl.ds(r0, 8), 0:128] = pack(c)
        tt[r, pl.ds(r0, 8), 128:] = pack(sg * sn)
        tt[r, pl.ds(32 + r0, 8), 0:128] = pack(jnp.where(is_nyq, nyq, -sn))
        tt[r, pl.ds(32 + r0, 8), 128:] = pack(sg * c)
        return carry
    lax.fori_loop(0, 20, gen_tt, 0)
    for c in c_f:
        c.start()

    def gen_ts(i, carry):
        n = iota((16, N2), 0) + 16.0 * jnp.maximum(i - 1, 0).astype(f32)
        c, sn = _cos_sin(jnp.where(i == 0, n, float(N1) * n) * iota((16, N2), 1), S)
        rows = pl.ds(pl.multiple_of(16 * i, 16), 16)
        ts[0, rows, :] = c
        ts[1, rows, :] = sn
        return carry
    lax.fori_loop(0, 1 + N2 // 16, gen_ts, 0)
    for c in (*c_w[:NQ], c_xp):
        c.start()
    for k in range(XG // 2):
        xb_words(k)

    def gen_gm(s1, carry):
        ca, sa = ts[0, pl.ds(s1, 1), :], ts[1, pl.ds(s1, 1), :]
        cb, sb = ts[0, N1:, :], ts[1, N1:, :]
        gm[s1, :, 0:N2] = pack(ca * cb - sa * sb)
        gm[s1, :, N2:] = pack(-(sa * cb + ca * sb))
        return carry
    lax.fori_loop(0, N1, gen_gm, 0)
    for c in (*c_w[NQ:], c_mem, c_xa0):
        c.start()
    c_wo.start(priority=1)
    for k in range(XG // 2, XG):
        xb_words(k)

    def dft_mats():
        return (pltpu.bitcast(tt[0, :, 0:128], bf16),
                pltpu.bitcast(jnp.concatenate([tt[1], tt[4]], axis=0), bf16),
                pltpu.bitcast(jnp.concatenate([tt[2], tt[3]], axis=0), bf16))

    nt = (((1,), (1,)), ((), ()))

    def p1(q):
        xw = [xb[j, pl.ds(q, N2, stride=N1 // 2), :] for j in range(NT)]
        us = [_radix5([pltpu.bitcast(sel(v), f32) for v in xw])
              for sel in (lambda v: v << 16, lambda v: v & u32(HI16))]
        u = [jnp.concatenate([us[0][k], us[1][k]], axis=0) for k in range(5)]
        t0, t1, t2 = dft_mats()
        x0 = lax.dot_general(t0, u[0].astype(bf16), nt, preferred_element_type=f32)
        x14 = lax.dot_general(t1, jnp.concatenate(u[1:3], axis=1).astype(bf16), nt, preferred_element_type=f32)
        x23 = lax.dot_general(t2, jnp.concatenate(u[3:5], axis=1).astype(bf16), nt, preferred_element_type=f32)
        return jnp.concatenate([x0, x14[0:128], x23, x14[128:]], axis=0)

    def bins(r, m0=0):
        return pl.ds(r + 5 * m0, 64 - m0, stride=5)

    def p2(q, xdt):
        for par in range(2):
            s1 = 2 * q + par
            t = jnp.dot(xdt[:, par * N2:(par + 1) * N2].astype(bf16), pltpu.bitcast(gm[s1], bf16),
                        preferred_element_type=f32)
            t1, t2 = t[:, 0:N2], t[:, N2:]
            vre[s1, pl.ds(0, 8, stride=5), :] = t1[0:8] - jnp.where(first, 0.0, t2[64:72])
            vim[s1, pl.ds(0, 8, stride=5), :] = jnp.where(first, 0.0, t1[64:72]) + t2[0:8]
            vre[s1, HF:HF + 8] = t1[64:72]
            vim[s1, HF:HF + 8] = t2[64:72]
            for r in range(5):
                m0 = 8 if r == 0 else 0
                re, im = slice(128 * r + m0, 128 * r + 64), slice(128 * r + 64 + m0, 128 * r + 128)
                vre[s1, bins(r, m0), :] = t1[re] - t2[im]
                vim[s1, bins(r, m0), :] = t1[im] + t2[re]

    def p12(i, carry):
        xs = [p1(UB * i + k) for k in range(UB)]
        for k in range(UB):
            p2(UB * i + k, xs[k])
        return carry
    lax.fori_loop(0, N1 // 2 // UB, p12, 0)

    for c in c_f:
        c.wait()

    def p3(rows, wrows):
        re = [vre[s1, rows, :] for s1 in range(N1)]
        im = [vim[s1, rows, :] for s1 in range(N1)]
        xr, xi = _fft_list(re, im, -1)
        yr, yi = [], []
        for k1 in range(N1):
            a = wr[wrows, k1 * N2:(k1 + 1) * N2].astype(f32)
            b = wi[wrows, k1 * N2:(k1 + 1) * N2].astype(f32)
            yr.append(xr[k1] * a - xi[k1] * b)
            yi.append(xr[k1] * b + xi[k1] * a)
        zr, zi = _fft_list(yr, yi, +1)
        for s1 in range(N1):
            vre[s1, rows, :] = zr[s1]
            vim[s1, rows, :] = zi[s1]

    def p3l(i, carry):
        for k in range(U3):
            rows = pl.ds(pl.multiple_of(8 * (U3 * i + k), 8), 8)
            p3(rows, rows)
        return carry
    lax.fori_loop(0, HF // 8 // U3, p3l, 0)
    p3(slice(HF, HF + 8), slice(HF, HF + 1))

    def p4(s1, r):
        zr, zi = vre[s1, bins(r), :], vim[s1, bins(r), :]
        top, bot = jnp.concatenate([zr, zi], axis=1), jnp.concatenate([zi, -zr], axis=1)
        if r == 0:
            f2 = jnp.concatenate([first, first], axis=1)
            nyq = jnp.concatenate([vre[s1, HF:HF + 8, :], vim[s1, HF:HF + 8, :]], axis=1)
            top = jnp.concatenate([jnp.where(f2, 0.5 * top[0:8], top[0:8]), top[8:]], axis=0)
            bot = jnp.concatenate([jnp.where(f2, 0.5 * nyq, bot[0:8]), bot[8:]], axis=0)
        t = lax.dot_general(pltpu.bitcast(gm[s1], bf16), jnp.concatenate([top, bot], axis=0).astype(bf16), nt,
                            preferred_element_type=f32)
        rsc[r, pl.ds(pl.multiple_of(s1 * RPITCH, 8), N2), :] = t
        return t

    def bq(g, k):
        rows = pl.ds(pl.multiple_of(g * QPITCH, 8), DP)
        w = pltpu.bitcast(jnp.concatenate([wq[0, rows, :], wq[1, rows, :]], axis=1), bf16)
        rb = NPAIR * QP // NBQ
        t = jnp.dot(pltpu.bitcast(xpk[k * rb // 2:(k + 1) * rb // 2, :], bf16), w, preferred_element_type=f32)
        qpre[g, k * rb:(k + 1) * rb, :] = t
        return t

    def pacer(u0, kv):
        relayout_wait(u0)
        relayout_wait(u0 + 1)
        state = [0, None]

        def rl(v):
            k, zero = state
            relayout(u0 + k // RLP, k % RLP, RLP, zero, kv)
            state[0], state[1] = k + 1, token(v)
        return rl

    def p4l(i, carry):
        rl = pacer(2 * i, False)
        for k in range(4):
            for r in range(5):
                rl(p4(4 * i + k, r))
        return carry
    lax.fori_loop(0, N1 // 4, p4l, 0)
    c_xp.wait()
    xpk[...] = pltpu.bitcast(xa[:, 0:QP, :].reshape(NPAIR * QP, D), u32)

    def p5q(q, carry):
        rl = pacer(NQ + 2 * q, True)
        t0, t1, t2 = dft_mats()
        ns = N1 // RB

        def p5(rb):
            rc = [jnp.concatenate([rsc[j, pl.ds(N1 * q + ns * rb + k, N1, stride=RPITCH), :] for k in range(ns)],
                                  axis=0) for j in range(NT)]
            z0 = jnp.dot(rc[0].astype(bf16), t0, preferred_element_type=f32)
            z1 = jnp.dot(jnp.concatenate([rc[1], rc[4]], axis=1).astype(bf16), t1, preferred_element_type=f32)
            z2 = jnp.dot(jnp.concatenate([rc[2], rc[3]], axis=1).astype(bf16), t2, preferred_element_type=f32)
            ys = _radix5_t(z0, z1[:, 0:128], z1[:, 128:], z2[:, 0:128], z2[:, 128:], 2.0 / (D * S))
            rows = pl.ds(pl.multiple_of(N1 * (N1 * q + ns * rb), N1 * ns), N1 * ns)
            obuf[rows, D:] = jnp.concatenate(ys, axis=1).astype(bf16)
            return z0

        nb = 2 * NBQ // RB
        for rb in range(RB):
            for k in range(rb * nb, (rb + 1) * nb):
                rl(bq(2 * q + k // NBQ, k % NBQ))
                if k == rb * nb + B0 - 1:
                    rl(p5(rb))
        return carry
    lax.fori_loop(0, N1 // 2, p5q, 0)

    c_mem.wait()
    c_xa0.wait()

    r = lax.broadcasted_iota(jnp.int32, (2 * L, 2 * L), 0)
    c = lax.broadcasted_iota(jnp.int32, (2 * L, 2 * L), 1)
    rb = r >= L
    cb = c >= L
    rr = jnp.where(rb, r - L, r)
    cc = jnp.where(cb, c - L, c)
    mask = (rb == cb) & ((rr < M) | (rr >= cc))
    scale = E ** -0.5

    def wcol(g, c):
        if c < 2:
            return wq[c, g * QPITCH:g * QPITCH + DP, :]
        r0 = g * KPITCH + (c // 2 - 1) * DP
        return wkv[c % 2, r0:r0 + DP, :]

    def filler(p, i0, i1):
        xn = xa[p, 0:32, :]
        if i0 == i1:
            return
        w = jnp.concatenate([wcol(g, c) for g, c in FG[i0:i1]], axis=1)
        t = jnp.dot(xn, pltpu.bitcast(w, bf16), preferred_element_type=f32)
        for i in range(i0, i1):
            fstash[i] = t[:, (i - i0) * E:(i - i0 + 1) * E]

    def step(lhs, even, p):
        nrow_o = 32 if even else 48
        qkv, ps, acc = {}, {}, [None]

        def proj(g):
            def mm(rows, cols):
                w = jnp.concatenate([wcol(g, c) for c in cols], axis=1)
                return jnp.dot(rows, pltpu.bitcast(w, bf16), preferred_element_type=f32)

            if not even:
                t = mm(lhs, range(6))
            else:
                tq = jnp.concatenate([qpre[g, pl.ds(pl.multiple_of(p * QP, QP), QP), :], mm(lhs[QP:], (0, 1))], axis=0)
                moved = [c for gg, c in FG if gg == g]
                if not moved:
                    t = jnp.concatenate([tq, mm(lhs, range(2, 6))], axis=1)
                else:
                    rest = [c for c in range(2, 6) if c not in moved]
                    order = [c for pr in zip(rest, moved + [None] * 4) for c in pr if c is not None]
                    tc = {}
                    for c in order:
                        if c in moved:
                            tc[c] = jnp.concatenate([fstash[FG.index((g, c))], mm(lhs[32:48], (c,))], axis=0)
                        else:
                            tc[c] = mm(lhs, (c,))
                    t = jnp.concatenate([tq] + [tc[c] for c in range(2, 6)], axis=1)
            col = lambda a, i: a[:, i * E:(i + 1) * E]
            if even:
                stash[g] = t[40:48]
                parts = [jnp.concatenate([col(t, 2 * i)[32:40], col(t, 2 * i)[0:32],
                                          col(t, 2 * i + 1)[32:40], col(t, 2 * i + 1)[0:32]], axis=0)
                         for i in range(3)]
            else:
                st = stash[g]
                parts = [jnp.concatenate(
                    [col(t, 2 * i)[16:24], col(st, 2 * i), col(t, 2 * i)[24:32], col(t, 2 * i)[0:16],
                     col(t, 2 * i + 1)[16:24], col(st, 2 * i + 1), col(t, 2 * i + 1)[24:32],
                     col(t, 2 * i + 1)[0:16]], axis=0)
                    for i in range(3)]
            qkv[g] = ((parts[0] * scale).astype(bf16), parts[1].astype(bf16), parts[2].astype(bf16))

        def scores(g):
            q2, k2, _ = qkv[g]
            s = lax.dot_general(q2, k2, (((1,), (1,)), ((), ())), preferred_element_type=f32)
            s = jnp.where(mask, s, -1e9)
            e = jnp.exp(s - jnp.max(s, axis=-1, keepdims=True))
            l = jnp.sum(e, axis=-1, keepdims=True)
            ps[g] = (e * pl.reciprocal(l, approx=True)).astype(bf16)

        def pv(g):
            o2 = jnp.dot(ps[g], qkv[g][2], preferred_element_type=f32)
            o_scr[0:40, (2 * g) * E:(2 * g + 1) * E] = o2[0:40]
            o_scr[0:40, (2 * g + 1) * E:(2 * g + 2) * E] = o2[40:80]

        def wo_chunk(c):
            a, b = CH[c] * 2 * E, CH[c + 1] * 2 * E
            t = jnp.dot(o_scr[0:nrow_o, a:b].astype(bf16), wo[a:b, :], preferred_element_type=f32)
            acc[0] = t if acc[0] is None else acc[0] + t

        ch = 0
        for t in range(G + LAG2):
            if t < G:
                proj(t)
            else:
                assert CH[ch + 1] <= t - LAG2
                wo_chunk(ch)
                ch += 1
            if 0 <= t - LAG1 < G:
                scores(t - LAG1)
            if 0 <= t - LAG2 < G:
                pv(t - LAG2)
        while ch < len(CH) - 1:
            wo_chunk(ch)
            ch += 1
        return acc[0]

    def out_copy(p):
        rows = pl.ds(pl.multiple_of(p * 64, 64), 64)
        return cp(obuf.at[rows, :], out_hbm.at[rows, :], sem_out.at[0])

    def pair(p, mem_v):
        base = pl.multiple_of(p * 64, 64)
        xs = xa[p].astype(f32)
        lhs = jnp.concatenate([xs[0:32], mem_v, xs[32:40]], axis=0).astype(bf16)
        out_e = step(lhs, True, p)
        o_scr[40:48, :] = o_scr[32:40, :]
        pn = jnp.minimum(p + 1, NPAIR - 1)
        filler(pn, 0, NF1)
        lhs = jnp.concatenate([xs[48:64], out_e[0:8], xs[40:48]], axis=0).astype(bf16)
        out_o = step(lhs, False, p)
        filler(pn, NF1, len(FG))
        res = jnp.concatenate([out_e[8:32], out_o[40:48], out_o[8:40]], axis=0)
        obuf[pl.ds(base, 64), 0:D] = res.astype(bf16)
        return out_o[0:8]

    def body(p, mem_v):
        @pl.when(p == 1)
        def _():
            c_xa1.wait()

        @pl.when(p > 0)
        def _():
            out_copy(p * UA - 1).start()
        for k in range(UA):
            if k > 0:
                out_copy(p * UA + k - 1).start()
            mem_v = pair(p * UA + k, mem_v)
        return mem_v

    filler(0, 0, len(FG))
    c_wo.wait()
    c_xa1.start(priority=1)
    lax.fori_loop(0, NPAIR // UA, body, mem[...].astype(f32))

    out_copy(NPAIR - 1).start()
    cp(obuf, obuf, sem_out.at[0]).wait()


@jax.jit
def pallas_concat_heads__memory_aug_recurrent_mem_tr__spectral_gfnet__prompt_kernel(
    A_x: jax.Array,
    A_mem0: jax.Array,
    A_Wq: jax.Array,
    A_Wk: jax.Array,
    A_Wv: jax.Array,
    A_Wo: jax.Array,
    A_seg_len,
    B_x: jax.Array,
    B_w_r: jax.Array,
    B_w_i: jax.Array,
):
    del A_seg_len
    assert A_x.shape == (1, S, D) and B_x.shape == (1, S, D)
    args = (
        A_x.reshape(NPAIR, 64, D), A_mem0.reshape(M, D),
        A_Wq.reshape(DP, 2 * H, E), A_Wk.reshape(DP, 2 * H, E), A_Wv.reshape(DP, 2 * H, E),
        A_Wo.reshape(H * E, D),
        B_x.reshape(S, D), B_w_r.T, B_w_i.T,
    )
    V = pltpu.VMEM
    scratch = [
        V((NPAIR, 64, D), bf16), V((M, D), bf16), V((3 * DP, 2 * H, E), bf16), V((H * E, D), bf16),
        V((S, D), bf16), V((NT, S // 2 + 8, 128), u32), V((DF, S), bf16), V((DF, S), bf16),
        V((2, N1 + N2, N2), f32), V((5, 64, 256), u32), V((N1, N2 // 2, 2 * N2), u32),
        V((2, (G + 1) * QPITCH, E), u32), V((2, (G + 1) * KPITCH, E), u32),
        V((N1, HF + 8, N2), f32), V((N1, HF + 8, N2), f32),
        V((NT, (N1 + 1) * RPITCH, 128), f32), V((NPAIR * QP // 2, D), u32), V((G, NPAIR * QP, 2 * E), f32),
        V((S, 2 * D), bf16), V((48, H * E), f32), V((G, 8, 6 * E), f32), V((len(FG), 32, E), f32),
        pltpu.SemaphoreType.DMA((7,)), pltpu.SemaphoreType.DMA((XG,)), pltpu.SemaphoreType.DMA((NPIECE,)),
        pltpu.SemaphoreType.DMA((1,)),
    ]
    out = pl.pallas_call(
        _kernel,
        out_shape=jax.ShapeDtypeStruct((S, 2 * D), bf16),
        in_specs=[pl.BlockSpec(memory_space=pltpu.HBM)] * len(args),
        out_specs=pl.BlockSpec(memory_space=pl.ANY),
        scratch_shapes=scratch,
        compiler_params=pltpu.CompilerParams(vmem_limit_bytes=110 * 1024 * 1024, disable_bounds_checks=True),
    )(*args)
    return out.reshape(1, S, 2 * D)
```

```python
import numpy as np
import jax
import jax.numpy as jnp
from jax import lax
import jax.experimental.pallas as pl
import jax.experimental.pallas.tpu as pltpu

bf16 = jnp.bfloat16
f32 = jnp.float32
u32 = jnp.uint32

S, D = 2048, 640
H, E = 32, 128
M, SEG = 8, 32
L = M + SEG
G = H // 2
DF = D // 2 + 1
HF = D // 2
NT = D // 128
N1, N2 = 16, 128
NPAIR = S // (2 * SEG)
LAG1, LAG2 = 2, 5
CH = (0, 3, 6, 9, 11, 13, 14, 15, 16)
DP = D // 2
WPIECE = 40
NPIECE = 3 * DP // WPIECE
NQ = DP // WPIECE
QPITCH = DP + 8
KPITCH = 2 * DP + 8
UB = 2
RB = 4
FG = [(4, 4), (8, 4), (12, 4), (14, 4)]
NF1 = 2
NBQ = 8
RLP = 10
B0 = 2
U3 = 2
RPITCH = N2 + 8
UA = 4
QP = 16
C5 = (float(np.cos(2 * np.pi / 5)), float(np.cos(4 * np.pi / 5)))
S5 = (float(np.sin(2 * np.pi / 5)), float(np.sin(4 * np.pi / 5)))
HI16 = 0xFFFF0000


def _cos_sin(num, den):
    r = num - den * jnp.floor((num + 0.5) * (1.0 / den))
    ang = r * (2.0 * np.pi / den)
    return jnp.cos(ang), jnp.sin(ang)


def _fft_list(re, im, sign):
    n = len(re)
    if n == 1:
        return re, im
    er, ei = _fft_list(re[0::2], im[0::2], sign)
    orr, oi = _fft_list(re[1::2], im[1::2], sign)
    h = n // 2
    outr = [None] * n
    outi = [None] * n
    r = np.float32(np.sqrt(0.5))
    for k in range(h):
        a, b = orr[k], oi[k]
        if 4 * k == n:
            if sign > 0:
                outr[k], outi[k] = er[k] - b, ei[k] + a
                outr[k + h], outi[k + h] = er[k] + b, ei[k] - a
            else:
                outr[k], outi[k] = er[k] + b, ei[k] - a
                outr[k + h], outi[k + h] = er[k] - b, ei[k] + a
            continue
        if k == 0:
            tr, ti = a, b
        elif 8 * k == n:
            tr, ti = ((a - b) * r, (a + b) * r) if sign > 0 else ((a + b) * r, (b - a) * r)
        elif 8 * k == 3 * n:
            tr, ti = ((a + b) * (-r), (a - b) * r) if sign > 0 else ((b - a) * r, (a + b) * (-r))
        else:
            c = np.float32(np.cos(2 * np.pi * k / n))
            s = np.float32(sign * np.sin(2 * np.pi * k / n))
            tr, ti = a * c - b * s, a * s + b * c
        outr[k], outi[k] = er[k] + tr, ei[k] + ti
        outr[k + h], outi[k + h] = er[k] - tr, ei[k] - ti
    return outr, outi


def _unzip_rows(a, b):
    lo = (a & u32(0xFFFF)) | (b << 16)
    hi = (a >> 16) | (b & u32(HI16))
    return lo, hi


def _radix5(x):
    t1, t2, t3, t4 = x[1] + x[4], x[2] + x[3], x[1] - x[4], x[2] - x[3]
    return (x[0] + t1 + t2,
            x[0] + C5[0] * t1 + C5[1] * t2, S5[0] * t3 + S5[1] * t4,
            x[0] + C5[1] * t1 + C5[0] * t2, S5[1] * t3 - S5[0] * t4)


def _radix5_t(z0, zc1, zs1, zc2, zs2, k):
    z0 = z0 * k
    p1 = z0 + (k * C5[0]) * zc1 + (k * C5[1]) * zc2
    p2 = z0 + (k * C5[1]) * zc1 + (k * C5[0]) * zc2
    q1 = (k * S5[0]) * zs1 + (k * S5[1]) * zs2
    q2 = (k * S5[1]) * zs1 - (k * S5[0]) * zs2
    return z0 + (zc1 + zc2) * k, p1 + q1, p2 + q2, p2 - q2, p1 - q1


def _kernel(xa_hbm, mem_hbm, wq_hbm, wk_hbm, wv_hbm, wo_hbm, xb_hbm, wr_hbm, wi_hbm,
            out_hbm,
            xa, mem, wraw, wo, xbr, xb, wr, wi, ts, tt, gm,
            wq, wkv, vre, vim, rsc, xpk, qpre, obuf, o_scr, stash, fstash,
            sem_in, sem_xb, sem_w, sem_out):
    def cp(src, dst, sem):
        return pltpu.make_async_copy(src, dst, sem)

    def xa_copy(p0, n, r0, nr, sem):
        return cp(xa_hbm.at[pl.ds(p0, n), pl.ds(r0, nr), :], xa.at[pl.ds(p0, n), pl.ds(r0, nr), :], sem)

    c_mem = cp(mem_hbm, mem, sem_in.at[0])
    c_xp = xa_copy(0, NPAIR, 0, QP, sem_in.at[1])
    c_xa0 = xa_copy(0, UA + 1, QP, 64 - QP, sem_in.at[2])
    c_xa1 = xa_copy(UA + 1, NPAIR - UA - 1, QP, 64 - QP, sem_in.at[3])
    c_f = [cp(wr_hbm, wr, sem_in.at[4]), cp(wi_hbm, wi, sem_in.at[5])]
    c_wo = cp(wo_hbm, wo, sem_in.at[6])
    c_xb = [cp(xb_hbm.at[:, pl.ds(8 * h, 8), :], xbr.at[h], sem_xb.at[h]) for h in range(2)]
    c_w = []
    for m, w_hbm in enumerate((wq_hbm, wk_hbm, wv_hbm)):
        for c in range(NQ):
            c_w.append(cp(w_hbm.at[pl.ds(c * WPIECE, WPIECE)], wraw.at[pl.ds(m * DP + c * WPIECE, WPIECE)],
                          sem_w.at[m * NQ + c]))
    c_xb[0].start()

    def relayout_wait(u):
        view = wraw.at[pl.ds(u * WPIECE, WPIECE)]
        cp(view, view, sem_w.at[u]).wait()

    def relayout(u, part, nparts, zero=None, kv=False):
        dst, pitch, off = (wkv, KPITCH, DP) if kv else (wq, QPITCH, 0)
        n = WPIECE // nparts
        for i in range(n):
            dp = u * WPIECE + part * n + i
            ab = pltpu.bitcast(wraw[dp], u32)
            a, b = ab[0:G], ab[G:]
            if zero is not None:
                a = a | zero
            lo, hi = _unzip_rows(a, b)
            dst[0, pl.ds(dp - off, G, stride=pitch), :] = lo
            dst[1, pl.ds(dp - off, G, stride=pitch), :] = hi

    def token(v):
        return (pltpu.bitcast(v[0:G, 0:128], u32) >> 16) >> 16

    first = lax.broadcasted_iota(jnp.int32, (8, N2), 0) == 0
    pack = lambda v: pltpu.bitcast(v.astype(bf16), u32)
    iota = lambda shape, dim: lax.broadcasted_iota(jnp.int32, shape, dim).astype(f32)

    def rotate(c, sn, cr, sr):
        return c * cr - sn * sr, sn * cr + c * sr

    lane = iota((16, 128), 1)
    c8, s8 = _cos_sin(iota((8, 128), 0) * iota((8, 128), 1), 8)

    def gen_tt(r, carry):
        c0, s0 = _cos_sin((r.astype(f32) + 5.0 * iota((16, 128), 0)) * lane, D)
        sg = jnp.where(r >= 3, 1.0, -1.0)
        for g4 in range(4):
            c, sn = (c0, s0) if g4 == 0 else rotate(c0, s0, c8[g4:g4 + 1], s8[g4:g4 + 1])
            ns = -sn
            if g4 == 0:
                ns = jnp.where(lax.broadcasted_iota(jnp.int32, (16, 128), 0) + r == 0, c8[4:5], ns)
            tt[r, 8 * g4:8 * g4 + 8, 0:128] = pack(c)
            tt[r, 8 * g4:8 * g4 + 8, 128:] = pack(sg * sn)
            tt[r, 32 + 8 * g4:40 + 8 * g4, 0:128] = pack(ns)
            tt[r, 32 + 8 * g4:40 + 8 * g4, 128:] = pack(sg * c)
        return carry
    lax.fori_loop(0, 5, gen_tt, 0)
    c_xb[1].start()

    ts[0, 0:N1, :], ts[1, 0:N1, :] = _cos_sin(iota((16, N2), 0) * lane, S)
    c0, s0 = _cos_sin(iota((16, N2), 0) * lane, N2)
    for a in range(N2 // 16):
        c, sn = (c0, s0) if a == 0 else rotate(c0, s0, c8[a:a + 1], s8[a:a + 1])
        ts[0, N1 + 16 * a:N1 + 16 * a + 16, :] = c
        ts[1, N1 + 16 * a:N1 + 16 * a + 16, :] = sn

    def gen_gm(s1, carry):
        ca, sa = ts[0, pl.ds(s1, 1), :], ts[1, pl.ds(s1, 1), :]
        cb, sb = ts[0, N1:, :], ts[1, N1:, :]
        gm[s1, :, 0:N2] = pack(ca * cb - sa * sb)
        gm[s1, :, N2:] = pack(-(sa * cb + ca * sb))
        return carry
    lax.fori_loop(0, N1, gen_gm, 0)
    for c in c_f:
        c.start()

    def dft_mats():
        return (pltpu.bitcast(tt[0, :, 0:128], bf16),
                pltpu.bitcast(jnp.concatenate([tt[1], tt[4]], axis=0), bf16),
                pltpu.bitcast(jnp.concatenate([tt[2], tt[3]], axis=0), bf16))

    nt = (((1,), (1,)), ((), ()))

    def p1(q):
        xw = [xb[j, pl.ds(q & 3, N2, stride=4), :] for j in range(NT)]
        us = [_radix5([pltpu.bitcast(sel(v), f32) for v in xw])
              for sel in (lambda v: v << 16, lambda v: v & u32(HI16))]
        u = [jnp.concatenate([us[0][k], us[1][k]], axis=0) for k in range(5)]
        t0, t1, t2 = dft_mats()
        x0 = lax.dot_general(t0, u[0].astype(bf16), nt, preferred_element_type=f32)
        x14 = lax.dot_general(t1, jnp.concatenate(u[1:3], axis=1).astype(bf16), nt, preferred_element_type=f32)
        x23 = lax.dot_general(t2, jnp.concatenate(u[3:5], axis=1).astype(bf16), nt, preferred_element_type=f32)
        return jnp.concatenate([x0, x14[0:128], x23, x14[128:]], axis=0)

    def bins(r, m0=0):
        return pl.ds(r + 5 * m0, 64 - m0, stride=5)

    def p2(q, xdt):
        for par in range(2):
            s1 = 2 * q + par
            t = jnp.dot(xdt[:, par * N2:(par + 1) * N2].astype(bf16), pltpu.bitcast(gm[s1], bf16),
                        preferred_element_type=f32)
            t1, t2 = t[:, 0:N2], t[:, N2:]
            vre[s1, pl.ds(0, 8, stride=5), :] = t1[0:8] - jnp.where(first, 0.0, t2[64:72])
            vim[s1, pl.ds(0, 8, stride=5), :] = jnp.where(first, 0.0, t1[64:72]) + t2[0:8]
            vre[s1, HF:HF + 8] = t1[64:72]
            vim[s1, HF:HF + 8] = t2[64:72]
            for r in range(5):
                m0 = 8 if r == 0 else 0
                re, im = slice(128 * r + m0, 128 * r + 64), slice(128 * r + 64 + m0, 128 * r + 128)
                vre[s1, bins(r, m0), :] = t1[re] - t2[im]
                vim[s1, bins(r, m0), :] = t1[im] + t2[re]

    def p12(i, carry):
        xs = [p1(UB * i + k) for k in range(UB)]
        for k in range(UB):
            p2(UB * i + k, xs[k])
        return carry

    def p12h(h, carry):
        cp(xbr.at[h], xbr.at[h], sem_xb.at[h]).wait()

        @pl.when(h == 0)
        def _():
            for c in (*c_w[:NQ], c_xp):
                c.start()

        @pl.when(h == 1)
        def _():
            for c in (*c_w[NQ:], c_mem, c_xa0):
                c.start()
            c_wo.start(priority=1)
        w = pltpu.bitcast(xbr[h].reshape(S // 2, D), u32)
        for j in range(NT):
            xb[j, 0:S // 4, :] = w[:, j * 128:(j + 1) * 128]
        return lax.fori_loop(h * (4 // UB), (h + 1) * (4 // UB), p12, carry)
    lax.fori_loop(0, 2, p12h, 0)

    for c in c_f:
        c.wait()

    def p3(rows, wrows):
        re = [vre[s1, rows, :] for s1 in range(N1)]
        im = [vim[s1, rows, :] for s1 in range(N1)]
        xr, xi = _fft_list(re, im, -1)
        yr, yi = [], []
        for k1 in range(N1):
            a = wr[wrows, k1 * N2:(k1 + 1) * N2].astype(f32)
            b = wi[wrows, k1 * N2:(k1 + 1) * N2].astype(f32)
            yr.append(xr[k1] * a - xi[k1] * b)
            yi.append(xr[k1] * b + xi[k1] * a)
        zr, zi = _fft_list(yr, yi, +1)
        for s1 in range(N1):
            vre[s1, rows, :] = zr[s1]
            vim[s1, rows, :] = zi[s1]

    def p3l(i, carry):
        for k in range(U3):
            rows = pl.ds(pl.multiple_of(8 * (U3 * i + k), 8), 8)
            p3(rows, rows)
        return carry
    lax.fori_loop(0, HF // 8 // U3, p3l, 0)
    p3(slice(HF, HF + 8), slice(HF, HF + 1))

    def p4(s1, r):
        zr, zi = vre[s1, bins(r), :], vim[s1, bins(r), :]
        top, bot = jnp.concatenate([zr, zi], axis=1), jnp.concatenate([zi, -zr], axis=1)
        if r == 0:
            f2 = jnp.concatenate([first, first], axis=1)
            nyq = jnp.concatenate([vre[s1, HF:HF + 8, :], vim[s1, HF:HF + 8, :]], axis=1)
            top = jnp.concatenate([jnp.where(f2, 0.5 * top[0:8], top[0:8]), top[8:]], axis=0)
            bot = jnp.concatenate([jnp.where(f2, 0.5 * nyq, bot[0:8]), bot[8:]], axis=0)
        t = lax.dot_general(pltpu.bitcast(gm[s1], bf16), jnp.concatenate([top, bot], axis=0).astype(bf16), nt,
                            preferred_element_type=f32)
        rsc[r, pl.ds(pl.multiple_of(s1 * RPITCH, 8), N2), :] = t
        return t

    def bq(g, k):
        rows = pl.ds(pl.multiple_of(g * QPITCH, 8), DP)
        w = pltpu.bitcast(jnp.concatenate([wq[0, rows, :], wq[1, rows, :]], axis=1), bf16)
        rb = NPAIR * QP // NBQ
        t = jnp.dot(pltpu.bitcast(xpk[k * rb // 2:(k + 1) * rb // 2, :], bf16), w, preferred_element_type=f32)
        qpre[g, k * rb:(k + 1) * rb, :] = t
        return t

    def pacer(u0, kv):
        relayout_wait(u0)
        relayout_wait(u0 + 1)
        state = [0, None]

        def rl(v):
            k, zero = state
            relayout(u0 + k // RLP, k % RLP, RLP, zero, kv)
            state[0], state[1] = k + 1, token(v)
        return rl

    def p4l(i, carry):
        rl = pacer(2 * i, False)
        for k in range(4):
            for r in range(5):
                rl(p4(4 * i + k, r))
        return carry
    lax.fori_loop(0, N1 // 4, p4l, 0)
    c_xp.wait()
    xpk[...] = pltpu.bitcast(xa[:, 0:QP, :].reshape(NPAIR * QP, D), u32)

    def p5q(q, carry):
        rl = pacer(NQ + 2 * q, True)
        t0, t1, t2 = dft_mats()
        ns = N1 // RB

        def p5(rb):
            rc = [jnp.concatenate([rsc[j, pl.ds(N1 * q + ns * rb + k, N1, stride=RPITCH), :] for k in range(ns)],
                                  axis=0) for j in range(NT)]
            z0 = jnp.dot(rc[0].astype(bf16), t0, preferred_element_type=f32)
            z1 = jnp.dot(jnp.concatenate([rc[1], rc[4]], axis=1).astype(bf16), t1, preferred_element_type=f32)
            z2 = jnp.dot(jnp.concatenate([rc[2], rc[3]], axis=1).astype(bf16), t2, preferred_element_type=f32)
            ys = _radix5_t(z0, z1[:, 0:128], z1[:, 128:], z2[:, 0:128], z2[:, 128:], 2.0 / (D * S))
            rows = pl.ds(pl.multiple_of(N1 * (N1 * q + ns * rb), N1 * ns), N1 * ns)
            obuf[rows, D:] = jnp.concatenate(ys, axis=1).astype(bf16)
            return z0

        nb = 2 * NBQ // RB
        for rb in range(RB):
            for k in range(rb * nb, (rb + 1) * nb):
                rl(bq(2 * q + k // NBQ, k % NBQ))
                if k == rb * nb + B0 - 1:
                    rl(p5(rb))
        return carry
    lax.fori_loop(0, N1 // 2, p5q, 0)

    c_mem.wait()
    c_xa0.wait()

    r = lax.broadcasted_iota(jnp.int32, (2 * L, 2 * L), 0)
    c = lax.broadcasted_iota(jnp.int32, (2 * L, 2 * L), 1)
    rb = r >= L
    cb = c >= L
    rr = jnp.where(rb, r - L, r)
    cc = jnp.where(cb, c - L, c)
    mask = (rb == cb) & ((rr < M) | (rr >= cc))
    scale = E ** -0.5

    def wcol(g, c):
        if c < 2:
            return wq[c, g * QPITCH:g * QPITCH + DP, :]
        r0 = g * KPITCH + (c // 2 - 1) * DP
        return wkv[c % 2, r0:r0 + DP, :]

    def filler(p, i0, i1):
        xn = xa[p, 0:32, :]
        if i0 == i1:
            return
        w = jnp.concatenate([wcol(g, c) for g, c in FG[i0:i1]], axis=1)
        t = jnp.dot(xn, pltpu.bitcast(w, bf16), preferred_element_type=f32)
        for i in range(i0, i1):
            fstash[i] = t[:, (i - i0) * E:(i - i0 + 1) * E]

    def step(lhs, even, p):
        nrow_o = 32 if even else 48
        qkv, ps, acc = {}, {}, [None]

        def proj(g):
            def mm(rows, cols):
                w = jnp.concatenate([wcol(g, c) for c in cols], axis=1)
                return jnp.dot(rows, pltpu.bitcast(w, bf16), preferred_element_type=f32)

            if not even:
                t = mm(lhs, range(6))
            else:
                tq = jnp.concatenate([qpre[g, pl.ds(pl.multiple_of(p * QP, QP), QP), :], mm(lhs[QP:], (0, 1))], axis=0)
                moved = [c for gg, c in FG if gg == g]
                if not moved:
                    t = jnp.concatenate([tq, mm(lhs, range(2, 6))], axis=1)
                else:
                    rest = [c for c in range(2, 6) if c not in moved]
                    order = [c for pr in zip(rest, moved + [None] * 4) for c in pr if c is not None]
                    tc = {}
                    for c in order:
                        if c in moved:
                            tc[c] = jnp.concatenate([fstash[FG.index((g, c))], mm(lhs[32:48], (c,))], axis=0)
                        else:
                            tc[c] = mm(lhs, (c,))
                    t = jnp.concatenate([tq] + [tc[c] for c in range(2, 6)], axis=1)
            col = lambda a, i: a[:, i * E:(i + 1) * E]
            if even:
                stash[g] = t[40:48]
                parts = [jnp.concatenate([col(t, 2 * i)[32:40], col(t, 2 * i)[0:32],
                                          col(t, 2 * i + 1)[32:40], col(t, 2 * i + 1)[0:32]], axis=0)
                         for i in range(3)]
            else:
                st = stash[g]
                parts = [jnp.concatenate(
                    [col(t, 2 * i)[16:24], col(st, 2 * i), col(t, 2 * i)[24:32], col(t, 2 * i)[0:16],
                     col(t, 2 * i + 1)[16:24], col(st, 2 * i + 1), col(t, 2 * i + 1)[24:32],
                     col(t, 2 * i + 1)[0:16]], axis=0)
                    for i in range(3)]
            qkv[g] = ((parts[0] * scale).astype(bf16), parts[1].astype(bf16), parts[2].astype(bf16))

        def scores(g):
            q2, k2, _ = qkv[g]
            s = lax.dot_general(q2, k2, (((1,), (1,)), ((), ())), preferred_element_type=f32)
            s = jnp.where(mask, s, -1e9)
            e = jnp.exp(s - jnp.max(s, axis=-1, keepdims=True))
            l = jnp.sum(e, axis=-1, keepdims=True)
            ps[g] = (e * pl.reciprocal(l, approx=True)).astype(bf16)

        def pv(g):
            o2 = jnp.dot(ps[g], qkv[g][2], preferred_element_type=f32)
            o_scr[0:40, (2 * g) * E:(2 * g + 1) * E] = o2[0:40]
            o_scr[0:40, (2 * g + 1) * E:(2 * g + 2) * E] = o2[40:80]

        def wo_chunk(c):
            a, b = CH[c] * 2 * E, CH[c + 1] * 2 * E
            t = jnp.dot(o_scr[0:nrow_o, a:b].astype(bf16), wo[a:b, :], preferred_element_type=f32)
            acc[0] = t if acc[0] is None else acc[0] + t

        ch = 0
        for t in range(G + LAG2):
            if t < G:
                proj(t)
            else:
                assert CH[ch + 1] <= t - LAG2
                wo_chunk(ch)
                ch += 1
            if 0 <= t - LAG1 < G:
                scores(t - LAG1)
            if 0 <= t - LAG2 < G:
                pv(t - LAG2)
        while ch < len(CH) - 1:
            wo_chunk(ch)
            ch += 1
        return acc[0]

    def out_copy(p):
        rows = pl.ds(pl.multiple_of(p * 64, 64), 64)
        return cp(obuf.at[rows, :], out_hbm.at[rows, :], sem_out.at[0])

    def pair(p, mem_v):
        base = pl.multiple_of(p * 64, 64)
        xs = xa[p].astype(f32)
        lhs = jnp.concatenate([xs[0:32], mem_v, xs[32:40]], axis=0).astype(bf16)
        out_e = step(lhs, True, p)
        o_scr[40:48, :] = o_scr[32:40, :]
        pn = jnp.minimum(p + 1, NPAIR - 1)
        filler(pn, 0, NF1)
        lhs = jnp.concatenate([xs[48:64], out_e[0:8], xs[40:48]], axis=0).astype(bf16)
        out_o = step(lhs, False, p)
        filler(pn, NF1, len(FG))
        res = jnp.concatenate([out_e[8:32], out_o[40:48], out_o[8:40]], axis=0)
        obuf[pl.ds(base, 64), 0:D] = res.astype(bf16)
        return out_o[0:8]

    def body(p, mem_v):
        @pl.when(p == 1)
        def _():
            c_xa1.wait()

        @pl.when(p > 0)
        def _():
            out_copy(p * UA - 1).start()
        for k in range(UA):
            if k > 0:
                out_copy(p * UA + k - 1).start()
            mem_v = pair(p * UA + k, mem_v)
        return mem_v

    filler(0, 0, len(FG))
    c_wo.wait()
    c_xa1.start(priority=1)
    lax.fori_loop(0, NPAIR // UA, body, mem[...].astype(f32))

    out_copy(NPAIR - 1).start()
    cp(obuf, obuf, sem_out.at[0]).wait()


@jax.jit
def pallas_concat_heads__memory_aug_recurrent_mem_tr__spectral_gfnet__prompt_kernel(
    A_x: jax.Array,
    A_mem0: jax.Array,
    A_Wq: jax.Array,
    A_Wk: jax.Array,
    A_Wv: jax.Array,
    A_Wo: jax.Array,
    A_seg_len,
    B_x: jax.Array,
    B_w_r: jax.Array,
    B_w_i: jax.Array,
):
    del A_seg_len
    assert A_x.shape == (1, S, D) and B_x.shape == (1, S, D)
    args = (
        A_x.reshape(NPAIR, 64, D), A_mem0.reshape(M, D),
        A_Wq.reshape(DP, 2 * H, E), A_Wk.reshape(DP, 2 * H, E), A_Wv.reshape(DP, 2 * H, E),
        A_Wo.reshape(H * E, D),
        B_x.reshape(N2, N1, D), B_w_r.T, B_w_i.T,
    )
    V = pltpu.VMEM
    scratch = [
        V((NPAIR, 64, D), bf16), V((M, D), bf16), V((3 * DP, 2 * H, E), bf16), V((H * E, D), bf16),
        V((2, N2, 8, D), bf16), V((NT, S // 4 + 8, 128), u32), V((DF, S), bf16), V((DF, S), bf16),
        V((2, N1 + N2, N2), f32), V((5, 64, 256), u32), V((N1, N2 // 2, 2 * N2), u32),
        V((2, (G + 1) * QPITCH, E), u32), V((2, (G + 1) * KPITCH, E), u32),
        V((N1, HF + 8, N2), f32), V((N1, HF + 8, N2), f32),
        V((NT, (N1 + 1) * RPITCH, 128), f32), V((NPAIR * QP // 2, D), u32), V((G, NPAIR * QP, 2 * E), f32),
        V((S, 2 * D), bf16), V((48, H * E), f32), V((G, 8, 6 * E), f32), V((len(FG), 32, E), f32),
        pltpu.SemaphoreType.DMA((7,)), pltpu.SemaphoreType.DMA((2,)), pltpu.SemaphoreType.DMA((NPIECE,)),
        pltpu.SemaphoreType.DMA((1,)),
    ]
    out = pl.pallas_call(
        _kernel,
        out_shape=jax.ShapeDtypeStruct((S, 2 * D), bf16),
        in_specs=[pl.BlockSpec(memory_space=pltpu.HBM)] * len(args),
        out_specs=pl.BlockSpec(memory_space=pl.ANY),
        scratch_shapes=scratch,
        compiler_params=pltpu.CompilerParams(vmem_limit_bytes=110 * 1024 * 1024, disable_bounds_checks=True),
    )(*args)
    return out.reshape(1, S, 2 * D)
```

```python
import functools
import numpy as np
import jax
import jax.numpy as jnp
from jax import lax
import jax.experimental.pallas as pl
import jax.experimental.pallas.tpu as pltpu

bf16 = jnp.bfloat16
f32 = jnp.float32
u32 = jnp.uint32

S, D = 2048, 640
H, E = 32, 128
M, SEG = 8, 32
L = M + SEG
G = H // 2
DF = D // 2 + 1
HF = D // 2
NT = D // 128
N1, N2 = 16, 128
NPAIR = S // (2 * SEG)
LAG1, LAG2 = 2, 5
CH = (0, 3, 6, 9, 11, 13, 14, 15, 16)
DP = D // 2
PITCH = DP + 8
KPC = DP // 2
VPC = (120, 120, 80)
RB = 4
FG = [(4, 4), (8, 4), (12, 4), (14, 4)]
NF1 = 2
NBQ = 8
FROWS = HF // 2
KG = (2, 5, 7, 10, 13, 15, 0)
RPITCH = N2 + 8
UA = 2
QP = 16
C5 = (float(np.cos(2 * np.pi / 5)), float(np.cos(4 * np.pi / 5)))
S5 = (float(np.sin(2 * np.pi / 5)), float(np.sin(4 * np.pi / 5)))
HI16 = 0xFFFF0000
LT = 1
P12 = 'w0 r00 a00 a10 a20 a30 b00 b10 b20 w1 b30 r01 a01 a11 b01 b11 a21 a31 b21 b31 c0 c1 w2 c2 r1 a4 a5 c3 b4 b5 a6 a7 b6 b7 c4 w3 h5 h6 h7 w4'
XO = 0
XBF = 0
PS = 50
EW = 1
NA = 3
RQS = 30
UM = 1
UL = 4
NPS = 3
TWC = [0, 16, 9, 16]
PCOST = ([16 + t for t in TWC] + [64 + t for t in TWC] + [16] * 4 if NPS == 3 else
         [16 + t for t in TWC] + [48] * 4 + [16 + t for t in TWC] + [16] * 4)
PCOST = [c + 8 for c in PCOST]
MS = 38
LT3 = 1


def _cos_sin(num, den):
    r = num - den * jnp.floor((num + 0.5) * (1.0 / den))
    ang = r * (2.0 * np.pi / den)
    return jnp.cos(ang), jnp.sin(ang)


def _fft_list(re, im, sign):
    n = len(re)
    if n == 1:
        return re, im
    er, ei = _fft_list(re[0::2], im[0::2], sign)
    orr, oi = _fft_list(re[1::2], im[1::2], sign)
    h = n // 2
    outr = [None] * n
    outi = [None] * n
    r = np.float32(np.sqrt(0.5))
    for k in range(h):
        a, b = orr[k], oi[k]
        if 4 * k == n:
            if sign > 0:
                outr[k], outi[k] = er[k] - b, ei[k] + a
                outr[k + h], outi[k + h] = er[k] + b, ei[k] - a
            else:
                outr[k], outi[k] = er[k] + b, ei[k] - a
                outr[k + h], outi[k + h] = er[k] - b, ei[k] + a
            continue
        if k == 0:
            tr, ti = a, b
        elif 8 * k == n:
            tr, ti = ((a - b) * r, (a + b) * r) if sign > 0 else ((a + b) * r, (b - a) * r)
        elif 8 * k == 3 * n:
            tr, ti = ((a + b) * (-r), (a - b) * r) if sign > 0 else ((b - a) * r, (a + b) * (-r))
        else:
            c = np.float32(np.cos(2 * np.pi * k / n))
            s = np.float32(sign * np.sin(2 * np.pi * k / n))
            tr, ti = a * c - b * s, a * s + b * c
        outr[k], outi[k] = er[k] + tr, ei[k] + ti
        outr[k + h], outi[k + h] = er[k] - tr, ei[k] - ti
    return outr, outi


def _twiddle(a, b, m, sign):
    m %= 16
    if m == 0:
        return a, b
    if m == 4:
        return (-b, a) if sign > 0 else (b, -a)
    r = np.float32(np.sqrt(0.5))
    if m == 2:
        return ((a - b) * r, (a + b) * r) if sign > 0 else ((a + b) * r, (b - a) * r)
    if m == 6:
        return ((a + b) * (-r), (a - b) * r) if sign > 0 else ((b - a) * r, (a + b) * (-r))
    c = np.float32(np.cos(2 * np.pi * m / 16))
    s = np.float32(sign * np.sin(2 * np.pi * m / 16))
    return a * c - b * s, a * s + b * c


def _unzip_rows(a, b):
    lo = (a & u32(0xFFFF)) | (b << 16)
    hi = (a >> 16) | (b & u32(HI16))
    return lo, hi


def _radix5(x):
    t1, t2, t3, t4 = x[1] + x[4], x[2] + x[3], x[1] - x[4], x[2] - x[3]
    return (x[0] + t1 + t2,
            x[0] + C5[0] * t1 + C5[1] * t2, S5[0] * t3 + S5[1] * t4,
            x[0] + C5[1] * t1 + C5[0] * t2, S5[1] * t3 - S5[0] * t4)


def _radix5_t(z0, zc1, zs1, zc2, zs2, k):
    z0 = z0 * k
    p1 = z0 + (k * C5[0]) * zc1 + (k * C5[1]) * zc2
    p2 = z0 + (k * C5[1]) * zc1 + (k * C5[0]) * zc2
    q1 = (k * S5[0]) * zs1 + (k * S5[1]) * zs2
    q2 = (k * S5[1]) * zs1 - (k * S5[0]) * zs2
    return z0 + (zc1 + zc2) * k, p1 + q1, p2 + q2, p2 - q2, p1 - q1


def _kernel(xa_hbm, mem_hbm, wq_hbm, wk_hbm, wv_hbm, wo_hbm, xb_hbm, wr_hbm, wi_hbm,
            out_hbm,
            xa, mem, wqr, wkr, wvr, wo, xbr, xb, wr, wi, ts, tt, gm,
            wq, wk, wv, vre, vim, rsc, xpk, qpre, obuf, o_scr, stash, fstash,
            sem_in, sem_f, sem_w, sem_out):
    def cp(src, dst, sem):
        return pltpu.make_async_copy(src, dst, sem)

    def xa_copy(p0, n, r0, nr, sem):
        return cp(xa_hbm.at[pl.ds(p0, n), pl.ds(r0, nr), :], xa.at[pl.ds(p0, n), pl.ds(r0, nr), :], sem)

    def rows_copy(src, dst, r0, n, sem):
        return cp(src.at[pl.ds(r0, n)], dst.at[pl.ds(r0, n)], sem)

    def start(*cs):
        for c in cs:
            c.start()

    def wait(*cs):
        for c in cs:
            c.wait()

    c_mem = cp(mem_hbm, mem, sem_in.at[0])
    c_xp = xa_copy(0, NPAIR, 0, QP, sem_in.at[1])
    c_xa0 = xa_copy(0, UA + 1, QP, 64 - QP, sem_in.at[2])
    c_xa1 = xa_copy(UA + 1, NPAIR - UA - 1, QP, 64 - QP, sem_in.at[3])
    c_fn = [rows_copy(wr_hbm, wr, HF, 1, sem_in.at[4]), rows_copy(wi_hbm, wi, HF, 1, sem_in.at[5])]
    c_wo = cp(wo_hbm, wo, sem_in.at[6])
    c_xb = [cp(xb_hbm.at[pl.ds(0, 64), pl.ds(0, 8), :], xbr.at[0, pl.ds(0, 64)], sem_in.at[7]),
            cp(xb_hbm.at[pl.ds(64, 64), pl.ds(0, 8), :], xbr.at[0, pl.ds(64, 64)], sem_in.at[11]),
            cp(xb_hbm.at[:, pl.ds(8, 8), :], xbr.at[1], sem_in.at[8])]
    c_q = [cp(wq_hbm.at[:, :, pl.ds(G * h, G), :], wqr.at[h], sem_in.at[9 + h]) for h in range(2)]
    c_f = lambda i: [rows_copy(wr_hbm, wr, pl.multiple_of(i * FROWS, FROWS), FROWS, sem_f.at[2 * i]),
                     rows_copy(wi_hbm, wi, pl.multiple_of(i * FROWS, FROWS), FROWS, sem_f.at[2 * i + 1])]
    c_k = lambda i: rows_copy(wk_hbm, wkr, i * KPC, KPC, sem_w.at[i])
    c_v = lambda i, n: rows_copy(wv_hbm, wvr, i * VPC[0], n, sem_w.at[2 + i])
    c_xb[0].start()

    def relayout(src, dst, dp, zero):
        ab = pltpu.bitcast(src[dp], u32)
        lo, hi = _unzip_rows(ab[0:G] if zero is None else ab[0:G] | zero, ab[G:])
        dst[0, pl.ds(dp, G, stride=PITCH), :] = lo
        dst[1, pl.ds(dp, G, stride=PITCH), :] = hi

    def relayout_q(h, dp, zero):
        a, b = pltpu.bitcast(wqr[h, dp, 0], u32), pltpu.bitcast(wqr[h, dp, 1], u32)
        lo, hi = _unzip_rows(a if zero is None else a | zero[0:8], b)
        wq[0, pl.ds(8 * h * PITCH + dp, 8, stride=PITCH), :] = lo
        wq[1, pl.ds(8 * h * PITCH + dp, 8, stride=PITCH), :] = hi

    def pacer(jobs, nslot, LT=LT, cost=None):
        toks = []
        cum = np.cumsum([0] + list(cost or [1] * len(jobs)))
        slot = (cum[:-1] + cum[1:]) * nslot // (2 * cum[-1])

        def hook(t):
            k = len(toks)
            for job, sl in zip(jobs, slot):
                if sl == k:
                    job(toks[k - LT] if k >= LT else None)
            toks.append(token(t))
        return hook

    def token(v):
        return (pltpu.bitcast(v[0:G, 0:128], u32) >> 16) >> 16

    first = lax.broadcasted_iota(jnp.int32, (8, N2), 0) == 0
    pack = lambda v: pltpu.bitcast(v.astype(bf16), u32)
    iota = lambda shape, dim: lax.broadcasted_iota(jnp.int32, shape, dim).astype(f32)

    def rotate(c, sn, cr, sr):
        return c * cr - sn * sr, sn * cr + c * sr

    lane = iota((16, 128), 1)
    c8, s8 = _cos_sin(iota((8, 128), 0) * iota((8, 128), 1), 8)

    def gen_tt(r, carry):
        c0, s0 = _cos_sin((r.astype(f32) + 5.0 * iota((16, 128), 0)) * lane, D)
        sg = jnp.where(r >= 3, 1.0, -1.0)
        for g4 in range(4):
            c, sn = (c0, s0) if g4 == 0 else rotate(c0, s0, c8[g4:g4 + 1], s8[g4:g4 + 1])
            ns = -sn
            if g4 == 0:
                ns = jnp.where(lax.broadcasted_iota(jnp.int32, (16, 128), 0) + r == 0, c8[4:5], ns)
            tt[r, 8 * g4:8 * g4 + 8, 0:128] = pack(c)
            tt[r, 8 * g4:8 * g4 + 8, 128:] = pack(sg * sn)
            tt[r, 32 + 8 * g4:40 + 8 * g4, 0:128] = pack(ns)
            tt[r, 32 + 8 * g4:40 + 8 * g4, 128:] = pack(sg * c)
        return carry
    lax.fori_loop(0, 5, gen_tt, 0)
    c_xb[1].start()
    if XO:
        c_xb[2].start()

    ts[0, 0:N1, :], ts[1, 0:N1, :] = _cos_sin(iota((16, N2), 0) * lane, S)
    c0, s0 = _cos_sin(iota((16, N2), 0) * lane, N2)
    for a in range(N2 // 16):
        c, sn = (c0, s0) if a == 0 else rotate(c0, s0, c8[a:a + 1], s8[a:a + 1])
        ts[0, N1 + 16 * a:N1 + 16 * a + 16, :] = c
        ts[1, N1 + 16 * a:N1 + 16 * a + 16, :] = sn

    def gen_gm(s1, carry):
        ca, sa = ts[0, pl.ds(s1, 1), :], ts[1, pl.ds(s1, 1), :]
        cb, sb = ts[0, N1:, :], ts[1, N1:, :]
        gm[s1, :, 0:N2] = pack(ca * cb - sa * sb)
        gm[s1, :, N2:] = pack(-(sa * cb + ca * sb))
        return carry
    lax.fori_loop(0, N1, gen_gm, 0)
    if not XO:
        c_xb[2].start()
    else:
        c_q[0].start()

    def dft_mats():
        return (pltpu.bitcast(tt[0, :, 0:128], bf16),
                pltpu.bitcast(jnp.concatenate([tt[1], tt[4]], axis=0), bf16),
                pltpu.bitcast(jnp.concatenate([tt[2], tt[3]], axis=0), bf16))

    nt = (((1,), (1,)), ((), ()))

    def p1a(q, m=None):
        rows = pl.ds(q % 4, N2, stride=4) if m is None else pl.ds(256 * m + q % 4, 64, stride=4)
        xw = [xb[q // 4, j, rows, :] for j in range(NT)]
        us = [_radix5([pltpu.bitcast(sel(v), f32) for v in xw])
              for sel in (lambda v: v << 16, lambda v: v & u32(HI16))]
        us = us[::-1] if m == 1 else us
        u = [jnp.concatenate([us[0][k], us[1][k]], axis=0) for k in range(5)]
        return (u[0].astype(bf16), jnp.concatenate(u[1:3], axis=1).astype(bf16),
                jnp.concatenate(u[3:5], axis=1).astype(bf16))

    def p1b(u):
        x0, x14, x23 = [lax.dot_general(t, v, nt, preferred_element_type=f32) for t, v in zip(dft_mats(), u)]
        x = jnp.concatenate([x0, x14[0:128], x23, x14[128:]], axis=0)
        return x.astype(bf16) if XBF else x

    def bins(r, m0=0):
        return pl.ds(r + 5 * m0, 64 - m0, stride=5)

    def p2(q, xdt, hook=None):
        for par in range(2):
            s1 = 2 * q + par
            if isinstance(xdt, tuple):
                low = lax.broadcasted_iota(jnp.int32, (NT * 128, N2), 1) < 64
                x, g = jnp.where(low, xdt[par], xdt[1 - par]), gm[s1]
                g = jnp.concatenate([g[32:], g[0:32]], axis=0) if par else g
            else:
                x, g = xdt[:, par * N2:(par + 1) * N2], gm[s1]
            t = jnp.dot(x.astype(bf16), pltpu.bitcast(g, bf16), preferred_element_type=f32)
            if hook is not None:
                for r in range(5):
                    hook(t[128 * r:])
            t1, t2 = t[:, 0:N2], t[:, N2:]
            vre[s1, pl.ds(0, 8, stride=5), :] = t1[0:8] - jnp.where(first, 0.0, t2[64:72])
            vim[s1, pl.ds(0, 8, stride=5), :] = jnp.where(first, 0.0, t1[64:72]) + t2[0:8]
            vre[s1, HF:HF + 8] = t1[64:72]
            vim[s1, HF:HF + 8] = t2[64:72]
            for r in range(5):
                m0 = 8 if r == 0 else 0
                re, im = slice(128 * r + m0, 128 * r + 64), slice(128 * r + 64 + m0, 128 * r + 128)
                vre[s1, bins(r, m0), :] = t1[re] - t2[im]
                vim[s1, bins(r, m0), :] = t1[im] + t2[re]

    def repack(h, m0, n):
        w = pltpu.bitcast(xbr[h, m0:m0 + n].reshape(8 * n, D), u32)
        for j in range(NT):
            xb[h, j, 4 * m0:4 * (m0 + n), :] = w[:, j * 128:(j + 1) * 128]

    us, xs = {}, {}
    hook = pacer([functools.partial(relayout_q, 0, dp) for dp in range(DP)], RQS)
    for op in P12.split():
        q, m = int(op[1]), (int(op[2]) if len(op) > 2 else None)
        if op == 'w0':
            c_xb[0].wait()
            if not XO:
                c_q[0].start()
        elif op == 'w1':
            c_xb[1].wait()
            start(c_xp, c_q[1], *c_fn)
        elif op == 'w2':
            c_xb[2].wait()
            start(*c_f(0), *c_f(1))
        elif op == 'w3':
            c_q[0].wait()
            start(c_k(0), c_k(1))
        elif op == 'w4':
            c_xp.wait()
            start(c_v(0, VPC[0]), c_v(1, VPC[1]), c_v(2, VPC[2]))
            xpk[...] = pltpu.bitcast(xa[:, 0:QP, :].reshape(NPAIR * QP, D), u32)
        elif op[0] == 'r':
            repack(q, *((0, N2) if m is None else (64 * m, 64)))
        elif op[0] == 'a':
            us[q, m] = p1a(q, m)
        elif op[0] == 'b':
            xs[q, m] = p1b(us[q, m])
        else:
            p2(q, xs[q, None] if (q, None) in xs else (xs[q, 0], xs[q, 1]), hook if op[0] == 'h' else None)

    def p3(rows, wrows, j, zero=None):
        ps, x = divmod(j, 4)
        last = NPS - 1
        slots = [4 * b + x for b in range(4)] if ps in (0, last) else [4 * x + a for a in range(4)]
        re = [vre[n, rows, :] for n in slots]
        im = [vim[n, rows, :] for n in slots]
        if zero is not None:
            re[0] = pltpu.bitcast(pltpu.bitcast(re[0], u32) | zero[0:8], f32)
            im[0] = pltpu.bitcast(pltpu.bitcast(im[0], u32) | zero[0:8], f32)
        re, im = _fft_list(re, im, +1 if ps >= 2 else -1)
        if ps == 1:
            yr, yi = [], []
            for d in range(4):
                k1 = x + 4 * d
                a = wr[wrows, k1 * N2:(k1 + 1) * N2].astype(f32)
                b = wi[wrows, k1 * N2:(k1 + 1) * N2].astype(f32)
                yr.append(re[d] * a - im[d] * b)
                yi.append(re[d] * b + im[d] * a)
            re, im = _fft_list(yr, yi, +1) if NPS == 3 else (yr, yi)
        if ps in (0, last - 1):
            tw = [_twiddle(re[i], im[i], x * i, -1 if ps == 0 else +1) for i in range(4)]
            re, im = [t[0] for t in tw], [t[1] for t in tw]
        for i, n in enumerate(slots):
            vre[n, rows, :] = re[i]
            vim[n, rows, :] = im[i]

    def p4(s1, r):
        zr, zi = vre[s1, bins(r), :], vim[s1, bins(r), :]
        top, bot = jnp.concatenate([zr, zi], axis=1), jnp.concatenate([zi, -zr], axis=1)
        if r == 0:
            f2 = jnp.concatenate([first, first], axis=1)
            nyq = jnp.concatenate([vre[s1, HF:HF + 8, :], vim[s1, HF:HF + 8, :]], axis=1)
            top = jnp.concatenate([jnp.where(f2, 0.5 * top[0:8], top[0:8]), top[8:]], axis=0)
            bot = jnp.concatenate([jnp.where(f2, 0.5 * nyq, bot[0:8]), bot[8:]], axis=0)
        t = lax.dot_general(pltpu.bitcast(gm[s1], bf16), jnp.concatenate([top, bot], axis=0).astype(bf16), nt,
                            preferred_element_type=f32)
        rsc[r, pl.ds(pl.multiple_of(s1 * RPITCH, 8), N2), :] = t
        return t

    def bq(w, g, j, k, hook=None):
        rows = pl.ds(pl.multiple_of(g * PITCH, 8), DP)
        w = pltpu.bitcast(jnp.concatenate([w[0, rows, :], w[1, rows, :]], axis=1), bf16)
        rb = NPAIR * QP // NBQ
        x = pltpu.bitcast(xpk[k * rb // 2:(k + 1) * rb // 2, :], bf16)
        if hook is None:
            t = jnp.dot(x, w, preferred_element_type=f32)
        else:
            t = None
            for c in range(NT):
                u = jnp.dot(x[:, c * 128:(c + 1) * 128], w[c * 128:(c + 1) * 128], preferred_element_type=f32)
                hook(u)
                t = u if t is None else t + u
        qpre[j, k * rb:(k + 1) * rb, :] = t
        return t

    def unit(w, g, j, hook=None):
        for k in range(NBQ):
            bq(w, g, j, k, hook)

    for g in range(NA):
        unit(wq, g, g)
    wait(c_q[1], *c_fn)
    start(c_mem, c_xa0)
    c_wo.start(priority=1)
    hook = pacer([functools.partial(p3, slice(HF, HF + 8), slice(HF, HF + 1), j) for j in range(4 * NPS)]
                 + [functools.partial(relayout_q, 1, dp) for dp in range(DP)], 2 * NBQ * NT)
    unit(wq, NA, NA, hook)
    unit(wq, NA + 1, NA + 1, hook)

    def p3q(i, carry):
        wait(*c_f(i))
        rows = lambda c: pl.ds(pl.multiple_of(i * FROWS + 8 * c, 8), 8)
        hook = pacer([functools.partial(p3, rows(c), rows(c), j) for c in range(FROWS // 8) for j in range(4 * NPS)],
                     UL * NBQ * NT - 2, LT3, PCOST * (FROWS // 8))
        for g in range(UL):
            unit(wq, NA + 2 + UL * i + g, NA + 2 + UL * i + g, hook)
        return carry
    lax.fori_loop(0, 2, p3q, 0)

    def p4l(i, carry):
        c_k(i).wait()
        hook = pacer([functools.partial(relayout, wkr, wk, i * KPC + d) for d in range(KPC)], 40 + UM * MS)
        for k in range(N1 // 2):
            if UM:
                bq(wq, NA + 2 + 2 * UL + i, NA + 2 + 2 * UL + i, k, hook)
            for r in range(5):
                hook(p4(N1 // 2 * i + k, r))
        return carry
    lax.fori_loop(0, 2, p4l, 0)

    def p5q(q, carry):
        c_v(q, VPC[0]).wait()
        hook = pacer([functools.partial(relayout, wvr, wv, q * VPC[0] + d) for d in range(VPC[0])], 44 - 8 * UM - 8 * (UL - 4))
        t0, t1, t2 = dft_mats()
        ns = N1 // RB

        def p5(rb):
            rc = [jnp.concatenate([rsc[j, pl.ds(ns * rb + k, N1, stride=RPITCH), :] for k in range(ns)],
                                  axis=0) for j in range(NT)]
            z0 = jnp.dot(rc[0].astype(bf16), t0, preferred_element_type=f32)
            z1 = jnp.dot(jnp.concatenate([rc[1], rc[4]], axis=1).astype(bf16), t1, preferred_element_type=f32)
            z2 = jnp.dot(jnp.concatenate([rc[2], rc[3]], axis=1).astype(bf16), t2, preferred_element_type=f32)
            ys = _radix5_t(z0, z1[:, 0:128], z1[:, 128:], z2[:, 0:128], z2[:, 128:], 2.0 / (D * S))
            rows = pl.ds(pl.multiple_of(N1 * (ns * rb), N1 * ns), N1 * ns)
            obuf[rows, D:] = jnp.concatenate(ys, axis=1).astype(bf16)
            return z0

        nk = 2 if NA == 2 else 3
        units = [(wq, 14 + q, 14 + q)] if NA == 2 else []
        units += [(wk, KG[k] + (KG[nk + k] - KG[k]) * q, G + k + nk * q) for k in range(nk)]
        nb = len(units) * NBQ
        for k in range(nb):
            hook(bq(*units[k // NBQ], k % NBQ))
            for rb in range(k * 16 // nb, (k + 1) * 16 // nb):
                hook(p5(16 * q + rb))
        return carry
    lax.fori_loop(0, 2, p5q, 0)

    c_v(2, VPC[2]).wait()
    if EW:
        wait(c_mem, c_xa0)
    hook = pacer([functools.partial(relayout, wvr, wv, 2 * VPC[0] + d) for d in range(VPC[2])], PS)
    if NA == 2:
        unit(wk, KG[4], G + 4, hook)
        unit(wk, KG[5], G + 5, hook)
    else:
        unit(wq, G - 1, G - 1, hook)
        unit(wk, KG[6], G + 6, hook)

    if not EW:
        wait(c_mem, c_xa0)

    r = lax.broadcasted_iota(jnp.int32, (2 * L, 2 * L), 0)
    c = lax.broadcasted_iota(jnp.int32, (2 * L, 2 * L), 1)
    rb = r >= L
    cb = c >= L
    rr = jnp.where(rb, r - L, r)
    cc = jnp.where(cb, c - L, c)
    mask = (rb == cb) & ((rr < M) | (rr >= cc))
    scale = E ** -0.5

    def wcol(g, c):
        return (wq, wk, wv)[c // 2][c % 2, g * PITCH:g * PITCH + DP, :]

    def filler(p, i0, i1):
        xn = xa[p, 0:32, :]
        if i0 == i1:
            return
        w = jnp.concatenate([wcol(g, c) for g, c in FG[i0:i1]], axis=1)
        t = jnp.dot(xn, pltpu.bitcast(w, bf16), preferred_element_type=f32)
        for i in range(i0, i1):
            fstash[i] = t[:, (i - i0) * E:(i - i0 + 1) * E]

    def step(lhs, even, p):
        nrow_o = 32 if even else 48
        qkv, ps, acc = {}, {}, [None]

        def proj(g):
            def mm(rows, cols):
                w = jnp.concatenate([wcol(g, c) for c in cols], axis=1)
                return jnp.dot(rows, pltpu.bitcast(w, bf16), preferred_element_type=f32)

            if not even:
                t = mm(lhs, range(6))
            else:
                pre = lambda j: qpre[j, pl.ds(pl.multiple_of(p * QP, QP), QP), :]
                tq = jnp.concatenate([pre(g), mm(lhs[QP:], (0, 1))], axis=0)
                moved = [c for gg, c in FG if gg == g]
                if g in KG:
                    assert not moved
                    tk = jnp.concatenate([pre(G + KG.index(g)), mm(lhs[QP:], (2, 3))], axis=0)
                    t = jnp.concatenate([tq, tk, mm(lhs, (4, 5))], axis=1)
                elif not moved:
                    t = jnp.concatenate([tq, mm(lhs, range(2, 6))], axis=1)
                else:
                    rest = [c for c in range(2, 6) if c not in moved]
                    order = [c for pr in zip(rest, moved + [None] * 4) for c in pr if c is not None]
                    tc = {}
                    for c in order:
                        if c in moved:
                            tc[c] = jnp.concatenate([fstash[FG.index((g, c))], mm(lhs[32:48], (c,))], axis=0)
                        else:
                            tc[c] = mm(lhs, (c,))
                    t = jnp.concatenate([tq] + [tc[c] for c in range(2, 6)], axis=1)
            col = lambda a, i: a[:, i * E:(i + 1) * E]
            if even:
                stash[g] = t[40:48]
                parts = [jnp.concatenate([col(t, 2 * i)[32:40], col(t, 2 * i)[0:32],
                                          col(t, 2 * i + 1)[32:40], col(t, 2 * i + 1)[0:32]], axis=0)
                         for i in range(3)]
            else:
                st = stash[g]
                parts = [jnp.concatenate(
                    [col(t, 2 * i)[16:24], col(st, 2 * i), col(t, 2 * i)[24:32], col(t, 2 * i)[0:16],
                     col(t, 2 * i + 1)[16:24], col(st, 2 * i + 1), col(t, 2 * i + 1)[24:32],
                     col(t, 2 * i + 1)[0:16]], axis=0)
                    for i in range(3)]
            qkv[g] = ((parts[0] * scale).astype(bf16), parts[1].astype(bf16), parts[2].astype(bf16))

        def scores(g):
            q2, k2, _ = qkv[g]
            s = lax.dot_general(q2, k2, (((1,), (1,)), ((), ())), preferred_element_type=f32)
            s = jnp.where(mask, s, -1e9)
            e = jnp.exp(s - jnp.max(s, axis=-1, keepdims=True))
            l = jnp.sum(e, axis=-1, keepdims=True)
            ps[g] = (e * pl.reciprocal(l, approx=True)).astype(bf16)

        def pv(g):
            o2 = jnp.dot(ps[g], qkv[g][2], preferred_element_type=f32)
            o_scr[0:40, (2 * g) * E:(2 * g + 1) * E] = o2[0:40]
            o_scr[0:40, (2 * g + 1) * E:(2 * g + 2) * E] = o2[40:80]

        def wo_chunk(c):
            a, b = CH[c] * 2 * E, CH[c + 1] * 2 * E
            t = jnp.dot(o_scr[0:nrow_o, a:b].astype(bf16), wo[a:b, :], preferred_element_type=f32)
            acc[0] = t if acc[0] is None else acc[0] + t

        ch = 0
        for t in range(G + LAG2):
            if t < G:
                proj(t)
            else:
                assert CH[ch + 1] <= t - LAG2
                wo_chunk(ch)
                ch += 1
            if 0 <= t - LAG1 < G:
                scores(t - LAG1)
            if 0 <= t - LAG2 < G:
                pv(t - LAG2)
        while ch < len(CH) - 1:
            wo_chunk(ch)
            ch += 1
        return acc[0]

    def out_copy(p):
        rows = pl.ds(pl.multiple_of(p * 64, 64), 64)
        return cp(obuf.at[rows, :], out_hbm.at[rows, :], sem_out.at[0])

    def pair(p, mem_v):
        base = pl.multiple_of(p * 64, 64)
        xs = xa[p].astype(f32)
        lhs = jnp.concatenate([xs[0:32], mem_v, xs[32:40]], axis=0).astype(bf16)
        out_e = step(lhs, True, p)
        o_scr[40:48, :] = o_scr[32:40, :]
        pn = jnp.minimum(p + 1, NPAIR - 1)
        filler(pn, 0, NF1)
        lhs = jnp.concatenate([xs[48:64], out_e[0:8], xs[40:48]], axis=0).astype(bf16)
        out_o = step(lhs, False, p)
        filler(pn, NF1, len(FG))
        res = jnp.concatenate([out_e[8:32], out_o[40:48], out_o[8:40]], axis=0)
        obuf[pl.ds(base, 64), 0:D] = res.astype(bf16)
        return out_o[0:8]

    def body(p, mem_v):
        @pl.when(p == 1)
        def _():
            c_xa1.wait()

        @pl.when(p > 0)
        def _():
            out_copy(p * UA - 1).start()
        for k in range(UA):
            if k > 0:
                out_copy(p * UA + k - 1).start()
            mem_v = pair(p * UA + k, mem_v)
        return mem_v

    filler(0, 0, len(FG))
    c_wo.wait()
    c_xa1.start(priority=1)
    lax.fori_loop(0, NPAIR // UA, body, mem[...].astype(f32))

    out_copy(NPAIR - 1).start()
    cp(obuf, obuf, sem_out.at[0]).wait()


@jax.jit
def pallas_concat_heads__memory_aug_recurrent_mem_tr__spectral_gfnet__prompt_kernel(
    A_x: jax.Array,
    A_mem0: jax.Array,
    A_Wq: jax.Array,
    A_Wk: jax.Array,
    A_Wv: jax.Array,
    A_Wo: jax.Array,
    A_seg_len,
    B_x: jax.Array,
    B_w_r: jax.Array,
    B_w_i: jax.Array,
):
    del A_seg_len
    assert A_x.shape == (1, S, D) and B_x.shape == (1, S, D)
    args = (
        A_x.reshape(NPAIR, 64, D), A_mem0.reshape(M, D),
        A_Wq.reshape(DP, 2, H, E), A_Wk.reshape(DP, 2 * H, E), A_Wv.reshape(DP, 2 * H, E),
        A_Wo.reshape(H * E, D),
        B_x.reshape(N2, N1, D), B_w_r.T, B_w_i.T,
    )
    V = pltpu.VMEM
    scratch = [
        V((NPAIR, 64, D), bf16), V((M, D), bf16),
        V((2, DP, 2, G, E), bf16), V((DP, 2 * H, E), bf16), V((DP, 2 * H, E), bf16), V((H * E, D), bf16),
        V((2, N2, 8, D), bf16), V((2, NT, S // 4 + 8, 128), u32), V((DF, S), bf16), V((DF, S), bf16),
        V((2, N1 + N2, N2), f32), V((5, 64, 256), u32), V((N1, N2 // 2, 2 * N2), u32),
        V((2, (G + 1) * PITCH, E), u32), V((2, (G + 1) * PITCH, E), u32), V((2, (G + 1) * PITCH, E), u32),
        V((N1, HF + 8, N2), f32), V((N1, HF + 8, N2), f32),
        V((NT, (N1 + 1) * RPITCH, 128), f32), V((NPAIR * QP // 2, D), u32),
        V((G + len(KG), NPAIR * QP, 2 * E), f32),
        V((S, 2 * D), bf16), V((48, H * E), f32), V((G, 8, 6 * E), f32), V((len(FG), 32, E), f32),
        pltpu.SemaphoreType.DMA((12,)), pltpu.SemaphoreType.DMA((4,)), pltpu.SemaphoreType.DMA((5,)),
        pltpu.SemaphoreType.DMA((1,)),
    ]
    out = pl.pallas_call(
        _kernel,
        out_shape=jax.ShapeDtypeStruct((S, 2 * D), bf16),
        in_specs=[pl.BlockSpec(memory_space=pltpu.HBM)] * len(args),
        out_specs=pl.BlockSpec(memory_space=pl.ANY),
        scratch_shapes=scratch,
        compiler_params=pltpu.CompilerParams(vmem_limit_bytes=110 * 1024 * 1024, disable_bounds_checks=True),
    )(*args)
    return out.reshape(1, S, 2 * D)
```

```python
import functools
import numpy as np
import jax
import jax.numpy as jnp
from jax import lax
import jax.experimental.pallas as pl
import jax.experimental.pallas.tpu as pltpu

bf16 = jnp.bfloat16
f32 = jnp.float32
u32 = jnp.uint32

S, D = 2048, 640
H, E = 32, 128
M, SEG = 8, 32
L = M + SEG
G = H // 2
DF = D // 2 + 1
HF = D // 2
NT = D // 128
N1, N2 = 16, 128
NPAIR = S // (2 * SEG)
LAG1, LAG2 = 2, 5
CH = (0, 3, 7, 10, 12, 13, 14, 15, 16)
DP = D // 2
PITCH = DP + 8
KPC = DP // 2
VPC = (120, 120, 80)
RB = 4
FG = [(4, 4), (8, 4), (12, 4), (14, 4)]
NF1 = 2
NBQ = 8
FROWS = HF // 2
KG = (0, 1, 2, 10, 13, 15, 6)
RPITCH = N2 + 8
UA = 2
QP = 16
C5 = (float(np.cos(2 * np.pi / 5)), float(np.cos(4 * np.pi / 5)))
S5 = (float(np.sin(2 * np.pi / 5)), float(np.sin(4 * np.pi / 5)))
HI16 = 0xFFFF0000
P12 = ('w0 r00 a00 a10 a20 a30 b00 b10 b20 w1 b30 r01 a01 a11 b01 b11 a21 a31 b21 b31 c0 c1 '
       'w2 c2 r1 a4 a5 c3 b4 b5 a6 a7 b6 b7 c4 w3 h5 h6 h7 w4')
P3COST = (24, 40, 33, 40, 72, 88, 81, 88, 24, 24, 24, 24)


def _cos_sin(num, den):
    r = num - den * jnp.floor((num + 0.5) * (1.0 / den))
    ang = r * (2.0 * np.pi / den)
    return jnp.cos(ang), jnp.sin(ang)


def _fft_list(re, im, sign):
    n = len(re)
    if n == 1:
        return re, im
    er, ei = _fft_list(re[0::2], im[0::2], sign)
    orr, oi = _fft_list(re[1::2], im[1::2], sign)
    h = n // 2
    outr = [None] * n
    outi = [None] * n
    r = np.float32(np.sqrt(0.5))
    for k in range(h):
        a, b = orr[k], oi[k]
        if 4 * k == n:
            if sign > 0:
                outr[k], outi[k] = er[k] - b, ei[k] + a
                outr[k + h], outi[k + h] = er[k] + b, ei[k] - a
            else:
                outr[k], outi[k] = er[k] + b, ei[k] - a
                outr[k + h], outi[k + h] = er[k] - b, ei[k] + a
            continue
        if k == 0:
            tr, ti = a, b
        elif 8 * k == n:
            tr, ti = ((a - b) * r, (a + b) * r) if sign > 0 else ((a + b) * r, (b - a) * r)
        elif 8 * k == 3 * n:
            tr, ti = ((a + b) * (-r), (a - b) * r) if sign > 0 else ((b - a) * r, (a + b) * (-r))
        else:
            c = np.float32(np.cos(2 * np.pi * k / n))
            s = np.float32(sign * np.sin(2 * np.pi * k / n))
            tr, ti = a * c - b * s, a * s + b * c
        outr[k], outi[k] = er[k] + tr, ei[k] + ti
        outr[k + h], outi[k + h] = er[k] - tr, ei[k] - ti
    return outr, outi


def _twiddle(a, b, m, sign):
    m %= 16
    if m == 0:
        return a, b
    if m == 4:
        return (-b, a) if sign > 0 else (b, -a)
    r = np.float32(np.sqrt(0.5))
    if m == 2:
        return ((a - b) * r, (a + b) * r) if sign > 0 else ((a + b) * r, (b - a) * r)
    if m == 6:
        return ((a + b) * (-r), (a - b) * r) if sign > 0 else ((b - a) * r, (a + b) * (-r))
    c = np.float32(np.cos(2 * np.pi * m / 16))
    s = np.float32(sign * np.sin(2 * np.pi * m / 16))
    return a * c - b * s, a * s + b * c


def _unzip_rows(a, b):
    lo = (a & u32(0xFFFF)) | (b << 16)
    hi = (a >> 16) | (b & u32(HI16))
    return lo, hi


def _radix5(x):
    t1, t2, t3, t4 = x[1] + x[4], x[2] + x[3], x[1] - x[4], x[2] - x[3]
    return (x[0] + t1 + t2,
            x[0] + C5[0] * t1 + C5[1] * t2, S5[0] * t3 + S5[1] * t4,
            x[0] + C5[1] * t1 + C5[0] * t2, S5[1] * t3 - S5[0] * t4)


def _radix5_t(z0, zc1, zs1, zc2, zs2, k):
    z0 = z0 * k
    p1 = z0 + (k * C5[0]) * zc1 + (k * C5[1]) * zc2
    p2 = z0 + (k * C5[1]) * zc1 + (k * C5[0]) * zc2
    q1 = (k * S5[0]) * zs1 + (k * S5[1]) * zs2
    q2 = (k * S5[1]) * zs1 - (k * S5[0]) * zs2
    return z0 + (zc1 + zc2) * k, p1 + q1, p2 + q2, p2 - q2, p1 - q1


def _kernel(xa_hbm, mem_hbm, wq_hbm, wk_hbm, wv_hbm, wo_hbm, xb_hbm, wr_hbm, wi_hbm,
            out_hbm,
            xa, mem, wqr, wkr, wvr, wo, xbr, xb, wr, wi, ts, tt, gm,
            wq, wk, wv, vre, vim, rsc, xpk, qpre, obuf, o_scr, stash, fstash,
            sem_in, sem_f, sem_w, sem_out):
    def cp(src, dst, sem):
        return pltpu.make_async_copy(src, dst, sem)

    def xa_copy(p0, n, r0, nr, sem):
        return cp(xa_hbm.at[pl.ds(p0, n), pl.ds(r0, nr), :], xa.at[pl.ds(p0, n), pl.ds(r0, nr), :], sem)

    def rows_copy(src, dst, r0, n, sem):
        return cp(src.at[pl.ds(r0, n)], dst.at[pl.ds(r0, n)], sem)

    def start(*cs):
        for c in cs:
            c.start()

    def wait(*cs):
        for c in cs:
            c.wait()

    c_mem = cp(mem_hbm, mem, sem_in.at[0])
    c_xp = xa_copy(0, NPAIR, 0, QP, sem_in.at[1])
    c_xa0 = xa_copy(0, UA + 1, QP, 64 - QP, sem_in.at[2])
    c_xa1 = xa_copy(UA + 1, NPAIR - UA - 1, QP, 64 - QP, sem_in.at[3])
    c_fn = [rows_copy(wr_hbm, wr, HF, 1, sem_in.at[4]), rows_copy(wi_hbm, wi, HF, 1, sem_in.at[5])]
    c_wo = cp(wo_hbm, wo, sem_in.at[6])
    c_xb = [cp(xb_hbm.at[pl.ds(0, 64), pl.ds(0, 8), :], xbr.at[0, pl.ds(0, 64)], sem_in.at[7]),
            cp(xb_hbm.at[pl.ds(64, 64), pl.ds(0, 8), :], xbr.at[0, pl.ds(64, 64)], sem_in.at[11]),
            cp(xb_hbm.at[:, pl.ds(8, 8), :], xbr.at[1], sem_in.at[8])]
    c_q = [cp(wq_hbm.at[:, :, pl.ds(G * h, G), :], wqr.at[h], sem_in.at[9 + h]) for h in range(2)]
    c_f = lambda i: [rows_copy(wr_hbm, wr, pl.multiple_of(i * FROWS, FROWS), FROWS, sem_f.at[2 * i]),
                     rows_copy(wi_hbm, wi, pl.multiple_of(i * FROWS, FROWS), FROWS, sem_f.at[2 * i + 1])]
    c_k = lambda i: rows_copy(wk_hbm, wkr, i * KPC, KPC, sem_w.at[i])
    c_v = lambda i, n: rows_copy(wv_hbm, wvr, i * VPC[0], n, sem_w.at[2 + i])
    c_xb[0].start()

    def relayout(src, dst, dp, zero):
        ab = pltpu.bitcast(src[dp], u32)
        lo, hi = _unzip_rows(ab[0:G] if zero is None else ab[0:G] | zero, ab[G:])
        dst[0, pl.ds(dp, G, stride=PITCH), :] = lo
        dst[1, pl.ds(dp, G, stride=PITCH), :] = hi

    def relayout_q(h, dp, zero):
        a, b = pltpu.bitcast(wqr[h, dp, 0], u32), pltpu.bitcast(wqr[h, dp, 1], u32)
        lo, hi = _unzip_rows(a if zero is None else a | zero[0:8], b)
        wq[0, pl.ds(8 * h * PITCH + dp, 8, stride=PITCH), :] = lo
        wq[1, pl.ds(8 * h * PITCH + dp, 8, stride=PITCH), :] = hi

    def pacer(jobs, nslot, cost=None):
        toks = []
        cum = np.cumsum([0] + list(cost or [1] * len(jobs)))
        slot = (cum[:-1] + cum[1:]) * nslot // (2 * cum[-1])

        def hook(t):
            k = len(toks)
            for job, sl in zip(jobs, slot):
                if sl == k:
                    job(toks[-1] if toks else None)
            toks.append(token(t))
        return hook

    def token(v):
        return (pltpu.bitcast(v[0:G, 0:128], u32) >> 16) >> 16

    first = lax.broadcasted_iota(jnp.int32, (8, N2), 0) == 0
    pack = lambda v: pltpu.bitcast(v.astype(bf16), u32)
    iota = lambda shape, dim: lax.broadcasted_iota(jnp.int32, shape, dim).astype(f32)

    def rotate(c, sn, cr, sr):
        return c * cr - sn * sr, sn * cr + c * sr

    lane = iota((16, 128), 1)
    c8, s8 = _cos_sin(iota((8, 128), 0) * iota((8, 128), 1), 8)

    def gen_tt(r, carry):
        c0, s0 = _cos_sin((r.astype(f32) + 5.0 * iota((16, 128), 0)) * lane, D)
        sg = jnp.where(r >= 3, 1.0, -1.0)
        for g4 in range(4):
            c, sn = (c0, s0) if g4 == 0 else rotate(c0, s0, c8[g4:g4 + 1], s8[g4:g4 + 1])
            ns = -sn
            if g4 == 0:
                ns = jnp.where(lax.broadcasted_iota(jnp.int32, (16, 128), 0) + r == 0, c8[4:5], ns)
            tt[r, 8 * g4:8 * g4 + 8, 0:128] = pack(c)
            tt[r, 8 * g4:8 * g4 + 8, 128:] = pack(sg * sn)
            tt[r, 32 + 8 * g4:40 + 8 * g4, 0:128] = pack(ns)
            tt[r, 32 + 8 * g4:40 + 8 * g4, 128:] = pack(sg * c)
        return carry
    lax.fori_loop(0, 5, gen_tt, 0)
    c_xb[1].start()

    ts[0, 0:N1, :], ts[1, 0:N1, :] = _cos_sin(iota((16, N2), 0) * lane, S)
    c0, s0 = _cos_sin(iota((16, N2), 0) * lane, N2)
    for a in range(N2 // 16):
        c, sn = (c0, s0) if a == 0 else rotate(c0, s0, c8[a:a + 1], s8[a:a + 1])
        ts[0, N1 + 16 * a:N1 + 16 * a + 16, :] = c
        ts[1, N1 + 16 * a:N1 + 16 * a + 16, :] = sn

    def gen_gm(s1, carry):
        ca, sa = ts[0, pl.ds(s1, 1), :], ts[1, pl.ds(s1, 1), :]
        cb, sb = ts[0, N1:, :], ts[1, N1:, :]
        gm[s1, :, 0:N2] = pack(ca * cb - sa * sb)
        gm[s1, :, N2:] = pack(-(sa * cb + ca * sb))
        return carry
    lax.fori_loop(0, N1, gen_gm, 0)
    c_xb[2].start()

    def dft_mats():
        return (pltpu.bitcast(tt[0, :, 0:128], bf16),
                pltpu.bitcast(jnp.concatenate([tt[1], tt[4]], axis=0), bf16),
                pltpu.bitcast(jnp.concatenate([tt[2], tt[3]], axis=0), bf16))

    nt = (((1,), (1,)), ((), ()))

    def p1a(q, m=None):
        rows = pl.ds(q % 4, N2, stride=4) if m is None else pl.ds(256 * m + q % 4, 64, stride=4)
        xw = [xb[q // 4, j, rows, :] for j in range(NT)]
        us = [_radix5([pltpu.bitcast(sel(v), f32) for v in xw])
              for sel in (lambda v: v << 16, lambda v: v & u32(HI16))]
        us = us[::-1] if m == 1 else us
        u = [jnp.concatenate([us[0][k], us[1][k]], axis=0) for k in range(5)]
        return (u[0].astype(bf16), jnp.concatenate(u[1:3], axis=1).astype(bf16),
                jnp.concatenate(u[3:5], axis=1).astype(bf16))

    def p1b(u):
        x0, x14, x23 = [lax.dot_general(t, v, nt, preferred_element_type=f32) for t, v in zip(dft_mats(), u)]
        return jnp.concatenate([x0, x14[0:128], x23, x14[128:]], axis=0)

    def bins(r, m0=0):
        return pl.ds(r + 5 * m0, 64 - m0, stride=5)

    def p2(q, xdt, hook=None):
        for par in range(2):
            s1 = 2 * q + par
            if isinstance(xdt, tuple):
                low = lax.broadcasted_iota(jnp.int32, (NT * 128, N2), 1) < 64
                x, g = jnp.where(low, xdt[par], xdt[1 - par]), gm[s1]
                g = jnp.concatenate([g[32:], g[0:32]], axis=0) if par else g
            else:
                x, g = xdt[:, par * N2:(par + 1) * N2], gm[s1]
            t = jnp.dot(x.astype(bf16), pltpu.bitcast(g, bf16), preferred_element_type=f32)
            if hook is not None:
                for r in range(5):
                    hook(t[128 * r:])
            t1, t2 = t[:, 0:N2], t[:, N2:]
            vre[s1, pl.ds(0, 8, stride=5), :] = t1[0:8] - jnp.where(first, 0.0, t2[64:72])
            vim[s1, pl.ds(0, 8, stride=5), :] = jnp.where(first, 0.0, t1[64:72]) + t2[0:8]
            vre[s1, HF:HF + 8] = t1[64:72]
            vim[s1, HF:HF + 8] = t2[64:72]
            for r in range(5):
                m0 = 8 if r == 0 else 0
                re, im = slice(128 * r + m0, 128 * r + 64), slice(128 * r + 64 + m0, 128 * r + 128)
                vre[s1, bins(r, m0), :] = t1[re] - t2[im]
                vim[s1, bins(r, m0), :] = t1[im] + t2[re]

    def repack(h, m0, n):
        w = pltpu.bitcast(xbr[h, m0:m0 + n].reshape(8 * n, D), u32)
        for j in range(NT):
            xb[h, j, 4 * m0:4 * (m0 + n), :] = w[:, j * 128:(j + 1) * 128]

    us, xs = {}, {}
    hook = pacer([functools.partial(relayout_q, 0, dp) for dp in range(DP)], 30)
    for op in P12.split():
        q, m = int(op[1]), (int(op[2]) if len(op) > 2 else None)
        if op == 'w0':
            c_xb[0].wait()
            c_q[0].start()
        elif op == 'w1':
            c_xb[1].wait()
            start(c_xp, c_q[1], *c_fn)
        elif op == 'w2':
            c_xb[2].wait()
            start(*c_f(0), *c_f(1))
        elif op == 'w3':
            c_q[0].wait()
            start(c_k(0), c_k(1))
        elif op == 'w4':
            c_xp.wait()
            start(c_v(0, VPC[0]), c_v(1, VPC[1]), c_v(2, VPC[2]))
            xpk[...] = pltpu.bitcast(xa[:, 0:QP, :].reshape(NPAIR * QP, D), u32)
        elif op[0] == 'r':
            repack(q, *((0, N2) if m is None else (64 * m, 64)))
        elif op[0] == 'a':
            us[q, m] = p1a(q, m)
        elif op[0] == 'b':
            xs[q, m] = p1b(us[q, m])
        else:
            p2(q, xs[q, None] if (q, None) in xs else (xs[q, 0], xs[q, 1]), hook if op[0] == 'h' else None)

    def p3(rows, wrows, j, zero=None):
        ps, x = divmod(j, 4)
        slots = [4 * x + a for a in range(4)] if ps == 1 else [4 * b + x for b in range(4)]
        re = [vre[n, rows, :] for n in slots]
        im = [vim[n, rows, :] for n in slots]
        if zero is not None:
            re[0] = pltpu.bitcast(pltpu.bitcast(re[0], u32) | zero[0:8], f32)
            im[0] = pltpu.bitcast(pltpu.bitcast(im[0], u32) | zero[0:8], f32)
        re, im = _fft_list(re, im, +1 if ps == 2 else -1)
        if ps == 1:
            yr, yi = [], []
            for d in range(4):
                k1 = x + 4 * d
                a = wr[wrows, k1 * N2:(k1 + 1) * N2].astype(f32)
                b = wi[wrows, k1 * N2:(k1 + 1) * N2].astype(f32)
                yr.append(re[d] * a - im[d] * b)
                yi.append(re[d] * b + im[d] * a)
            re, im = _fft_list(yr, yi, +1)
        if ps < 2:
            tw = [_twiddle(re[i], im[i], x * i, +1 if ps == 1 else -1) for i in range(4)]
            re, im = [t[0] for t in tw], [t[1] for t in tw]
        for i, n in enumerate(slots):
            vre[n, rows, :] = re[i]
            vim[n, rows, :] = im[i]

    def p4(s1, r):
        zr, zi = vre[s1, bins(r), :], vim[s1, bins(r), :]
        top, bot = jnp.concatenate([zr, zi], axis=1), jnp.concatenate([zi, -zr], axis=1)
        if r == 0:
            f2 = jnp.concatenate([first, first], axis=1)
            nyq = jnp.concatenate([vre[s1, HF:HF + 8, :], vim[s1, HF:HF + 8, :]], axis=1)
            top = jnp.concatenate([jnp.where(f2, 0.5 * top[0:8], top[0:8]), top[8:]], axis=0)
            bot = jnp.concatenate([jnp.where(f2, 0.5 * nyq, bot[0:8]), bot[8:]], axis=0)
        t = lax.dot_general(pltpu.bitcast(gm[s1], bf16), jnp.concatenate([top, bot], axis=0).astype(bf16), nt,
                            preferred_element_type=f32)
        rsc[r, pl.ds(pl.multiple_of(s1 * RPITCH, 8), N2), :] = t
        return t

    def bq(w, g, j, k, hook=None):
        rows = pl.ds(pl.multiple_of(g * PITCH, 8), DP)
        rb = NPAIR * QP // NBQ
        w = pltpu.bitcast(jnp.concatenate([w[0, rows, :], w[1, rows, :]], axis=1), bf16)
        x = pltpu.bitcast(xpk[k * rb // 2:(k + 1) * rb // 2, :], bf16)
        if hook is None:
            t = jnp.dot(x, w, preferred_element_type=f32)
        else:
            t = None
            for c in range(NT):
                u = jnp.dot(x[:, c * 128:(c + 1) * 128], w[c * 128:(c + 1) * 128], preferred_element_type=f32)
                hook(u)
                t = u if t is None else t + u
        qpre[j, k * rb:(k + 1) * rb, :] = t
        return t

    def unit(w, g, j, hook=None):
        for k in range(NBQ):
            bq(w, g, j, k, hook)

    for g in range(3):
        unit(wq, g, g)
    wait(c_q[1], *c_fn)
    start(c_mem, c_xa0)
    c_wo.start(priority=1)
    hook = pacer([functools.partial(p3, slice(HF, HF + 8), slice(HF, HF + 1), j) for j in range(12)]
                 + [functools.partial(relayout_q, 1, dp) for dp in range(DP)], 2 * NBQ * NT)
    unit(wq, 3, 3, hook)
    unit(wq, 4, 4, hook)

    def p3q(i, carry):
        wait(*c_f(i))
        rows = lambda c: pl.ds(pl.multiple_of(i * FROWS + 8 * c, 8), 8)
        hook = pacer([functools.partial(p3, rows(c), rows(c), j) for c in range(FROWS // 8) for j in range(12)],
                     4 * NBQ * NT - 2, P3COST * (FROWS // 8))
        for g in range(4):
            unit(wq, 5 + 4 * i + g, 5 + 4 * i + g, hook)
        return carry
    lax.fori_loop(0, 2, p3q, 0)

    def p4l(i, carry):
        c_k(i).wait()
        hook = pacer([functools.partial(relayout, wkr, wk, i * KPC + d) for d in range(KPC)], 78)
        for k in range(N1 // 2):
            bq(wq, 13 + i, 13 + i, k, hook)
            for r in range(5):
                hook(p4(N1 // 2 * i + k, r))
        return carry
    lax.fori_loop(0, 2, p4l, 0)

    def p5q(q, carry):
        c_v(q, VPC[0]).wait()
        hook = pacer([functools.partial(relayout, wvr, wv, q * VPC[0] + d) for d in range(VPC[0])], 36)
        t0, t1, t2 = dft_mats()
        ns = N1 // RB

        def p5(rb):
            rc = [jnp.concatenate([rsc[j, pl.ds(ns * rb + k, N1, stride=RPITCH), :] for k in range(ns)],
                                  axis=0) for j in range(NT)]
            z0 = jnp.dot(rc[0].astype(bf16), t0, preferred_element_type=f32)
            z1 = jnp.dot(jnp.concatenate([rc[1], rc[4]], axis=1).astype(bf16), t1, preferred_element_type=f32)
            z2 = jnp.dot(jnp.concatenate([rc[2], rc[3]], axis=1).astype(bf16), t2, preferred_element_type=f32)
            ys = _radix5_t(z0, z1[:, 0:128], z1[:, 128:], z2[:, 0:128], z2[:, 128:], 2.0 / (D * S))
            rows = pl.ds(pl.multiple_of(N1 * (ns * rb), N1 * ns), N1 * ns)
            obuf[rows, D:] = jnp.concatenate(ys, axis=1).astype(bf16)
            return z0

        units = [(wk, KG[k] + (KG[3 + k] - KG[k]) * q, G + k + 3 * q) for k in range(3)]
        nb = len(units) * NBQ
        for k in range(nb):
            hook(bq(*units[k // NBQ], k % NBQ))
            for rb in range(k * 16 // nb, (k + 1) * 16 // nb):
                hook(p5(16 * q + rb))
        return carry
    lax.fori_loop(0, 2, p5q, 0)

    wait(c_v(2, VPC[2]), c_mem, c_xa0)
    hook = pacer([functools.partial(relayout, wvr, wv, 2 * VPC[0] + d) for d in range(VPC[2])], 50)
    unit(wq, G - 1, G - 1, hook)
    unit(wk, KG[6], G + 6, hook)

    r = lax.broadcasted_iota(jnp.int32, (2 * L, 2 * L), 0)
    c = lax.broadcasted_iota(jnp.int32, (2 * L, 2 * L), 1)
    rb = r >= L
    cb = c >= L
    rr = jnp.where(rb, r - L, r)
    cc = jnp.where(cb, c - L, c)
    mask = (rb == cb) & ((rr < M) | (rr >= cc))
    scale = E ** -0.5

    def wcol(g, c):
        return (wq, wk, wv)[c // 2][c % 2, g * PITCH:g * PITCH + DP, :]

    def filler(p, i0, i1):
        xn = xa[p, 0:32, :]
        if i0 == i1:
            return
        w = jnp.concatenate([wcol(g, c) for g, c in FG[i0:i1]], axis=1)
        t = jnp.dot(xn, pltpu.bitcast(w, bf16), preferred_element_type=f32)
        for i in range(i0, i1):
            fstash[i] = t[:, (i - i0) * E:(i - i0 + 1) * E]

    def step(lhs, even, p):
        nrow_o = 32 if even else 48
        qkv, ps, acc = {}, {}, [None]

        def proj(g):
            def mm(rows, cols):
                w = jnp.concatenate([wcol(g, c) for c in cols], axis=1)
                return jnp.dot(rows, pltpu.bitcast(w, bf16), preferred_element_type=f32)

            if not even:
                t = mm(lhs, range(6))
            else:
                pre = lambda j: qpre[j, pl.ds(pl.multiple_of(p * QP, QP), QP), :]
                tq = jnp.concatenate([pre(g), mm(lhs[QP:], (0, 1))], axis=0)
                moved = [c for gg, c in FG if gg == g]
                if g in KG:
                    assert not moved
                    tk = jnp.concatenate([pre(G + KG.index(g)), mm(lhs[QP:], (2, 3))], axis=0)
                    t = jnp.concatenate([tq, tk, mm(lhs, (4, 5))], axis=1)
                elif not moved:
                    t = jnp.concatenate([tq, mm(lhs, range(2, 6))], axis=1)
                else:
                    rest = [c for c in range(2, 6) if c not in moved]
                    order = [c for pr in zip(rest, moved + [None] * 4) for c in pr if c is not None]
                    tc = {}
                    for c in order:
                        if c in moved:
                            tc[c] = jnp.concatenate([fstash[FG.index((g, c))], mm(lhs[32:48], (c,))], axis=0)
                        else:
                            tc[c] = mm(lhs, (c,))
                    t = jnp.concatenate([tq] + [tc[c] for c in range(2, 6)], axis=1)
            col = lambda a, i: a[:, i * E:(i + 1) * E]
            if even:
                stash[g] = t[40:48]
                parts = [jnp.concatenate([col(t, 2 * i)[32:40], col(t, 2 * i)[0:32],
                                          col(t, 2 * i + 1)[32:40], col(t, 2 * i + 1)[0:32]], axis=0)
                         for i in range(3)]
            else:
                st = stash[g]
                parts = [jnp.concatenate(
                    [col(t, 2 * i)[16:24], col(st, 2 * i), col(t, 2 * i)[24:32], col(t, 2 * i)[0:16],
                     col(t, 2 * i + 1)[16:24], col(st, 2 * i + 1), col(t, 2 * i + 1)[24:32],
                     col(t, 2 * i + 1)[0:16]], axis=0)
                    for i in range(3)]
            qkv[g] = ((parts[0] * scale).astype(bf16), parts[1].astype(bf16), parts[2].astype(bf16))

        def scores(g):
            q2, k2, _ = qkv[g]
            s = lax.dot_general(q2, k2, (((1,), (1,)), ((), ())), preferred_element_type=f32)
            s = jnp.where(mask, s, -1e9)
            e = jnp.exp(s - jnp.max(s, axis=-1, keepdims=True))
            l = jnp.sum(e, axis=-1, keepdims=True)
            ps[g] = (e * pl.reciprocal(l, approx=True)).astype(bf16)

        def pv(g):
            o2 = jnp.dot(ps[g], qkv[g][2], preferred_element_type=f32)
            o_scr[0:40, (2 * g) * E:(2 * g + 1) * E] = o2[0:40]
            o_scr[0:40, (2 * g + 1) * E:(2 * g + 2) * E] = o2[40:80]

        def wo_chunk(c):
            a, b = CH[c] * 2 * E, CH[c + 1] * 2 * E
            t = jnp.dot(o_scr[0:nrow_o, a:b].astype(bf16), wo[a:b, :], preferred_element_type=f32)
            acc[0] = t if acc[0] is None else acc[0] + t

        ch = 0
        for t in range(G + LAG2):
            if t < G:
                proj(t)
            else:
                assert CH[ch + 1] <= t - LAG2
                wo_chunk(ch)
                ch += 1
            if 0 <= t - LAG1 < G:
                scores(t - LAG1)
            if 0 <= t - LAG2 < G:
                pv(t - LAG2)
        while ch < len(CH) - 1:
            wo_chunk(ch)
            ch += 1
        return acc[0]

    def out_copy(p):
        rows = pl.ds(pl.multiple_of(p * 64, 64), 64)
        return cp(obuf.at[rows, pl.ds(0, D)], out_hbm.at[rows, pl.ds(0, D)], sem_out.at[0])

    def pair(p, mem_v):
        base = pl.multiple_of(p * 64, 64)
        xs = xa[p].astype(f32)
        lhs = jnp.concatenate([xs[0:32], mem_v, xs[32:40]], axis=0).astype(bf16)
        out_e = step(lhs, True, p)
        o_scr[40:48, :] = o_scr[32:40, :]
        pn = jnp.minimum(p + 1, NPAIR - 1)
        filler(pn, 0, NF1)
        lhs = jnp.concatenate([xs[48:64], out_e[0:8], xs[40:48]], axis=0).astype(bf16)
        out_o = step(lhs, False, p)
        filler(pn, NF1, len(FG))
        res = jnp.concatenate([out_e[8:32], out_o[40:48], out_o[8:40]], axis=0)
        obuf[pl.ds(base, 64), 0:D] = res.astype(bf16)
        return out_o[0:8]

    def body(p, mem_v):
        @pl.when(p == 1)
        def _():
            c_xa1.wait()

        @pl.when(p > 0)
        def _():
            out_copy(p * UA - 1).start()
        for k in range(UA):
            if k > 0:
                out_copy(p * UA + k - 1).start()
            mem_v = pair(p * UA + k, mem_v)
        return mem_v

    filler(0, 0, len(FG))
    c_wo.wait()
    c_xa1.start(priority=1)
    cp(obuf.at[:, pl.ds(D, D)], out_hbm.at[:, pl.ds(D, D)], sem_out.at[0]).start()
    lax.fori_loop(0, NPAIR // UA, body, mem[...].astype(f32))

    out_copy(NPAIR - 1).start()
    cp(obuf, obuf, sem_out.at[0]).wait()


@jax.jit
def pallas_concat_heads__memory_aug_recurrent_mem_tr__spectral_gfnet__prompt_kernel(
    A_x: jax.Array,
    A_mem0: jax.Array,
    A_Wq: jax.Array,
    A_Wk: jax.Array,
    A_Wv: jax.Array,
    A_Wo: jax.Array,
    A_seg_len,
    B_x: jax.Array,
    B_w_r: jax.Array,
    B_w_i: jax.Array,
):
    del A_seg_len
    assert A_x.shape == (1, S, D) and B_x.shape == (1, S, D)
    args = (
        A_x.reshape(NPAIR, 64, D), A_mem0.reshape(M, D),
        A_Wq.reshape(DP, 2, H, E), A_Wk.reshape(DP, 2 * H, E), A_Wv.reshape(DP, 2 * H, E),
        A_Wo.reshape(H * E, D),
        B_x.reshape(N2, N1, D), B_w_r.T, B_w_i.T,
    )
    V = pltpu.VMEM
    scratch = [
        V((NPAIR, 64, D), bf16), V((M, D), bf16),
        V((2, DP, 2, G, E), bf16), V((DP, 2 * H, E), bf16), V((DP, 2 * H, E), bf16), V((H * E, D), bf16),
        V((2, N2, 8, D), bf16), V((2, NT, S // 4 + 8, 128), u32), V((DF, S), bf16), V((DF, S), bf16),
        V((2, N1 + N2, N2), f32), V((5, 64, 256), u32), V((N1, N2 // 2, 2 * N2), u32),
        V((2, (G + 1) * PITCH, E), u32), V((2, (G + 1) * PITCH, E), u32), V((2, (G + 1) * PITCH, E), u32),
        V((N1, HF + 8, N2), f32), V((N1, HF + 8, N2), f32),
        V((NT, (N1 + 1) * RPITCH, 128), f32), V((NPAIR * QP // 2, D), u32),
        V((G + len(KG), NPAIR * QP, 2 * E), f32),
        V((S, 2 * D), bf16), V((48, H * E), f32), V((G, 8, 6 * E), f32), V((len(FG), 32, E), f32),
        pltpu.SemaphoreType.DMA((12,)), pltpu.SemaphoreType.DMA((4,)), pltpu.SemaphoreType.DMA((5,)),
        pltpu.SemaphoreType.DMA((1,)),
    ]
    out = pl.pallas_call(
        _kernel,
        out_shape=jax.ShapeDtypeStruct((S, 2 * D), bf16),
        in_specs=[pl.BlockSpec(memory_space=pltpu.HBM)] * len(args),
        out_specs=pl.BlockSpec(memory_space=pl.ANY),
        scratch_shapes=scratch,
        compiler_params=pltpu.CompilerParams(vmem_limit_bytes=110 * 1024 * 1024, disable_bounds_checks=True),
    )(*args)
    return out.reshape(1, S, 2 * D)
```

```python
import functools
import numpy as np
import jax
import jax.numpy as jnp
from jax import lax
import jax.experimental.pallas as pl
import jax.experimental.pallas.tpu as pltpu

bf16 = jnp.bfloat16
f32 = jnp.float32
u32 = jnp.uint32

S, D = 2048, 640
H, E = 32, 128
M, SEG = 8, 32
L = M + SEG
G = H // 2
DF = D // 2 + 1
HF = D // 2
NT = D // 128
N1, N2 = 16, 128
NPAIR = S // (2 * SEG)
LAG1, LAG2 = 2, 5
CH = (0, 4, 7, 10, 12, 13, 14, 15, 16)
DP = D // 2
PITCH = DP + 8
KPC = DP // 2
VPC = (120, 120, 80)
RB = 4
FG = [(4, 4), (8, 4), (12, 4), (14, 4)]
NF1 = 2
NBQ = 8
FROWS = HF // 2
KG = (0, 1, 2, 10, 13, 15, 6)
RPITCH = N2 + 8
UA = 2
QP = 16
C5 = (float(np.cos(2 * np.pi / 5)), float(np.cos(4 * np.pi / 5)))
S5 = (float(np.sin(2 * np.pi / 5)), float(np.sin(4 * np.pi / 5)))
HI16 = 0xFFFF0000
P12 = ('w0 r00 a00 a10 a20 a30 b00 b10 b20 w1 b30 r01 a01 a11 b01 b11 a21 a31 b21 b31 c0 c1 '
       'w2 c2 r1 a4 a5 c3 b4 b5 a6 a7 b6 b7 c4 c5 w3 h6 h7 w4')
P3COST = (24, 40, 33, 40, 72, 88, 81, 88, 24, 24, 24, 24)


def _cos_sin(num, den):
    r = num - den * jnp.floor((num + 0.5) * (1.0 / den))
    ang = r * (2.0 * np.pi / den)
    return jnp.cos(ang), jnp.sin(ang)


def _fft_list(re, im, sign):
    n = len(re)
    if n == 1:
        return re, im
    er, ei = _fft_list(re[0::2], im[0::2], sign)
    orr, oi = _fft_list(re[1::2], im[1::2], sign)
    h = n // 2
    outr = [None] * n
    outi = [None] * n
    r = np.float32(np.sqrt(0.5))
    for k in range(h):
        a, b = orr[k], oi[k]
        if 4 * k == n:
            if sign > 0:
                outr[k], outi[k] = er[k] - b, ei[k] + a
                outr[k + h], outi[k + h] = er[k] + b, ei[k] - a
            else:
                outr[k], outi[k] = er[k] + b, ei[k] - a
                outr[k + h], outi[k + h] = er[k] - b, ei[k] + a
            continue
        if k == 0:
            tr, ti = a, b
        elif 8 * k == n:
            tr, ti = ((a - b) * r, (a + b) * r) if sign > 0 else ((a + b) * r, (b - a) * r)
        elif 8 * k == 3 * n:
            tr, ti = ((a + b) * (-r), (a - b) * r) if sign > 0 else ((b - a) * r, (a + b) * (-r))
        else:
            c = np.float32(np.cos(2 * np.pi * k / n))
            s = np.float32(sign * np.sin(2 * np.pi * k / n))
            tr, ti = a * c - b * s, a * s + b * c
        outr[k], outi[k] = er[k] + tr, ei[k] + ti
        outr[k + h], outi[k + h] = er[k] - tr, ei[k] - ti
    return outr, outi


def _twiddle(a, b, m, sign):
    m %= 16
    if m == 0:
        return a, b
    if m == 4:
        return (-b, a) if sign > 0 else (b, -a)
    r = np.float32(np.sqrt(0.5))
    if m == 2:
        return ((a - b) * r, (a + b) * r) if sign > 0 else ((a + b) * r, (b - a) * r)
    if m == 6:
        return ((a + b) * (-r), (a - b) * r) if sign > 0 else ((b - a) * r, (a + b) * (-r))
    c = np.float32(np.cos(2 * np.pi * m / 16))
    s = np.float32(sign * np.sin(2 * np.pi * m / 16))
    return a * c - b * s, a * s + b * c


def _unzip_rows(a, b):
    lo = (a & u32(0xFFFF)) | (b << 16)
    hi = (a >> 16) | (b & u32(HI16))
    return lo, hi


def _radix5(x):
    t1, t2, t3, t4 = x[1] + x[4], x[2] + x[3], x[1] - x[4], x[2] - x[3]
    return (x[0] + t1 + t2,
            x[0] + C5[0] * t1 + C5[1] * t2, S5[0] * t3 + S5[1] * t4,
            x[0] + C5[1] * t1 + C5[0] * t2, S5[1] * t3 - S5[0] * t4)


def _radix5_t(z0, zc1, zs1, zc2, zs2, k):
    z0 = z0 * k
    p1 = z0 + (k * C5[0]) * zc1 + (k * C5[1]) * zc2
    p2 = z0 + (k * C5[1]) * zc1 + (k * C5[0]) * zc2
    q1 = (k * S5[0]) * zs1 + (k * S5[1]) * zs2
    q2 = (k * S5[1]) * zs1 - (k * S5[0]) * zs2
    return z0 + (zc1 + zc2) * k, p1 + q1, p2 + q2, p2 - q2, p1 - q1


def _kernel(xa_hbm, mem_hbm, wq_hbm, wk_hbm, wv_hbm, wo_hbm, xb_hbm, wr_hbm, wi_hbm,
            out_hbm,
            xa, mem, wqr, wkr, wvr, wo, xbr, xb, wr, wi, ts, tt, gm, gp,
            wq, wk, wv, vre, vim, rsc, xpk, qpre, obuf, o_scr, stash, fstash,
            sem_in, sem_f, sem_w, sem_out):
    def cp(src, dst, sem):
        return pltpu.make_async_copy(src, dst, sem)

    def xa_copy(p0, n, r0, nr, sem):
        return cp(xa_hbm.at[pl.ds(p0, n), pl.ds(r0, nr), :], xa.at[pl.ds(p0, n), pl.ds(r0, nr), :], sem)

    def rows_copy(src, dst, r0, n, sem):
        return cp(src.at[pl.ds(r0, n)], dst.at[pl.ds(r0, n)], sem)

    def start(*cs):
        for c in cs:
            c.start()

    def wait(*cs):
        for c in cs:
            c.wait()

    c_mem = cp(mem_hbm, mem, sem_in.at[0])
    c_xp = xa_copy(0, NPAIR, 0, QP, sem_in.at[1])
    c_xa0 = xa_copy(0, UA + 1, QP, 64 - QP, sem_in.at[2])
    c_xa1 = xa_copy(UA + 1, NPAIR - UA - 1, QP, 64 - QP, sem_in.at[3])
    c_fn = [rows_copy(wr_hbm, wr, HF, 1, sem_in.at[4]), rows_copy(wi_hbm, wi, HF, 1, sem_in.at[5])]
    c_wo = cp(wo_hbm, wo, sem_in.at[6])
    c_xb = [cp(xb_hbm.at[pl.ds(0, 64), pl.ds(0, 8), :], xbr.at[0, pl.ds(0, 64)], sem_in.at[7]),
            cp(xb_hbm.at[pl.ds(64, 64), pl.ds(0, 8), :], xbr.at[0, pl.ds(64, 64)], sem_in.at[11]),
            cp(xb_hbm.at[:, pl.ds(8, 8), :], xbr.at[1], sem_in.at[8])]
    c_q = [cp(wq_hbm.at[:, :, pl.ds(G * h, G), :], wqr.at[h], sem_in.at[9 + h]) for h in range(2)]
    c_f = lambda i: [rows_copy(wr_hbm, wr, pl.multiple_of(i * FROWS, FROWS), FROWS, sem_f.at[2 * i]),
                     rows_copy(wi_hbm, wi, pl.multiple_of(i * FROWS, FROWS), FROWS, sem_f.at[2 * i + 1])]
    c_k = lambda i: rows_copy(wk_hbm, wkr, i * KPC, KPC, sem_w.at[i])
    c_v = lambda i, n: rows_copy(wv_hbm, wvr, i * VPC[0], n, sem_w.at[2 + i])
    c_xb[0].start()

    def relayout(src, dst, dp, zero):
        ab = pltpu.bitcast(src[dp], u32)
        lo, hi = _unzip_rows(ab[0:G] if zero is None else ab[0:G] | zero, ab[G:])
        dst[0, pl.ds(dp, G, stride=PITCH), :] = lo
        dst[1, pl.ds(dp, G, stride=PITCH), :] = hi

    def relayout_q(h, dp, zero):
        a, b = pltpu.bitcast(wqr[h, dp, 0], u32), pltpu.bitcast(wqr[h, dp, 1], u32)
        lo, hi = _unzip_rows(a if zero is None else a | zero[0:8], b)
        wq[0, pl.ds(8 * h * PITCH + dp, 8, stride=PITCH), :] = lo
        wq[1, pl.ds(8 * h * PITCH + dp, 8, stride=PITCH), :] = hi

    def pacer(jobs, nslot, cost=None):
        toks = []
        cum = np.cumsum([0] + list(cost or [1] * len(jobs)))
        slot = (cum[:-1] + cum[1:]) * nslot // (2 * cum[-1])

        def hook(t):
            k = len(toks)
            for job, sl in zip(jobs, slot):
                if sl == k:
                    job(toks[-1] if toks else None)
            toks.append(token(t))
        return hook

    def token(v):
        return (pltpu.bitcast(v[0:G, 0:128], u32) >> 16) >> 16

    first = lax.broadcasted_iota(jnp.int32, (8, N2), 0) == 0
    pack = lambda v: pltpu.bitcast(v.astype(bf16), u32)
    iota = lambda shape, dim: lax.broadcasted_iota(jnp.int32, shape, dim).astype(f32)

    def rotate(c, sn, cr, sr):
        return c * cr - sn * sr, sn * cr + c * sr

    lane = iota((16, 128), 1)
    c8, s8 = _cos_sin(iota((8, 128), 0) * iota((8, 128), 1), 8)

    def gen_tt(r, carry):
        c0, s0 = _cos_sin((r.astype(f32) + 5.0 * iota((16, 128), 0)) * lane, D)
        sg = jnp.where(r >= 3, 1.0, -1.0)
        for g4 in range(4):
            c, sn = (c0, s0) if g4 == 0 else rotate(c0, s0, c8[g4:g4 + 1], s8[g4:g4 + 1])
            ns = -sn
            if g4 == 0:
                ns = jnp.where(lax.broadcasted_iota(jnp.int32, (16, 128), 0) == 0, c8[4:5], ns)
            tt[r, 8 * g4:8 * g4 + 8, 0:128] = pack(c)
            tt[r, 8 * g4:8 * g4 + 8, 128:256] = pack(jnp.where(r == 0, ns, sg * sn - c))
            tt[r, 8 * g4:8 * g4 + 8, 256:] = pack(sg * c + sn)
        return carry
    lax.fori_loop(0, 5, gen_tt, 0)
    start(c_xb[1], *c_fn)

    ts[0, 0:N1, :], ts[1, 0:N1, :] = _cos_sin(iota((16, N2), 0) * lane, S)
    c0, s0 = _cos_sin(iota((16, N2), 0) * lane, N2)
    for a in range(N2 // 16):
        c, sn = (c0, s0) if a == 0 else rotate(c0, s0, c8[a:a + 1], s8[a:a + 1])
        ts[0, N1 + 16 * a:N1 + 16 * a + 16, :] = c
        ts[1, N1 + 16 * a:N1 + 16 * a + 16, :] = sn

    def gen_gm(s1, carry):
        ca, sa = ts[0, pl.ds(s1, 1), :], ts[1, pl.ds(s1, 1), :]
        cb, sb = ts[0, N1:, :], ts[1, N1:, :]
        gm[s1, :, 0:N2] = pack(ca * cb - sa * sb)
        gm[s1, :, N2:] = pack(-(sa * cb + ca * sb))
        return carry
    lax.fori_loop(0, N1, gen_gm, 0)
    c_xb[2].start()

    def gen_gp(s1, c, zero):
        ca, sa = ts[0, s1:s1 + 1, :], ts[1, s1:s1 + 1, :]
        cb, sb = ts[0, N1 + 32 * c:N1 + 32 * c + 32, :], ts[1, N1 + 32 * c:N1 + 32 * c + 32, :]
        if zero is not None:
            ca = pltpu.bitcast(pltpu.bitcast(ca, u32) | zero[0:1], f32)
        u, v = ca + sa, ca - sa
        gp[s1, 16 * c:16 * c + 16, 0:N2] = pack(sb * u - cb * v)
        gp[s1, 16 * c:16 * c + 16, N2:] = pack(cb * u + sb * v)

    def dft_mat(k, j):
        if k == 0:
            return pltpu.bitcast(jnp.concatenate([tt[0, :, 0:128], tt[0, :, 128:256]], axis=0), bf16)
        cols = slice(128 * j, 128 * j + 128)
        return pltpu.bitcast(jnp.concatenate([tt[k, :, cols], tt[5 - k, :, cols]], axis=0), bf16)

    nt = (((1,), (1,)), ((), ()))

    def p1a(q, m=None):
        rows = pl.ds(q % 4, N2, stride=4) if m is None else pl.ds(256 * m + q % 4, 64, stride=4)
        xw = [xb[q // 4, j, rows, :] for j in range(NT)]
        us = [_radix5([pltpu.bitcast(sel(v), f32) for v in xw])
              for sel in (lambda v: v << 16, lambda v: v & u32(HI16))]
        us = us[::-1] if m == 1 else us
        u = [jnp.concatenate([us[0][k], us[1][k]], axis=0) for k in range(5)]
        return [v.astype(bf16) for v in (u[0], u[1], u[2], u[1] + u[2], u[3], u[4], u[3] + u[4])]

    def p1b(u):
        mm = lambda t, v: lax.dot_general(t, v, nt, preferred_element_type=f32)
        x = [mm(dft_mat(0, 0), u[0])]
        for k in (1, 2):
            c, sn, cs = u[3 * k - 2:3 * k + 1]
            k2, k3, k1 = mm(dft_mat(k, 1), sn), mm(dft_mat(k, 2), c), mm(dft_mat(k, 0), cs)
            x += [k1 + k2, k1[0:64] + k3[0:64], k1[64:] - k3[64:]]
        return jnp.concatenate(x, axis=0)

    def bins(r, m0=0):
        return pl.ds(r + 5 * m0, 64 - m0, stride=5)

    def p2(q, xdt, hook=None):
        for par in range(2):
            s1 = 2 * q + par
            if isinstance(xdt, tuple):
                low = lax.broadcasted_iota(jnp.int32, (NT * 128, N2), 1) < 64
                x, g = jnp.where(low, xdt[par], xdt[1 - par]), gm[s1]
                g = jnp.concatenate([g[32:], g[0:32]], axis=0) if par else g
            else:
                x, g = xdt[:, par * N2:(par + 1) * N2], gm[s1]
            t = jnp.dot(x.astype(bf16), pltpu.bitcast(g, bf16), preferred_element_type=f32)
            if hook is not None:
                for r in range(5):
                    hook(t[128 * r:])
            t1, t2 = t[:, 0:N2], t[:, N2:]
            vre[s1, pl.ds(0, 8, stride=5), :] = t1[0:8] - jnp.where(first, 0.0, t2[64:72])
            vim[s1, pl.ds(0, 8, stride=5), :] = jnp.where(first, 0.0, t1[64:72]) + t2[0:8]
            vre[s1, HF:HF + 8] = t1[64:72]
            vim[s1, HF:HF + 8] = t2[64:72]
            for r in range(5):
                m0 = 8 if r == 0 else 0
                r0, i0 = ((0, 64), (128, 256), (384, 512), (448, 576), (192, 320))[r]
                re, im = slice(r0 + m0, r0 + 64), slice(i0 + m0, i0 + 64)
                if r in (1, 2):
                    vre[s1, bins(r), :] = t1[re] + t2[im]
                    vim[s1, bins(r), :] = t2[re] - t1[im]
                else:
                    vre[s1, bins(r, m0), :] = t1[re] - t2[im]
                    vim[s1, bins(r, m0), :] = t1[im] + t2[re]

    def repack(h, m0, n):
        w = pltpu.bitcast(xbr[h, m0:m0 + n].reshape(8 * n, D), u32)
        for j in range(NT):
            xb[h, j, 4 * m0:4 * (m0 + n), :] = w[:, j * 128:(j + 1) * 128]

    us, xs = {}, {}
    hook = pacer([functools.partial(relayout_q, 0, dp) for dp in range(DP)], 19)
    for op in P12.split():
        q, m = int(op[1]), (int(op[2]) if len(op) > 2 else None)
        if op == 'w0':
            c_xb[0].wait()
            c_q[0].start()
        elif op == 'w1':
            c_xb[1].wait()
            start(c_xp, c_q[1])
        elif op == 'w2':
            c_xb[2].wait()
            start(*c_f(0), *c_f(1))
        elif op == 'w3':
            c_q[0].wait()
            start(c_k(0), c_k(1))
        elif op == 'w4':
            wait(c_xp, *c_fn)
            start(c_v(0, VPC[0]), c_v(1, VPC[1]), c_v(2, VPC[2]))
            xpk[...] = pltpu.bitcast(xa[:, 0:QP, :].reshape(NPAIR * QP, D), u32)
        elif op[0] == 'r':
            repack(q, *((0, N2) if m is None else (64 * m, 64)))
        elif op[0] == 'a':
            us[q, m] = p1a(q, m)
        elif op[0] == 'b':
            xs[q, m] = p1b(us[q, m])
        else:
            p2(q, xs[q, None] if (q, None) in xs else (xs[q, 0], xs[q, 1]), hook if op[0] == 'h' else None)

    def p3(rows, wrows, j, zero=None):
        ps, x = divmod(j, 4)
        slots = [4 * x + a for a in range(4)] if ps == 1 else [4 * b + x for b in range(4)]
        re = [vre[n, rows, :] for n in slots]
        im = [vim[n, rows, :] for n in slots]
        if zero is not None:
            re[0] = pltpu.bitcast(pltpu.bitcast(re[0], u32) | zero[0:8], f32)
            im[0] = pltpu.bitcast(pltpu.bitcast(im[0], u32) | zero[0:8], f32)
        re, im = _fft_list(re, im, +1 if ps == 2 else -1)
        if ps == 1:
            yr, yi = [], []
            for d in range(4):
                k1 = x + 4 * d
                a = wr[wrows, k1 * N2:(k1 + 1) * N2].astype(f32)
                b = wi[wrows, k1 * N2:(k1 + 1) * N2].astype(f32)
                yr.append(re[d] * a - im[d] * b)
                yi.append(re[d] * b + im[d] * a)
            re, im = _fft_list(yr, yi, +1)
        if ps < 2:
            tw = [_twiddle(re[i], im[i], x * i, +1 if ps == 1 else -1) for i in range(4)]
            re, im = [t[0] for t in tw], [t[1] for t in tw]
        for i, n in enumerate(slots):
            vre[n, rows, :] = re[i]
            vim[n, rows, :] = im[i]

    def p4(s1, k, hook):
        rows = pl.ds(pl.multiple_of(s1 * RPITCH, 8), N2)
        if k == 0:
            zr, zi = vre[s1, bins(0), :], vim[s1, bins(0), :]
            top, bot = jnp.concatenate([zr, zi], axis=1), jnp.concatenate([zi, -zr], axis=1)
            f2 = jnp.concatenate([first, first], axis=1)
            nyq = jnp.concatenate([vre[s1, HF:HF + 8, :], vim[s1, HF:HF + 8, :]], axis=1)
            top = jnp.concatenate([jnp.where(f2, 0.5 * top[0:8], top[0:8]), top[8:]], axis=0)
            bot = jnp.concatenate([jnp.where(f2, 0.5 * nyq, bot[0:8]), bot[8:]], axis=0)
            t = lax.dot_general(pltpu.bitcast(gm[s1], bf16), jnp.concatenate([top, bot], axis=0).astype(bf16), nt,
                                preferred_element_type=f32)
            hook(t)
            rsc[0, rows, :] = t
            return
        zr = jnp.concatenate([vre[s1, bins(k), :], vre[s1, bins(5 - k), :]], axis=0)
        zi = jnp.concatenate([vim[s1, bins(k), :], vim[s1, bins(5 - k), :]], axis=0)
        mm = lambda g, z: lax.dot_general(pltpu.bitcast(g, bf16), z.astype(bf16), nt, preferred_element_type=f32)
        k2, k3, k1 = mm(gp[s1, :, 0:N2], zr), mm(gp[s1, :, N2:], zi), mm(gm[s1, :, 0:N2], zr + zi)
        hook(k2)
        hook(k1)
        rsc[k, rows, :] = k1 - k3
        rsc[5 - k, rows, :] = k1 + k2

    def bq(w, g, j, k, hook=None):
        rows = pl.ds(pl.multiple_of(g * PITCH, 8), DP)
        rb = NPAIR * QP // NBQ
        w = pltpu.bitcast(jnp.concatenate([w[0, rows, :], w[1, rows, :]], axis=1), bf16)
        x = pltpu.bitcast(xpk[k * rb // 2:(k + 1) * rb // 2, :], bf16)
        if hook is None:
            t = jnp.dot(x, w, preferred_element_type=f32)
        else:
            t = None
            for c in range(NT):
                u = jnp.dot(x[:, c * 128:(c + 1) * 128], w[c * 128:(c + 1) * 128], preferred_element_type=f32)
                hook(u)
                t = u if t is None else t + u
        qpre[j, k * rb:(k + 1) * rb, :] = t
        return t

    def unit(w, g, j, hook=None):
        for k in range(NBQ):
            bq(w, g, j, k, hook)

    hook = pacer([functools.partial(p3, slice(HF, HF + 8), slice(HF, HF + 1), j) for j in range(12)]
                 + [functools.partial(gen_gp, s1, c) for s1 in range(N1) for c in range(4)], 3 * NBQ * NT - 4)
    for g in range(3):
        unit(wq, g, g, hook)
    c_q[1].wait()
    start(c_mem, c_xa0)
    c_wo.start(priority=1)
    hook = pacer([functools.partial(relayout_q, 1, dp) for dp in range(DP)], 76)
    unit(wq, 3, 3, hook)
    unit(wq, 4, 4, hook)

    def p3q(i, carry):
        wait(*c_f(i))
        rows = lambda c: pl.ds(pl.multiple_of(i * FROWS + 8 * c, 8), 8)
        hook = pacer([functools.partial(p3, rows(c), rows(c), j) for c in range(FROWS // 8) for j in range(12)],
                     4 * NBQ * NT, P3COST * (FROWS // 8))
        for g in range(4):
            unit(wq, 5 + 4 * i + g, 5 + 4 * i + g, hook)
        return carry
    lax.fori_loop(0, 2, p3q, 0)

    def p4l(i, carry):
        c_k(i).wait()
        hook = pacer([functools.partial(relayout, wkr, wk, i * KPC + d) for d in range(KPC)], 78)
        for k in range(N1 // 2):
            bq(wq, 13 + i, 13 + i, k, hook)
            for r in range(3):
                p4(N1 // 2 * i + k, r, hook)
        return carry
    lax.fori_loop(0, 2, p4l, 0)

    def p5q(q, carry):
        c_v(q, VPC[0]).wait()
        hook = pacer([functools.partial(relayout, wvr, wv, q * VPC[0] + d) for d in range(VPC[0])], 36)
        low = lax.broadcasted_iota(jnp.int32, (N1 * N1 // RB, 128), 1) < 64
        ns = N1 // RB

        def p5(rb):
            rc = [jnp.concatenate([rsc[j, pl.ds(ns * rb + k, N1, stride=RPITCH), :] for k in range(ns)],
                                  axis=0) for j in range(NT)]
            mm = lambda z, t: jnp.dot(z.astype(bf16), t, preferred_element_type=f32)
            z0, z = mm(rc[0], dft_mat(0, 0)), []
            for k in (1, 2):
                a, b = rc[k], rc[5 - k]
                k2 = mm(a, dft_mat(k, 1))
                k3 = mm(b, dft_mat(k, 2))
                k1 = mm(jnp.where(low, a - b, a + b), dft_mat(k, 0))
                z += [k1 - k3, k1 + k2]
            ys = _radix5_t(z0, *z, 2.0 / (D * S))
            rows = pl.ds(pl.multiple_of(N1 * (ns * rb), N1 * ns), N1 * ns)
            obuf[rows, D:] = jnp.concatenate(ys, axis=1).astype(bf16)
            return z0

        units = [(wk, KG[k] + (KG[3 + k] - KG[k]) * q, G + k + 3 * q) for k in range(3)]
        nb = len(units) * NBQ
        for k in range(nb):
            hook(bq(*units[k // NBQ], k % NBQ))
            for rb in range(k * 16 // nb, (k + 1) * 16 // nb):
                hook(p5(16 * q + rb))
        return carry
    lax.fori_loop(0, 2, p5q, 0)

    wait(c_v(2, VPC[2]), c_mem, c_xa0)
    hook = pacer([functools.partial(relayout, wvr, wv, 2 * VPC[0] + d) for d in range(VPC[2])], 50)
    unit(wq, G - 1, G - 1, hook)
    unit(wk, KG[6], G + 6, hook)

    r = lax.broadcasted_iota(jnp.int32, (2 * L, 2 * L), 0)
    c = lax.broadcasted_iota(jnp.int32, (2 * L, 2 * L), 1)
    rb = r >= L
    cb = c >= L
    rr = jnp.where(rb, r - L, r)
    cc = jnp.where(cb, c - L, c)
    mask = (rb == cb) & ((rr < M) | (rr >= cc))
    scale = E ** -0.5

    def wcol(g, c):
        return (wq, wk, wv)[c // 2][c % 2, g * PITCH:g * PITCH + DP, :]

    def filler(p, i0, i1):
        xn = xa[p, 0:32, :]
        if i0 == i1:
            return
        w = jnp.concatenate([wcol(g, c) for g, c in FG[i0:i1]], axis=1)
        t = jnp.dot(xn, pltpu.bitcast(w, bf16), preferred_element_type=f32)
        for i in range(i0, i1):
            fstash[i] = t[:, (i - i0) * E:(i - i0 + 1) * E]

    def step(lhs, even, p):
        nrow_o = 32 if even else 48
        qkv, ps, acc = {}, {}, [None]

        def proj(g):
            def mm(rows, cols):
                w = jnp.concatenate([wcol(g, c) for c in cols], axis=1)
                return jnp.dot(rows, pltpu.bitcast(w, bf16), preferred_element_type=f32)

            if not even:
                t = mm(lhs, range(6))
            else:
                pre = lambda j: qpre[j, pl.ds(pl.multiple_of(p * QP, QP), QP), :]
                tq = jnp.concatenate([pre(g), mm(lhs[QP:], (0, 1))], axis=0)
                moved = [c for gg, c in FG if gg == g]
                if g in KG:
                    assert not moved
                    tk = jnp.concatenate([pre(G + KG.index(g)), mm(lhs[QP:], (2, 3))], axis=0)
                    t = jnp.concatenate([tq, tk, mm(lhs, (4, 5))], axis=1)
                elif not moved:
                    t = jnp.concatenate([tq, mm(lhs, range(2, 6))], axis=1)
                else:
                    rest = [c for c in range(2, 6) if c not in moved]
                    order = [c for pr in zip(rest, moved + [None] * 4) for c in pr if c is not None]
                    tc = {}
                    for c in order:
                        if c in moved:
                            tc[c] = jnp.concatenate([fstash[FG.index((g, c))], mm(lhs[32:48], (c,))], axis=0)
                        else:
                            tc[c] = mm(lhs, (c,))
                    t = jnp.concatenate([tq] + [tc[c] for c in range(2, 6)], axis=1)
            col = lambda a, i: a[:, i * E:(i + 1) * E]
            if even:
                stash[g] = t[40:48]
                parts = [jnp.concatenate([col(t, 2 * i)[32:40], col(t, 2 * i)[0:32],
                                          col(t, 2 * i + 1)[32:40], col(t, 2 * i + 1)[0:32]], axis=0)
                         for i in range(3)]
            else:
                st = stash[g]
                parts = [jnp.concatenate(
                    [col(t, 2 * i)[16:24], col(st, 2 * i), col(t, 2 * i)[24:32], col(t, 2 * i)[0:16],
                     col(t, 2 * i + 1)[16:24], col(st, 2 * i + 1), col(t, 2 * i + 1)[24:32],
                     col(t, 2 * i + 1)[0:16]], axis=0)
                    for i in range(3)]
            qkv[g] = ((parts[0] * scale).astype(bf16), parts[1].astype(bf16), parts[2].astype(bf16))

        def scores(g):
            q2, k2, _ = qkv[g]
            s = lax.dot_general(q2, k2, (((1,), (1,)), ((), ())), preferred_element_type=f32)
            s = jnp.where(mask, s, -1e9)
            e = jnp.exp(s - jnp.max(s, axis=-1, keepdims=True))
            l = jnp.sum(e, axis=-1, keepdims=True)
            r0 = pl.reciprocal(l, approx=True)
            ps[g] = (e * (r0 * (2.0 - l * r0))).astype(bf16)

        def pv(g):
            o2 = jnp.dot(ps[g], qkv[g][2], preferred_element_type=f32)
            o_scr[0:40, (2 * g) * E:(2 * g + 1) * E] = o2[0:40]
            o_scr[0:40, (2 * g + 1) * E:(2 * g + 2) * E] = o2[40:80]

        def wo_chunk(c):
            a, b = CH[c] * 2 * E, CH[c + 1] * 2 * E
            t = jnp.dot(o_scr[0:nrow_o, a:b].astype(bf16), wo[a:b, :], preferred_element_type=f32)
            acc[0] = t if acc[0] is None else acc[0] + t

        ch = 0
        for t in range(G + LAG2):
            if t < G:
                proj(t)
            else:
                assert CH[ch + 1] <= t - LAG2
                wo_chunk(ch)
                ch += 1
            if 0 <= t - LAG1 < G:
                scores(t - LAG1)
            if 0 <= t - LAG2 < G:
                pv(t - LAG2)
        while ch < len(CH) - 1:
            wo_chunk(ch)
            ch += 1
        return acc[0]

    def out_copy(p):
        rows = pl.ds(pl.multiple_of(p * 64, 64), 64)
        return cp(obuf.at[rows, pl.ds(0, D)], out_hbm.at[rows, pl.ds(0, D)], sem_out.at[0])

    def pair(p, mem_v):
        base = pl.multiple_of(p * 64, 64)
        xs = xa[p].astype(f32)
        lhs = jnp.concatenate([xs[0:32], mem_v, xs[32:40]], axis=0).astype(bf16)
        out_e = step(lhs, True, p)
        o_scr[40:48, :] = o_scr[32:40, :]
        pn = jnp.minimum(p + 1, NPAIR - 1)
        filler(pn, 0, NF1)
        lhs = jnp.concatenate([xs[48:64], out_e[0:8], xs[40:48]], axis=0).astype(bf16)
        out_o = step(lhs, False, p)
        filler(pn, NF1, len(FG))
        res = jnp.concatenate([out_e[8:32], out_o[40:48], out_o[8:40]], axis=0)
        obuf[pl.ds(base, 64), 0:D] = res.astype(bf16)
        return out_o[0:8]

    def body(p, mem_v):
        @pl.when(p == 1)
        def _():
            c_xa1.wait()

        @pl.when(p > 0)
        def _():
            out_copy(p * UA - 1).start()
        for k in range(UA):
            if k > 0:
                out_copy(p * UA + k - 1).start()
            mem_v = pair(p * UA + k, mem_v)
        return mem_v

    filler(0, 0, len(FG))
    c_wo.wait()
    c_xa1.start(priority=1)
    cp(obuf.at[:, pl.ds(D, D)], out_hbm.at[:, pl.ds(D, D)], sem_out.at[0]).start()
    lax.fori_loop(0, NPAIR // UA, body, mem[...].astype(f32))

    out_copy(NPAIR - 1).start()
    cp(obuf, obuf, sem_out.at[0]).wait()


@jax.jit
def pallas_concat_heads__memory_aug_recurrent_mem_tr__spectral_gfnet__prompt_kernel(
    A_x: jax.Array,
    A_mem0: jax.Array,
    A_Wq: jax.Array,
    A_Wk: jax.Array,
    A_Wv: jax.Array,
    A_Wo: jax.Array,
    A_seg_len,
    B_x: jax.Array,
    B_w_r: jax.Array,
    B_w_i: jax.Array,
):
    del A_seg_len
    assert A_x.shape == (1, S, D) and B_x.shape == (1, S, D)
    args = (
        A_x.reshape(NPAIR, 64, D), A_mem0.reshape(M, D),
        A_Wq.reshape(DP, 2, H, E), A_Wk.reshape(DP, 2 * H, E), A_Wv.reshape(DP, 2 * H, E),
        A_Wo.reshape(H * E, D),
        B_x.reshape(N2, N1, D), B_w_r.T, B_w_i.T,
    )
    V = pltpu.VMEM
    scratch = [
        V((NPAIR, 64, D), bf16), V((M, D), bf16),
        V((2, DP, 2, G, E), bf16), V((DP, 2 * H, E), bf16), V((DP, 2 * H, E), bf16), V((H * E, D), bf16),
        V((2, N2, 8, D), bf16), V((2, NT, S // 4 + 8, 128), u32), V((DF, S), bf16), V((DF, S), bf16),
        V((2, N1 + N2, N2), f32), V((5, 32, 384), u32),
        V((N1, N2 // 2, 2 * N2), u32), V((N1, N2 // 2, 2 * N2), u32),
        V((2, (G + 1) * PITCH, E), u32), V((2, (G + 1) * PITCH, E), u32), V((2, (G + 1) * PITCH, E), u32),
        V((N1, HF + 8, N2), f32), V((N1, HF + 8, N2), f32),
        V((NT, (N1 + 1) * RPITCH, 128), f32), V((NPAIR * QP // 2, D), u32),
        V((G + len(KG), NPAIR * QP, 2 * E), f32),
        V((S, 2 * D), bf16), V((48, H * E), f32), V((G, 8, 6 * E), f32), V((len(FG), 32, E), f32),
        pltpu.SemaphoreType.DMA((12,)), pltpu.SemaphoreType.DMA((4,)), pltpu.SemaphoreType.DMA((5,)),
        pltpu.SemaphoreType.DMA((1,)),
    ]
    out = pl.pallas_call(
        _kernel,
        out_shape=jax.ShapeDtypeStruct((S, 2 * D), bf16),
        in_specs=[pl.BlockSpec(memory_space=pltpu.HBM)] * len(args),
        out_specs=pl.BlockSpec(memory_space=pl.ANY),
        scratch_shapes=scratch,
        compiler_params=pltpu.CompilerParams(vmem_limit_bytes=110 * 1024 * 1024, disable_bounds_checks=True),
    )(*args)
    return out.reshape(1, S, 2 * D)
```
